```python
import os as _os
_os.environ.setdefault("JAX_PLATFORMS", "cpu")
import jax
import jax.numpy as jnp

def _softmax(x, axis=-1):
    return jax.nn.softmax(x, axis=axis)
def _gelu(x):
    return jax.nn.gelu(x, approximate=True)
def _silu(x):
    return jax.nn.silu(x)
def _sigmoid(x):
    return jax.nn.sigmoid(x)
def _layernorm(x, axis=-1, eps=1e-5):
    m = jnp.mean(x, axis=axis, keepdims=True)
    v = jnp.var(x, axis=axis, keepdims=True)
    return (x - m) / jnp.sqrt(v + eps)
def _scatter_add(tgt, idx, src, axis=0):
    return tgt.at[idx].add(src)
def _segment_sum(src, seg, n):
    return jax.ops.segment_sum(src, seg, n)
class _Rng:
    def __init__(self, key):
        self._k = key
    def _next(self):
        self._k, sub = jax.random.split(self._k)
        return sub
    def normal(self, shape):
        return jax.random.normal(self._next(), shape, dtype=jnp.bfloat16)
    def randint(self, lo, hi, shape):
        return jax.random.randint(self._next(), shape, lo, hi, dtype=jnp.int32)
    def uniform(self, shape, lo=0.0, hi=1.0):
        return jax.random.uniform(self._next(), shape, jnp.bfloat16, lo, hi)
    def permutation(self, n):
        return jax.random.permutation(self._next(), n)


kernel_name = 'standalone__layernorm_linear__sampling'

def setup_inputs():
    _rng = _Rng(jax.random.key(int.from_bytes(__import__("os").urandom(4), "little")))
    _w = (lambda a: (lambda t: t.astype(jnp.bfloat16) if jnp.issubdtype(t.dtype, jnp.floating) else t)(jnp.asarray(a)))
    B, S, D = 1024, 32, 576
    return {
        "x": _w((lambda *s: _rng.normal(s) * 0.05)(B, S, D)),
        "g": _w((lambda *s: _rng.normal(s) * 0.05)(D) + 1.0),
        "b": _w((lambda *s: _rng.normal(s) * 0.05)(D)),
        "w": _w((lambda *s: _rng.normal(s) * 0.05)(D, D)),
    }

def reference(x, g, b, w):
    return (_layernorm(x, axis=-1) * g + b) @ w
```

```python
import functools

import jax
import jax.numpy as jnp
import jax.experimental.pallas as pl
import jax.experimental.pallas.tpu as pltpu

F32 = jnp.float32
BF16 = jnp.bfloat16
U32 = jnp.uint32

EPS = 1e-5
D = 576
H = D // 2
KH = 256
KR = D - 2 * KH
KX = KR + 16
GW = 512
N_RAMP = 3
SPB = 4
T_END = 7.5


def _pack(v):
    return pltpu.bitcast(v, U32)


def _unpack(v):
    return pltpu.bitcast(v, BF16)


def _prep_weights(g_ref, b_ref, w_ref, a_ref, ar_ref):
    g = g_ref[...].astype(F32).reshape(1, D)
    b16 = jnp.broadcast_to(b_ref[...].reshape(1, D), (16, D))
    c = jnp.dot(b16, w_ref[...], preferred_element_type=F32)
    c_hi = c.astype(BF16).astype(F32)
    rest = c - c_hi
    c_mid = rest.astype(BF16).astype(F32)
    c_lo = rest - c_mid
    row = jax.lax.broadcasted_iota(jnp.int32, (16, D), 0)
    ext = jnp.where(row == 0, c_hi,
                    jnp.where(row == 1, c_mid,
                              jnp.where(row == 2, c_lo, 0.0))).astype(BF16)
    wr = jnp.concatenate(
        [w_ref[2 * KH:, :], ext, jnp.zeros((128 - KX, D), BF16)], axis=0)
    gr = jnp.concatenate([g[:, 2 * KH:], jnp.ones((1, 128 - KR), F32)], axis=1)
    ar_ref[...] = _pack((wr.astype(F32).T * gr).astype(BF16))
    w1 = w_ref[:KH, :].astype(F32).T * g[:, :KH]
    w2 = w_ref[KH:2 * KH, :].astype(F32).T * g[:, KH:2 * KH]
    a11, a21, a12, a22 = w1[:H], w1[H:], w2[:H], w2[H:]
    ops = [a11 + a22, a21 + a22, a11, a22, a11 + a12, a21 - a11, a12 - a22]
    for t in range(7):
        a_ref[t] = _pack(ops[t].astype(BF16))


class _Norm:
    def __init__(self, x_ref, col0, q, zb, zr):
        self.x, self.q, self.zb, self.zr = x_ref, q, zb, zr
        self.cs = pl.ds(col0, 256)
        self.stat_items = [(functools.partial(self.stat, r0, 32), 40)
                           for r0 in range(0, D, 32)]
        self.out_items = [(functools.partial(self.bside, r0, 16), 41)
                          for r0 in range(0, KH, 16)]
        self.out_items += [(functools.partial(self.brem, r0, 32), 28)
                           for r0 in range(0, KR, 32)]
        self.s1 = self.s2 = self.p = self.m = self.r = None

    def stat(self, r0, rows, tie):
        if self.p is None:
            first = self.x[0:16, self.cs].astype(F32)[0:1, :]
            self.p = jnp.broadcast_to(first, (8, 256))
        p = tie(self.p)
        xf = self.x[r0:r0 + rows, self.cs].astype(F32).reshape(rows // 8, 8, 256)
        s1 = s2 = None
        for t in range(rows // 8):
            d = xf[t] - p
            s1 = d if s1 is None else s1 + d
            s2 = d * d if s2 is None else s2 + d * d
        self.s1 = s1 if self.s1 is None else self.s1 + s1
        self.s2 = s2 if self.s2 is None else self.s2 + s2
        if r0 + rows == D:
            e1 = jnp.sum(self.s1, axis=0, keepdims=True) * (1.0 / D)
            e2 = jnp.sum(self.s2, axis=0, keepdims=True) * (1.0 / D)
            var = jnp.maximum(e2 - e1 * e1, 0.0)
            self.m = self.p + e1
            self.r = jnp.broadcast_to(jax.lax.rsqrt(var + EPS), (8, 256))

    def z(self, r0, rows, m):
        xf = self.x[r0:r0 + rows, self.cs].astype(F32).reshape(rows // 8, 8, 256)
        return ((xf - m[None]) * self.r[None]).reshape(rows, 256)

    def bside(self, r0, rows, tie):
        m = tie(self.m)
        top, bot = self.z(r0, rows, m), self.z(KH + r0, rows, m)
        b11, b12, b21, b22 = top[:, :128], top[:, 128:], bot[:, :128], bot[:, 128:]
        ops = [b11 + b22, b11, b12 - b22, b21 - b11, b22, b11 + b12, b21 + b22]
        for t in range(0, 6, 2):
            self.zb[t // 2, self.q, r0:r0 + rows, :] = jnp.concatenate(
                [ops[t], ops[t + 1]], axis=1).astype(BF16)
        self.zb[3, self.q, r0:r0 + rows, :128] = ops[6].astype(BF16)

    def brem(self, r0, rows, tie):
        z = self.z(2 * KH + r0, rows, tie(self.m))
        self.zr[self.q, r0:r0 + rows, :] = z.astype(BF16)


def _norm_items(x_ref, col0, zb, zr):
    n0 = _Norm(x_ref, col0, 0, zb, zr)
    n1 = _Norm(x_ref, col0 + 256, 1, zb, zr)
    return n0.stat_items + n1.stat_items + n0.out_items + n1.out_items


def _mm_group(a_ref, ar_ref, zb, zr, o_ref, col0, items, never):
    total = sum(cost for _, cost in items)
    pos, cum = [], 0
    for _, cost in items:
        pos.append(T_END * cum / total)
        cum += cost
    ms, k = [], 0
    for t in range(8):
        if t < 7:
            lanes = pl.ds(128 * (t % 2), 128)
            bt = jnp.concatenate([zb[t // 2, q, :, lanes] for q in range(2)], axis=1)
            mt = jnp.dot(_unpack(a_ref[t]), bt, preferred_element_type=F32)
            ms.append(mt)
            lo, hi, rows = t, t + 1, H
        else:
            br = jnp.concatenate([zr[q] for q in range(2)], axis=1)
            mt = rem = jnp.dot(_unpack(ar_ref[...])[:, :KX], br,
                               preferred_element_type=F32)
            lo, hi, rows = 7, 9, D
        while k < len(items) and pos[k] < hi:
            rr = min(rows - 8, int((pos[k] - lo) / (hi - lo) * rows) // 8 * 8)
            src = mt[rr:rr + 8, :128]
            src = jnp.concatenate([src, src], axis=1)
            items[k][0](lambda v, src=src: jnp.where(never, src, v))
            k += 1
    c11 = ms[0] + ms[3] - ms[4] + ms[6]
    c12 = ms[2] + ms[4]
    c21 = ms[1] + ms[3]
    c22 = ms[0] - ms[1] + ms[2] + ms[5]
    for j in range(2):
        sl = slice(128 * j, 128 * j + 128)
        cols = slice(256 * j, 256 * j + 256)
        top = jnp.concatenate([c11[:, sl], c12[:, sl]], axis=1) + rem[:H, cols]
        bot = jnp.concatenate([c21[:, sl], c22[:, sl]], axis=1) + rem[H:, cols]
        dst = pl.ds(col0 + 256 * j, 256)
        o_ref[:H, dst] = top.astype(BF16)
        o_ref[H:, dst] = bot.astype(BF16)


def _kernel(x_hbm, g_hbm, b_hbm, w_hbm, o_hbm,
            xbuf, obuf, gbuf, bbuf, wbuf, a_ref, ar_ref, zb0, zr0, zb1, zr1,
            sem_x0, sem_w, sem_x, sem_o):
    S = xbuf.shape[0]
    n_body = (S - 1 - N_RAMP) // SPB

    def x0_copy(h):
        cols = pl.ds(GW * h, GW)
        return pltpu.make_async_copy(x_hbm.at[0, :, cols], xbuf.at[0, :, cols],
                                     sem_x0.at[h])

    def x_copy(s):
        return pltpu.make_async_copy(x_hbm.at[s], xbuf.at[s], sem_x.at[s])

    def o_half_copy(s, h):
        cols = pl.ds(GW * h, GW)
        return pltpu.make_async_copy(obuf.at[s, :, cols], o_hbm.at[s, :, cols], sem_o)

    def o_copy(s):
        return pltpu.make_async_copy(obuf.at[s], o_hbm.at[s], sem_o)

    w_copies = [pltpu.make_async_copy(g_hbm, gbuf, sem_w.at[0]),
                pltpu.make_async_copy(b_hbm, bbuf, sem_w.at[1]),
                pltpu.make_async_copy(w_hbm, wbuf, sem_w.at[2])]

    x0_copy(0).start()
    for c in w_copies:
        c.start()
    x0_copy(1).start()

    row = jax.lax.broadcasted_iota(jnp.int32, (2, 16, 256), 1)
    ones = jnp.where(row < 3, 1.0, 0.0).astype(BF16)
    zr0[:, KR:, :] = ones
    zr1[:, KR:, :] = ones

    x0_copy(0).wait()
    for item, _ in _norm_items(xbuf.at[0], 0, zb0, zr0):
        item(lambda v: v)
    for c in w_copies:
        c.wait()
    for s in range(1, S):
        x_copy(s).start()
    _prep_weights(gbuf, bbuf, wbuf, a_ref, ar_ref)
    gv = jnp.broadcast_to(gbuf[...].astype(F32).reshape(1, D)[:, :256], (8, 256))
    never = gv != gv
    x0_copy(1).wait()

    def slab(i, write, wait_next=False):
        xi, oi = xbuf.at[i], obuf.at[i]
        _mm_group(a_ref, ar_ref, zb0, zr0, oi, 0,
                  _norm_items(xi, GW, zb1, zr1), never)
        if write:
            o_half_copy(i, 0).start()
        if wait_next:
            x_copy(i + 1).wait()
        nxt = jnp.minimum(i + 1, S - 1)
        _mm_group(a_ref, ar_ref, zb1, zr1, oi, GW,
                  _norm_items(xbuf.at[nxt], 0, zb0, zr0), never)
        if write:
            o_half_copy(i, 1).start()

    slab(0, False, wait_next=True)

    def ramp_body(i, carry):
        x_copy(i + 1).wait()
        slab(i, False)
        return carry

    jax.lax.fori_loop(1, 1 + N_RAMP, ramp_body, 0)

    def body(j, carry):
        i0 = 1 + N_RAMP + j * SPB
        for u in range(SPB - 1):
            x_copy(i0 + u + 1).wait()

        @pl.when(j < n_body - 1)
        def _():
            x_copy(i0 + SPB).wait()

        @pl.when(j == 1)
        def _():
            for s in range(1 + N_RAMP):
                o_copy(s).start()

        for u in range(SPB):
            slab(i0 + u, True)
        return carry

    jax.lax.fori_loop(0, n_body, body, 0)
    pltpu.make_async_copy(obuf, o_hbm, sem_o).wait()


@jax.jit
def pallas_standalone__layernorm_linear__sampling_kernel(
    x: jax.Array,
    g: jax.Array,
    b: jax.Array,
    w: jax.Array,
):
    B, S, d = x.shape
    assert d == D and B == 2 * GW and (S - 1 - N_RAMP) % SPB == 0
    xt = jnp.transpose(x, (1, 2, 0))
    out = pl.pallas_call(
        _kernel,
        in_specs=[pl.BlockSpec(memory_space=pl.ANY)] * 4,
        out_specs=pl.BlockSpec(memory_space=pl.ANY),
        out_shape=jax.ShapeDtypeStruct((S, D, B), x.dtype),
        scratch_shapes=[
            pltpu.VMEM((S, D, B), BF16),
            pltpu.VMEM((S, D, B), BF16),
            pltpu.VMEM((D,), BF16),
            pltpu.VMEM((D,), BF16),
            pltpu.VMEM((D, D), BF16),
            pltpu.VMEM((7, H // 2, KH), U32),
            pltpu.VMEM((D // 2, 128), U32),
            pltpu.VMEM((4, 2, KH, 256), BF16),
            pltpu.VMEM((2, KX, 256), BF16),
            pltpu.VMEM((4, 2, KH, 256), BF16),
            pltpu.VMEM((2, KX, 256), BF16),
            pltpu.SemaphoreType.DMA((2,)),
            pltpu.SemaphoreType.DMA((3,)),
            pltpu.SemaphoreType.DMA((S,)),
            pltpu.SemaphoreType.DMA(()),
        ],
        compiler_params=pltpu.CompilerParams(
            vmem_limit_bytes=110 * 1024 * 1024,
            disable_bounds_checks=True,
            disable_semaphore_checks=True,
        ),
    )(xt, g, b, w)
    return jnp.transpose(out, (2, 0, 1))
```

```python
import functools

import jax
import jax.numpy as jnp
import jax.experimental.pallas as pl
import jax.experimental.pallas.tpu as pltpu

F32 = jnp.float32
BF16 = jnp.bfloat16
U32 = jnp.uint32

EPS = 1e-5
D = 576
H = D // 2
Q = H // 2
KH = 256
KR = D - 2 * KH
KX = KR + 16
GW = 512
N_RAMP = 3
SPB = 4
W_START = 12

DEEP = (1, 2, 3, 4)
FLAT = (0, 6, 5)
PHASES = (0, 1008, 1296, 1584, 1872, 2448)
ROOM = (0.9, 1.25, 1.1, 1.1, 1.0)
T_END = 0.76 * PHASES[-1]

TILE = {}
for _t in DEEP:
    for _u in range(7):
        TILE[(_t, _u)] = len(TILE)
for _t in FLAT:
    for _h in range(2):
        for _p in range(2):
            TILE[(_t, _h, _p)] = len(TILE)
N_TILES = len(TILE)


def _pack(v):
    return pltpu.bitcast(v, U32)


def _unpack(v):
    return pltpu.bitcast(v, BF16)


def _a_ops(a11, a12, a21, a22):
    return [a11 + a22, a21 + a22, a11, a22, a11 + a12, a21 - a11, a12 - a22]


def _b_op(t, b11, b12, b21, b22):
    return [lambda: b11 + b22, lambda: b11, lambda: b12 - b22, lambda: b21 - b11,
            lambda: b22, lambda: b11 + b12, lambda: b21 + b22][t]()


def _prep_weights(g_ref, b_ref, w_ref, a1_ref, a2_ref, ar_ref):
    g = g_ref[...].astype(F32).reshape(1, D)
    b16 = jnp.broadcast_to(b_ref[...].reshape(1, D), (16, D))
    c = jnp.dot(b16, w_ref[...], preferred_element_type=F32)
    c_hi = c.astype(BF16).astype(F32)
    rest = c - c_hi
    c_mid = rest.astype(BF16).astype(F32)
    c_lo = rest - c_mid
    row = jax.lax.broadcasted_iota(jnp.int32, (16, D), 0)
    ext = jnp.where(row == 0, c_hi,
                    jnp.where(row == 1, c_mid,
                              jnp.where(row == 2, c_lo, 0.0))).astype(BF16)
    wr = jnp.concatenate(
        [w_ref[2 * KH:, :], ext, jnp.zeros((128 - KX, D), BF16)], axis=0)
    gr = jnp.concatenate([g[:, 2 * KH:], jnp.ones((1, 128 - KR), F32)], axis=1)
    ar_ref[...] = _pack((wr.astype(F32).T * gr).astype(BF16))
    w1 = w_ref[:KH, :].astype(F32).T * g[:, :KH]
    w2 = w_ref[KH:2 * KH, :].astype(F32).T * g[:, KH:2 * KH]
    ops = _a_ops(w1[:H], w2[:H], w1[H:], w2[H:])
    for i, t in enumerate(FLAT):
        a1_ref[i] = _pack(ops[t].astype(BF16))
    for i, t in enumerate(DEEP):
        a = ops[t]
        sub = _a_ops(a[:Q, :128], a[:Q, 128:], a[Q:, :128], a[Q:, 128:])
        for u in range(0, 6, 2):
            a2_ref[i, u // 2] = _pack(
                jnp.concatenate([sub[u], sub[u + 1]], axis=1).astype(BF16))
        a2_ref[i, 3, :, :128] = _pack(sub[6].astype(BF16))


class _Stats:
    def __init__(self, x_ref, col0):
        self.x, self.cs = x_ref, pl.ds(col0, 256)
        self.items = [(functools.partial(self.stat, r0, 32), 40)
                      for r0 in range(0, D, 32)]
        self.s1 = self.s2 = self.p = self.m = self.r = None

    def stat(self, r0, rows, tie):
        if self.p is None:
            first = self.x[0:16, self.cs].astype(F32)[0:1, :]
            self.p = jnp.broadcast_to(first, (8, 256))
        p = tie(self.p)
        xf = self.x[r0:r0 + rows, self.cs].astype(F32).reshape(rows // 8, 8, 256)
        s1 = s2 = None
        for t in range(rows // 8):
            d = xf[t] - p
            s1 = d if s1 is None else s1 + d
            s2 = d * d if s2 is None else s2 + d * d
        self.s1 = s1 if self.s1 is None else self.s1 + s1
        self.s2 = s2 if self.s2 is None else self.s2 + s2
        if r0 + rows == D:
            e1 = jnp.sum(self.s1, axis=0, keepdims=True) * (1.0 / D)
            e2 = jnp.sum(self.s2, axis=0, keepdims=True) * (1.0 / D)
            var = jnp.maximum(e2 - e1 * e1, 0.0)
            self.m = self.p + e1
            self.r = jnp.broadcast_to(jax.lax.rsqrt(var + EPS), (8, 256))

    def z(self, r0, rows, m):
        xf = self.x[r0:r0 + rows, self.cs].astype(F32).reshape(rows // 8, 8, 256)
        return ((xf - m[None]) * self.r[None]).reshape(rows, 256)


def _norm_items(x_ref, col0, zb, zr):
    st = [_Stats(x_ref, col0), _Stats(x_ref, col0 + 256)]
    held = {}

    def sums(j):
        tiles = [None] * N_TILES
        for t in DEEP + FLAT:
            bt = {}
            for p in range(2):
                z = held[(j, p)]
                for h in range(2):
                    bt[(h, p)] = _b_op(t, z[h][:, :128], z[h][:, 128:],
                                       z[2 + h][:, :128], z[2 + h][:, 128:])
            if t in DEEP:
                for u in range(7):
                    tiles[TILE[(t, u)]] = _b_op(u, bt[(0, 0)], bt[(0, 1)],
                                                bt[(1, 0)], bt[(1, 1)])
            else:
                for key, val in bt.items():
                    tiles[TILE[(t,) + key]] = val
        for e in range(0, N_TILES, 2):
            zb[e // 2, j:j + 8, :] = jnp.concatenate(
                [tiles[e], tiles[e + 1]], axis=1).astype(BF16)

    def zpart(j, p, tie):
        m = tie(st[p].m)
        held[(j, p)] = [st[p].z(128 * kq + j, 8, m) for kq in range(4)]
        if p == 1:
            sums(j)

    def zrem(p, r0, tie):
        z = st[p].z(2 * KH + r0, 32, tie(st[p].m))
        zr[r0:r0 + 32, pl.ds(256 * p, 256)] = z.astype(BF16)

    items = st[0].items + st[1].items
    items += [(functools.partial(zrem, 0, r0), 28) for r0 in range(0, KR, 32)]
    for j in range(0, 128, 8):
        items.append((functools.partial(zpart, j, 0), 24))
        items.append((functools.partial(zpart, j, 1), 84))
    items += [(functools.partial(zrem, 1, r0), 28) for r0 in range(0, KR, 32)]
    return items


def _time_slots(items):
    segs = [(PHASES[i], min(PHASES[i + 1], T_END), ROOM[i])
            for i in range(5) if PHASES[i] < T_END]
    room = sum((b - a) * d for a, b, d in segs)
    total = sum(cost for _, cost in items)
    pos, cum = [], 0
    for _, cost in items:
        c = room * cum / total
        for a, b, d in segs:
            if c <= (b - a) * d + 1e-9:
                pos.append(a + c / d)
                break
            c -= (b - a) * d
        cum += cost
    return pos


def _mm_group(a1_ref, a2_ref, ar_ref, e_ref, t_ref, zb, zr, o_ref, col0, items,
              never):
    pos = _time_slots(items)
    state = [0, 0]

    def release(mt, span):
        lo = state[1]
        rows = mt.shape[0]
        while state[0] < len(items) and pos[state[0]] < lo + span:
            rr = min(rows - 8, int((pos[state[0]] - lo) / span * rows) // 8 * 8)
            src = mt[rr:rr + 8, :128]
            src = jnp.concatenate([src, src], axis=1)
            items[state[0]][0](lambda v, src=src: jnp.where(never, src, v))
            state[0] += 1
        state[1] += span

    def tile(key):
        e = TILE[key]
        return zb[e // 2, :, pl.ds(128 * (e % 2), 128)]

    for u in range(7):
        p = {}
        for i, t in enumerate(DEEP):
            a = _unpack(a2_ref[i, u // 2, :, pl.ds(128 * (u % 2), 128)])
            p[t] = jnp.dot(a, tile((t, u)), preferred_element_type=F32)
        e_ref[0, u] = p[3] - p[4]
        e_ref[1, u] = p[2] + p[4]
        e_ref[2, u] = p[1] + p[3]
        e_ref[3, u] = p[2] - p[1]
        release(p[1], 144)

    def flat(i):
        t = FLAT[i]
        bt = jnp.concatenate(
            [jnp.concatenate([tile((t, h, p)) for p in range(2)], axis=1)
             for h in range(2)], axis=0)
        return jnp.dot(_unpack(a1_ref[i]), bt, preferred_element_type=F32)

    m1 = flat(0)
    t_ref[0] = m1
    release(m1, 288)
    m7 = flat(1)
    t_ref[1] = m7 + t_ref[0]
    release(m7, 288)
    m6 = flat(2)
    t_ref[2] = m6 + t_ref[0]
    release(m6, 288)
    rem = jnp.dot(_unpack(ar_ref[...])[:, :KX], zr[...], preferred_element_type=F32)
    release(rem, 576)

    def family(f, base):
        e = [e_ref[f, u] for u in range(7)]
        x11 = base[:Q, :128] + e[0] + e[3] - e[4] + e[6]
        x12 = base[:Q, 128:] + e[2] + e[4]
        x21 = base[Q:, :128] + e[1] + e[3]
        x22 = base[Q:, 128:] + e[0] - e[1] + e[2] + e[5]
        return jnp.concatenate([jnp.concatenate([x11, x12], axis=1),
                                jnp.concatenate([x21, x22], axis=1)], axis=0)

    rem_l = jnp.concatenate([rem[:, 0:128], rem[:, 256:384]], axis=1)
    rem_r = jnp.concatenate([rem[:, 128:256], rem[:, 384:512]], axis=1)
    c11 = family(0, rem_l[:H] + t_ref[1])
    c12 = family(1, rem_r[:H])
    c21 = family(2, rem_l[H:])
    c22 = family(3, rem_r[H:] + t_ref[2])
    for j in range(2):
        sl = slice(128 * j, 128 * j + 128)
        dst = pl.ds(col0 + 256 * j, 256)
        o_ref[:H, dst] = jnp.concatenate([c11[:, sl], c12[:, sl]], axis=1).astype(BF16)
        o_ref[H:, dst] = jnp.concatenate([c21[:, sl], c22[:, sl]], axis=1).astype(BF16)


def _kernel(x_hbm, g_hbm, b_hbm, w_hbm, o_hbm,
            xbuf, obuf, gbuf, bbuf, wbuf, a1_ref, a2_ref, ar_ref, e_ref, t_ref,
            zb0, zr0, zb1, zr1, sem_x0, sem_w, sem_x, sem_o):
    S = xbuf.shape[0]
    n_body = (S - 1 - N_RAMP) // SPB

    def x0_copy(h):
        cols = pl.ds(GW * h, GW)
        return pltpu.make_async_copy(x_hbm.at[0, :, cols], xbuf.at[0, :, cols],
                                     sem_x0.at[h])

    def x_copy(s):
        return pltpu.make_async_copy(x_hbm.at[s], xbuf.at[s], sem_x.at[s])

    def o_half_copy(s, h):
        cols = pl.ds(GW * h, GW)
        return pltpu.make_async_copy(obuf.at[s, :, cols], o_hbm.at[s, :, cols], sem_o)

    def o_copy(s):
        return pltpu.make_async_copy(obuf.at[s], o_hbm.at[s], sem_o)

    w_copies = [pltpu.make_async_copy(g_hbm, gbuf, sem_w.at[0]),
                pltpu.make_async_copy(b_hbm, bbuf, sem_w.at[1]),
                pltpu.make_async_copy(w_hbm, wbuf, sem_w.at[2])]

    first = [x0_copy(0)] + w_copies + [x0_copy(1)]

    def issue_first(k, carry):
        for kk, cp in enumerate(first):
            pl.when(k == kk)(cp.start)
        return carry

    jax.lax.fori_loop(0, len(first), issue_first, 0)

    def issue_x(s, carry):
        x_copy(s).start()
        return carry

    jax.lax.fori_loop(1, S, issue_x, 0)

    row = jax.lax.broadcasted_iota(jnp.int32, (16, GW), 0)
    ones = jnp.where(row < 3, 1.0, 0.0).astype(BF16)
    zr0[KR:, :] = ones
    zr1[KR:, :] = ones

    x0_copy(0).wait()
    for item, _ in _norm_items(xbuf.at[0], 0, zb0, zr0):
        item(lambda v: v)
    for c in w_copies:
        c.wait()
    _prep_weights(gbuf, bbuf, wbuf, a1_ref, a2_ref, ar_ref)
    x0_copy(1).wait()
    gv = jnp.broadcast_to(gbuf[...].astype(F32).reshape(1, D)[:, :256], (8, 256))
    never = gv != gv
    mm = functools.partial(_mm_group, a1_ref, a2_ref, ar_ref, e_ref, t_ref)

    def slab(i, write, wait_next=False):
        xi, oi = xbuf.at[i], obuf.at[i]
        mm(zb0, zr0, oi, 0, _norm_items(xi, GW, zb1, zr1), never)
        if write:
            pl.when(i == S - 1)(o_half_copy(i, 0).start)
        if wait_next:
            x_copy(i + 1).wait()
        nxt = jnp.minimum(i + 1, S - 1)
        mm(zb1, zr1, oi, GW, _norm_items(xbuf.at[nxt], 0, zb0, zr0), never)
        if write:
            pl.when(i == S - 1)(o_half_copy(i, 1).start)
            pl.when(jnp.logical_and(i >= W_START, i < S - 1))(o_copy(i).start)

    slab(0, False, wait_next=True)

    def ramp_body(i, carry):
        x_copy(i + 1).wait()
        slab(i, False)
        return carry

    jax.lax.fori_loop(1, 1 + N_RAMP, ramp_body, 0)

    def body(j, carry):
        i0 = 1 + N_RAMP + j * SPB
        for u in range(SPB - 1):
            x_copy(i0 + u + 1).wait()
        pl.when(j < n_body - 1)(x_copy(jnp.minimum(i0 + SPB, S - 1)).wait)

        @pl.when(i0 == W_START)
        def _():
            def flush(s, c):
                o_copy(s).start()
                return c
            jax.lax.fori_loop(0, W_START, flush, 0)

        for u in range(SPB):
            slab(i0 + u, True)
        return carry

    jax.lax.fori_loop(0, n_body, body, 0)
    pltpu.make_async_copy(obuf, o_hbm, sem_o).wait()


@jax.jit
def pallas_standalone__layernorm_linear__sampling_kernel(
    x: jax.Array,
    g: jax.Array,
    b: jax.Array,
    w: jax.Array,
):
    B, S, d = x.shape
    assert d == D and B == 2 * GW and (S - 1 - N_RAMP) % SPB == 0
    assert (W_START - 1 - N_RAMP) % SPB == 0
    xt = jnp.transpose(x, (1, 2, 0))
    out = pl.pallas_call(
        _kernel,
        in_specs=[pl.BlockSpec(memory_space=pl.ANY)] * 4,
        out_specs=pl.BlockSpec(memory_space=pl.ANY),
        out_shape=jax.ShapeDtypeStruct((S, D, B), x.dtype),
        scratch_shapes=[
            pltpu.VMEM((S, D, B), BF16),
            pltpu.VMEM((S, D, B), BF16),
            pltpu.VMEM((D,), BF16),
            pltpu.VMEM((D,), BF16),
            pltpu.VMEM((D, D), BF16),
            pltpu.VMEM((3, H // 2, KH), U32),
            pltpu.VMEM((4, 4, Q // 2, 256), U32),
            pltpu.VMEM((D // 2, 128), U32),
            pltpu.VMEM((4, 7, Q, 128), F32),
            pltpu.VMEM((3, H, 256), F32),
            pltpu.VMEM((N_TILES // 2, 128, 256), BF16),
            pltpu.VMEM((KX, GW), BF16),
            pltpu.VMEM((N_TILES // 2, 128, 256), BF16),
            pltpu.VMEM((KX, GW), BF16),
            pltpu.SemaphoreType.DMA((2,)),
            pltpu.SemaphoreType.DMA((3,)),
            pltpu.SemaphoreType.DMA((S,)),
            pltpu.SemaphoreType.DMA(()),
        ],
        compiler_params=pltpu.CompilerParams(
            vmem_limit_bytes=110 * 1024 * 1024,
            disable_bounds_checks=True,
            disable_semaphore_checks=True,
        ),
    )(xt, g, b, w)
    return jnp.transpose(out, (2, 0, 1))
```

```python
import functools

import jax
import jax.numpy as jnp
import jax.experimental.pallas as pl
import jax.experimental.pallas.tpu as pltpu

F32 = jnp.float32
BF16 = jnp.bfloat16
U32 = jnp.uint32

EPS = 1e-5
D = 576
H = D // 2
Q = H // 2
KH = 256
KR = D - 2 * KH
KX = KR + 16
GW = 512
RAMP = (1, 2)
SPB = 4
W_START = 14

DEEP = (1, 2, 3, 4, 5, 6)
A_IDX = {(t, u): 7 * i + u for i, t in enumerate(DEEP) for u in range(7)}
TILE = {}
for _t in (1, 4, 2, 5, 3, 6):
    for _u in range(7):
        TILE[(_t, _u)] = len(TILE)
for _h in range(2):
    for _p in range(2):
        TILE[(0, _h, _p)] = len(TILE)
N_TILES = len(TILE)
HP = ((0, 0), (0, 1), (1, 0), (1, 1))
ROOM = {True: ((0, 720, 2.1), (720, 1440, 1.6), (1440, 1728, 2.6), (1728, 1850, 0.5)),
        False: ((0, 792, 2.1), (792, 1584, 1.6), (1584, 1872, 2.6), (1872, 2000, 0.5))}


def _pack(v):
    return pltpu.bitcast(v, U32)


def _unpack(v):
    return pltpu.bitcast(v, BF16)


def _a_ops(a11, a12, a21, a22):
    return [a11 + a22, a21 + a22, a11, a22, a11 + a12, a21 - a11, a12 - a22]


def _b_ops(b11, b12, b21, b22):
    return [b11 + b22, b11, b12 - b22, b21 - b11, b22, b11 + b12, b21 + b22]


def _prep_weights(g_ref, b_ref, w_ref, a1_ref, a2_ref, ar_ref):
    g = g_ref[...].astype(F32).reshape(1, D)
    b16 = jnp.broadcast_to(b_ref[...].reshape(1, D), (16, D))
    c = jnp.dot(b16, w_ref[...], preferred_element_type=F32)
    c_hi = c.astype(BF16).astype(F32)
    rest = c - c_hi
    c_mid = rest.astype(BF16).astype(F32)
    c_lo = rest - c_mid
    row = jax.lax.broadcasted_iota(jnp.int32, (16, D), 0)
    ext = jnp.where(row == 0, c_hi,
                    jnp.where(row == 1, c_mid,
                              jnp.where(row == 2, c_lo, 0.0))).astype(BF16)
    wr = jnp.concatenate(
        [w_ref[2 * KH:, :], ext, jnp.zeros((128 - KX, D), BF16)], axis=0)
    gr = jnp.concatenate([g[:, 2 * KH:], jnp.ones((1, 128 - KR), F32)], axis=1)
    ar_ref[...] = _pack((wr.astype(F32).T * gr).astype(BF16))
    w1 = w_ref[:KH, :].astype(F32).T * g[:, :KH]
    w2 = w_ref[KH:2 * KH, :].astype(F32).T * g[:, KH:2 * KH]
    ops = _a_ops(w1[:H], w2[:H], w1[H:], w2[H:])
    a1_ref[...] = _pack(ops[0].astype(BF16))
    subs = []
    for t in DEEP:
        a = ops[t]
        subs += _a_ops(a[:Q, :128], a[:Q, 128:], a[Q:, :128], a[Q:, 128:])
    for e in range(0, len(subs), 2):
        a2_ref[e // 2] = _pack(
            jnp.concatenate([subs[e], subs[e + 1]], axis=1).astype(BF16))


class _Stats:
    def __init__(self, x_ref, col0):
        self.x, self.cs = x_ref, pl.ds(col0, 256)
        self.items = [(functools.partial(self.stat, r0, 32), 40)
                      for r0 in range(0, D, 32)]
        self.s1 = self.s2 = self.p = self.m = self.r = None

    def stat(self, r0, rows, tie):
        if self.p is None:
            first = self.x[0:16, self.cs].astype(F32)[0:1, :]
            self.p = jnp.broadcast_to(first, (8, 256))
        p = _tie2(tie, self.p)
        xf = self.x[r0:r0 + rows, self.cs].astype(F32).reshape(rows // 8, 8, 256)
        s1 = s2 = None
        for t in range(rows // 8):
            d = xf[t] - p
            s1 = d if s1 is None else s1 + d
            s2 = d * d if s2 is None else s2 + d * d
        self.s1 = s1 if self.s1 is None else self.s1 + s1
        self.s2 = s2 if self.s2 is None else self.s2 + s2
        if r0 + rows == D:
            e1 = jnp.sum(self.s1, axis=0, keepdims=True) * (1.0 / D)
            e2 = jnp.sum(self.s2, axis=0, keepdims=True) * (1.0 / D)
            var = jnp.maximum(e2 - e1 * e1, 0.0)
            self.m = self.p + e1
            self.r = jnp.broadcast_to(jax.lax.rsqrt(var + EPS), (8, 256))


def _tie2(tie, v):
    return jnp.concatenate([tie(v[:, :128]), tie(v[:, 128:])], axis=1)


def _norm_items(x_ref, col0, zb, zr):
    st = [_Stats(x_ref, col0), _Stats(x_ref, col0 + 256)]
    held, pending = {}, {}

    def put(keys, j, vals):
        for key, v in zip(keys, vals):
            e = TILE[key]
            other = pending.pop((e ^ 1, j), None)
            if other is None:
                pending[(e, j)] = v
                continue
            pair = [v, other] if e % 2 == 0 else [other, v]
            zb[e // 2, j:j + 8, :] = jnp.concatenate(pair, axis=1).astype(BF16)

    def deep(t, j, bt):
        put([(t, u) for u in range(7)], j, _b_ops(*[bt[k] for k in HP]))

    def zblock(j, kq, side, tie):
        out = {}
        for p in range(2):
            ls = slice(128 * side, 128 * side + 128)
            m, r = tie(st[p].m[:, ls]), st[p].r[:, ls]
            for h in range(2):
                r0 = 128 * (kq + h) + j
                out[(h, p)] = (x_ref[r0:r0 + 8, st[p].cs].astype(F32)[:, ls] - m) * r
        return out

    def step1(j, tie):
        b11 = held[(j, 11)] = zblock(j, 0, 0, tie)
        deep(1, j, b11)

    def step2(j, tie):
        b11, b22 = held[(j, 11)], zblock(j, 2, 1, tie)
        held[(j, 22)] = b22
        deep(4, j, b22)
        put([(0,) + k for k in HP], j, [b11[k] + b22[k] for k in HP])

    def step3(j, tie):
        b11, b22, b12 = held[(j, 11)], held[(j, 22)], zblock(j, 0, 1, tie)
        deep(2, j, {k: b12[k] - b22[k] for k in HP})
        deep(5, j, {k: b11[k] + b12[k] for k in HP})

    def step4(j, tie):
        b11, b22, b21 = held[(j, 11)], held[(j, 22)], zblock(j, 2, 0, tie)
        deep(3, j, {k: b21[k] - b11[k] for k in HP})
        deep(6, j, {k: b21[k] + b22[k] for k in HP})

    def zrem(p, r0, tie):
        m = _tie2(tie, st[p].m)
        xf = x_ref[2 * KH + r0:2 * KH + r0 + 32, st[p].cs].astype(F32)
        z = (xf.reshape(4, 8, 256) - m[None]) * st[p].r[None]
        zr[r0:r0 + 32, pl.ds(256 * p, 256)] = z.reshape(32, 256).astype(BF16)

    items = st[0].items + st[1].items
    items += [(functools.partial(zrem, 0, r0), 28) for r0 in range(0, KR, 32)]
    for j in range(0, 128, 8):
        items += [(functools.partial(step1, j), 20.5), (functools.partial(step2, j), 26.5),
                  (functools.partial(step3, j), 37), (functools.partial(step4, j), 37)]
    items += [(functools.partial(zrem, 1, r0), 28) for r0 in range(0, KR, 32)]
    return items


def _time_slots(items, segs):
    room = sum((b - a) * d for a, b, d in segs)
    total = sum(cost for _, cost in items)
    pos, cum = [], 0
    for _, cost in items:
        c = room * cum / total
        for a, b, d in segs:
            if c <= (b - a) * d + 1e-9:
                pos.append(a + c / d)
                break
            c -= (b - a) * d
        cum += cost
    return pos


def _mm_group(a1_ref, a2_ref, ar_ref, e_ref, s_ref, t_ref, first, zb, zr, o_ref,
              col0, items, never, after_rows=None):
    pos = _time_slots(items, ROOM[first])
    state = [0, 0]

    def release(mt):
        lo, span = state[1], mt.shape[0]
        while state[0] < len(items) and pos[state[0]] < lo + span:
            rr = min(span - 8, int(pos[state[0]] - lo) // 8 * 8)
            src = mt[rr:rr + 8, :128]
            items[state[0]][0](lambda v, src=src: jnp.where(never, src, v))
            state[0] += 1
        state[1] += span

    def tile(key):
        e = TILE[key]
        return zb[e // 2, :, pl.ds(128 * (e % 2), 128)]

    def prod(t, u):
        e = A_IDX[(t, u)]
        a = _unpack(a2_ref[e // 2, :, pl.ds(128 * (e % 2), 128)])
        return jnp.dot(a, tile((t, u)), preferred_element_type=F32)

    def round_2345(u, with_67):
        p = {t: prod(t, u) for t in (1, 2, 3, 4)}
        e11, e22 = p[3] - p[4], p[2] - p[1]
        if with_67:
            e11, e22 = e11 + s_ref[0], e22 + s_ref[1]
        e_ref[0, u] = e11
        e_ref[1, u] = p[2] + p[4]
        e_ref[2, u] = p[1] + p[3]
        e_ref[3, u] = e22
        release(p[1])

    def add_67(u):
        p7, p6 = prod(6, u), prod(5, u)
        e_ref[0, u] = p7 + e_ref[0, u]
        e_ref[3, u] = p6 + e_ref[3, u]
        return p7

    def hold_67(u):
        p7, p6 = prod(6, u), prod(5, u)
        s_ref[0] = p7
        s_ref[1] = p6
        return p7

    def three_rounds(u):
        round_2345(u, False)
        p7 = add_67(u)
        hold_67(u + 1)
        release(p7)
        round_2345(u + 1, True)

    if first:
        for u in (0, 2, 4):
            three_rounds(u)
        round_2345(6, False)
        add_67(6)
    else:
        release(hold_67(0))
        round_2345(0, True)
        for u in (1, 3, 5):
            three_rounds(u)

    bt = jnp.concatenate(
        [jnp.concatenate([tile((0, h, p)) for p in range(2)], axis=1)
         for h in range(2)], axis=0)
    m1 = jnp.dot(_unpack(a1_ref[...]), bt, preferred_element_type=F32)
    t_ref[...] = m1
    release(m1)
    rem = jnp.dot(_unpack(ar_ref[...])[:, :KX], zr[...], preferred_element_type=F32)
    release(rem)

    def quadrant(f, q, p, base):
        if (q, p) == (0, 0):
            return base + e_ref[f, 0] + e_ref[f, 3] - e_ref[f, 4] + e_ref[f, 6]
        if (q, p) == (0, 1):
            return base + e_ref[f, 2] + e_ref[f, 4]
        if (q, p) == (1, 0):
            return base + e_ref[f, 1] + e_ref[f, 3]
        return base + e_ref[f, 0] - e_ref[f, 1] + e_ref[f, 2] + e_ref[f, 5]

    for half in range(2):
        for q in range(2):
            r0 = half * H + q * Q
            for p in range(2):
                left = rem[r0:r0 + Q, 256 * p:256 * p + 128]
                right = rem[r0:r0 + Q, 256 * p + 128:256 * p + 256]
                m1_part = t_ref[pl.ds(q * Q, Q), pl.ds(128 * p, 128)]
                if half == 0:
                    left = quadrant(0, q, p, left + m1_part)
                    right = quadrant(1, q, p, right)
                else:
                    left = quadrant(2, q, p, left)
                    right = quadrant(3, q, p, right + m1_part)
                o_ref[pl.ds(r0, Q), pl.ds(col0 + 256 * p, 256)] = jnp.concatenate(
                    [left, right], axis=1).astype(BF16)
            if after_rows is not None:
                after_rows(r0)


def _kernel(x_hbm, g_hbm, b_hbm, w_hbm, o_hbm,
            xbuf, obuf, gbuf, bbuf, wbuf, a1_ref, a2_ref, ar_ref, e_ref, s_ref, t_ref,
            zb0, zr0, zb1, zr1, sem_x0, sem_w, sem_x, sem_o):
    S = xbuf.shape[0]
    n_ramp = sum(RAMP)
    n_body = (S - 1 - n_ramp) // SPB

    def x0_copy(h):
        cols = pl.ds(GW * h, GW)
        return pltpu.make_async_copy(x_hbm.at[0, :, cols], xbuf.at[0, :, cols],
                                     sem_x0.at[h])

    def x_copy(s):
        return pltpu.make_async_copy(x_hbm.at[s], xbuf.at[s], sem_x.at[s])

    def o_part_start(s, h, r0, rows):
        sl = (s, pl.ds(r0, rows), pl.ds(GW * h, GW))
        pltpu.make_async_copy(obuf.at[sl], o_hbm.at[sl], sem_o).start()

    def o_start(s0, n):
        for c in range(2 * GW // 128):
            sl = (pl.ds(s0, n), slice(None), pl.ds(c * 128, 128))
            pltpu.make_async_copy(obuf.at[sl], o_hbm.at[sl], sem_o).start(priority=c % 2)

    w_copies = [pltpu.make_async_copy(g_hbm, gbuf, sem_w.at[0]),
                pltpu.make_async_copy(b_hbm, bbuf, sem_w.at[1]),
                pltpu.make_async_copy(w_hbm, wbuf, sem_w.at[2])]

    head = [x0_copy(0)] + w_copies + [x0_copy(1)]

    def issue_head(k, carry):
        for kk, cp in enumerate(head):
            pl.when(k == kk)(cp.start)
        return carry

    jax.lax.fori_loop(0, len(head), issue_head, 0)

    def issue_x(s, carry):
        x_copy(s).start()
        return carry

    jax.lax.fori_loop(1, S, issue_x, 0)

    row = jax.lax.broadcasted_iota(jnp.int32, (16, GW), 0)
    ones = jnp.where(row < 3, 1.0, 0.0).astype(BF16)
    zr0[KR:, :] = ones
    zr1[KR:, :] = ones

    x0_copy(0).wait()
    for item, _ in _norm_items(xbuf.at[0], 0, zb0, zr0):
        item(lambda v: v)
    for c in w_copies:
        c.wait()
    _prep_weights(gbuf, bbuf, wbuf, a1_ref, a2_ref, ar_ref)
    x0_copy(1).wait()
    gv = jnp.broadcast_to(gbuf[...].astype(F32).reshape(1, D)[:, :128], (8, 128))
    never = gv != gv
    mm_a = functools.partial(_mm_group, a1_ref, a2_ref, ar_ref, e_ref.at[0],
                             s_ref.at[0], t_ref.at[0], True)
    mm_b = functools.partial(_mm_group, a1_ref, a2_ref, ar_ref, e_ref.at[1],
                             s_ref.at[1], t_ref.at[1], False)

    def block(i0, n, write):
        for u in range(n):
            i = i0 + u
            last = write and u == n - 1
            mm_a(zb0, zr0, obuf.at[i], 0,
                 _norm_items(xbuf.at[i], GW, zb1, zr1), never)
            after_rows = None
            if last:
                pl.when(i == S - 1)(functools.partial(o_part_start, i, 0, 0, D))

                def after_rows(r0, i=i):
                    pl.when(i == S - 1)(functools.partial(o_part_start, i, 1, r0, Q))
            nxt = jnp.minimum(i + 1, S - 1)
            mm_b(zb1, zr1, obuf.at[i], GW,
                 _norm_items(xbuf.at[nxt], 0, zb0, zr0), never, after_rows)
            if write:
                if (W_START - 2 - n_ramp) % SPB == u:
                    pl.when(i == W_START - 1)(functools.partial(o_start, 0, W_START))
                pl.when(jnp.logical_and(i >= W_START, i < S - 1))(
                    functools.partial(o_start, i, 1))

    mm_a(zb0, zr0, obuf.at[0], 0, _norm_items(xbuf.at[0], GW, zb1, zr1), never)
    x_copy(1).wait()
    mm_a(zb1, zr1, obuf.at[0], GW, _norm_items(xbuf.at[1], 0, zb0, zr0), never)
    i = 1
    for n in RAMP:
        for u in range(n):
            x_copy(i + u + 1).wait()
        block(i, n, False)
        i += n

    def body(j, carry):
        i0 = 1 + n_ramp + j * SPB
        for u in range(SPB - 1):
            x_copy(i0 + u + 1).wait()
        pl.when(j < n_body - 1)(x_copy(jnp.minimum(i0 + SPB, S - 1)).wait)
        block(i0, SPB, True)
        return carry

    jax.lax.fori_loop(0, n_body, body, 0)
    pltpu.make_async_copy(obuf, o_hbm, sem_o).wait()


@jax.jit
def pallas_standalone__layernorm_linear__sampling_kernel(
    x: jax.Array,
    g: jax.Array,
    b: jax.Array,
    w: jax.Array,
):
    B, S, d = x.shape
    assert d == D and B == 2 * GW and (S - 1 - sum(RAMP)) % SPB == 0
    assert 1 + sum(RAMP) < W_START < S
    xt = jnp.transpose(x, (1, 2, 0))
    out = pl.pallas_call(
        _kernel,
        in_specs=[pl.BlockSpec(memory_space=pl.ANY)] * 4,
        out_specs=pl.BlockSpec(memory_space=pl.ANY),
        out_shape=jax.ShapeDtypeStruct((S, D, B), x.dtype),
        scratch_shapes=[
            pltpu.VMEM((S, D, B), BF16),
            pltpu.VMEM((S, D, B), BF16),
            pltpu.VMEM((D,), BF16),
            pltpu.VMEM((D,), BF16),
            pltpu.VMEM((D, D), BF16),
            pltpu.VMEM((H // 2, KH), U32),
            pltpu.VMEM((21, Q // 2, 256), U32),
            pltpu.VMEM((D // 2, 128), U32),
            pltpu.VMEM((2, 4, 7, Q, 128), F32),
            pltpu.VMEM((2, 2, Q, 128), F32),
            pltpu.VMEM((2, H, 256), F32),
            pltpu.VMEM((N_TILES // 2, 128, 256), BF16),
            pltpu.VMEM((KX, GW), BF16),
            pltpu.VMEM((N_TILES // 2, 128, 256), BF16),
            pltpu.VMEM((KX, GW), BF16),
            pltpu.SemaphoreType.DMA((2,)),
            pltpu.SemaphoreType.DMA((3,)),
            pltpu.SemaphoreType.DMA((S,)),
            pltpu.SemaphoreType.DMA(()),
        ],
        compiler_params=pltpu.CompilerParams(
            vmem_limit_bytes=110 * 1024 * 1024,
            disable_bounds_checks=True,
            disable_semaphore_checks=True,
        ),
    )(xt, g, b, w)
    return jnp.transpose(out, (2, 0, 1))
```

```python
import functools

import jax
import jax.numpy as jnp
import jax.experimental.pallas as pl
import jax.experimental.pallas.tpu as pltpu

F32 = jnp.float32
BF16 = jnp.bfloat16
U32 = jnp.uint32

EPS = 1e-5
D = 576
H = D // 2
Q = H // 2
KH = 256
KR = D - 2 * KH
KX = KR + 16
GW = 512
RAMP = (1, 2)
SPB = 4
W_START = 14

DEEP = (1, 2, 3, 4, 5, 6)
A_IDX = {(t, u): 7 * i + u for i, t in enumerate(DEEP) for u in range(7)}
TILE = {}
for _t in (1, 4, 2, 5, 3, 6):
    for _u in range(7):
        TILE[(_t, _u)] = len(TILE)
for _h in range(2):
    for _p in range(2):
        TILE[(0, _h, _p)] = len(TILE)
N_TILES = len(TILE)
HP = ((0, 0), (0, 1), (1, 0), (1, 1))
ROUNDS = {True: "qsq" * 3 + "q", False: "sq" + "qsq" * 3}
TAIL = {True: (1750, 2290), False: (1890, 2430)}


def _pack(v):
    return pltpu.bitcast(v, U32)


def _unpack(v):
    return pltpu.bitcast(v, BF16)


def _a_ops(a11, a12, a21, a22):
    return [a11 + a22, a21 + a22, a11, a22, a11 + a12, a21 - a11, a12 - a22]


def _b_ops(b11, b12, b21, b22):
    return [b11 + b22, b11, b12 - b22, b21 - b11, b22, b11 + b12, b21 + b22]


def _prep_weights(g_ref, b_ref, w_ref, a1_ref, a2_ref, ar_ref):
    g = g_ref[...].astype(F32).reshape(1, D)
    b16 = jnp.broadcast_to(b_ref[...].reshape(1, D), (16, D))
    c = jnp.dot(b16, w_ref[...], preferred_element_type=F32)
    c_hi = c.astype(BF16).astype(F32)
    rest = c - c_hi
    c_mid = rest.astype(BF16).astype(F32)
    c_lo = rest - c_mid
    row = jax.lax.broadcasted_iota(jnp.int32, (16, D), 0)
    ext = jnp.where(row == 0, c_hi,
                    jnp.where(row == 1, c_mid,
                              jnp.where(row == 2, c_lo, 0.0))).astype(BF16)
    wr = jnp.concatenate(
        [w_ref[2 * KH:, :], ext, jnp.zeros((128 - KX, D), BF16)], axis=0)
    gr = jnp.concatenate([g[:, 2 * KH:], jnp.ones((1, 128 - KR), F32)], axis=1)
    ar_ref[...] = _pack((wr.astype(F32).T * gr).astype(BF16))
    w1 = w_ref[:KH, :].astype(F32).T * g[:, :KH]
    w2 = w_ref[KH:2 * KH, :].astype(F32).T * g[:, KH:2 * KH]
    ops = _a_ops(w1[:H], w2[:H], w1[H:], w2[H:])
    a1_ref[...] = _pack(ops[0].astype(BF16))
    subs = []
    for t in DEEP:
        a = ops[t]
        subs += _a_ops(a[:Q, :128], a[:Q, 128:], a[Q:, :128], a[Q:, 128:])
    for e in range(0, len(subs), 2):
        a2_ref[e // 2] = _pack(
            jnp.concatenate([subs[e], subs[e + 1]], axis=1).astype(BF16))


class _Stats:
    def __init__(self, x_ref, col0, save=None, load=None):
        self.x, self.cs, self.save = x_ref, pl.ds(col0, 256), save
        self.s1 = self.s2 = self.p = self.m = self.r = None
        self.items = []
        if load is not None:
            self.m, self.r = load[0], load[1]
        else:
            self.items = [(functools.partial(self.stat, r0, 32), 40)
                          for r0 in range(0, D, 32)]

    def stat(self, r0, rows, tie):
        if self.p is None:
            first = self.x[0:16, self.cs].astype(F32)[0:1, :]
            self.p = jnp.broadcast_to(first, (8, 256))
        p = _tie2(tie, self.p)
        xf = self.x[r0:r0 + rows, self.cs].astype(F32).reshape(rows // 8, 8, 256)
        s1 = s2 = None
        for t in range(rows // 8):
            d = xf[t] - p
            s1 = d if s1 is None else s1 + d
            s2 = d * d if s2 is None else s2 + d * d
        self.s1 = s1 if self.s1 is None else self.s1 + s1
        self.s2 = s2 if self.s2 is None else self.s2 + s2
        if r0 + rows == D:
            e1 = jnp.sum(self.s1, axis=0, keepdims=True) * (1.0 / D)
            e2 = jnp.sum(self.s2, axis=0, keepdims=True) * (1.0 / D)
            var = jnp.maximum(e2 - e1 * e1, 0.0)
            self.m = self.p + e1
            self.r = jnp.broadcast_to(jax.lax.rsqrt(var + EPS), (8, 256))
            if self.save is not None:
                self.save[0] = self.m
                self.save[1] = self.r


def _tie2(tie, v):
    return jnp.concatenate([tie(v[:, :128]), tie(v[:, 128:])], axis=1)


def _norm_items(x_ref, col0, zb, zr, stats0=None):
    st = [_Stats(x_ref, col0, load=stats0), _Stats(x_ref, col0 + 256)]
    held, pending = {}, {}

    def put(keys, j, vals):
        for key, v in zip(keys, vals):
            e = TILE[key]
            other = pending.pop((e ^ 1, j), None)
            if other is None:
                pending[(e, j)] = v
                continue
            pair = [v, other] if e % 2 == 0 else [other, v]
            zb[e // 2, j:j + 8, :] = jnp.concatenate(pair, axis=1).astype(BF16)

    def deep(t, j, bt):
        put([(t, u) for u in range(7)], j, _b_ops(*[bt[k] for k in HP]))

    def zblock(j, kq, side, tie):
        out = {}
        for p in range(2):
            ls = slice(128 * side, 128 * side + 128)
            m, r = tie(st[p].m[:, ls]), st[p].r[:, ls]
            for h in range(2):
                r0 = 128 * (kq + h) + j
                out[(h, p)] = (x_ref[r0:r0 + 8, st[p].cs].astype(F32)[:, ls] - m) * r
        return out

    def step1(j, tie):
        b11 = held[(j, 11)] = zblock(j, 0, 0, tie)
        deep(1, j, b11)

    def step2(j, tie):
        b11, b22 = held[(j, 11)], zblock(j, 2, 1, tie)
        held[(j, 22)] = b22
        deep(4, j, b22)
        put([(0,) + k for k in HP], j, [b11[k] + b22[k] for k in HP])

    def step3(j, tie):
        b11, b22, b12 = held[(j, 11)], held[(j, 22)], zblock(j, 0, 1, tie)
        deep(2, j, {k: b12[k] - b22[k] for k in HP})
        deep(5, j, {k: b11[k] + b12[k] for k in HP})

    def step4(j, tie):
        b11, b22, b21 = held[(j, 11)], held[(j, 22)], zblock(j, 2, 0, tie)
        deep(3, j, {k: b21[k] - b11[k] for k in HP})
        deep(6, j, {k: b21[k] + b22[k] for k in HP})

    def zrem(p, r0, tie):
        m = _tie2(tie, st[p].m)
        xf = x_ref[2 * KH + r0:2 * KH + r0 + 32, st[p].cs].astype(F32)
        z = (xf.reshape(4, 8, 256) - m[None]) * st[p].r[None]
        zr[r0:r0 + 32, pl.ds(256 * p, 256)] = z.reshape(32, 256).astype(BF16)

    items = st[0].items + st[1].items
    items += [(functools.partial(zrem, 0, r0), 28) for r0 in range(0, KR, 32)]
    for j in range(0, 128, 8):
        items += [(functools.partial(step1, j), 20.5), (functools.partial(step2, j), 26.5),
                  (functools.partial(step3, j), 37), (functools.partial(step4, j), 37)]
    items += [(functools.partial(zrem, 1, r0), 28) for r0 in range(0, KR, 32)]
    return items


def _time_slots(items, first):
    room = []
    for kind in ROUNDS[first]:
        for _ in range(Q // 8):
            t = 8 * len(room)
            r = 2.1 if t < (400 if first else 472) else 1.6
            room.append(0.0 if t < 32 else r * (1.2 if kind == "s" else 1.0))
    room += [2.6] * (H // 8)
    scale = sum(room) / sum(cost for _, cost in items)
    pos, cum, acc, k = [], 0, 0.0, 0
    for _, cost in items:
        while acc + room[k] <= scale * cum + 1e-9:
            acc += room[k]
            k += 1
        pos.append(8 * k)
        cum += cost
    return pos


def _mm_group(a1_ref, a2_ref, ar_ref, e_ref, s_ref, t_ref, first, zb, zr, o_ref,
              col0, items, tail, never, after_rows=None):
    t0, t1 = TAIL[first]
    pos = _time_slots(items, first)
    pos += [t0 + (t1 - t0) * k / len(tail) for k in range(len(tail))]
    items = items + tail
    state = [0, 0]

    def release(mt):
        lo, span = state[1], mt.shape[0]
        while state[0] < len(items) and pos[state[0]] < lo + span:
            rr = min(span - 8, int(pos[state[0]] - lo) // 8 * 8)
            src = mt[rr:rr + 8, :128]
            items[state[0]][0](lambda v, src=src: jnp.where(never, src, v))
            state[0] += 1
        state[1] += span

    def tile(key):
        e = TILE[key]
        return zb[e // 2, :, pl.ds(128 * (e % 2), 128)]

    def prod(t, u):
        e = A_IDX[(t, u)]
        a = _unpack(a2_ref[e // 2, :, pl.ds(128 * (e % 2), 128)])
        return jnp.dot(a, tile((t, u)), preferred_element_type=F32)

    def round_2345(u, with_67):
        p = {t: prod(t, u) for t in (1, 2, 3, 4)}
        e11, e22 = p[3] - p[4], p[2] - p[1]
        if with_67:
            e11, e22 = e11 + s_ref[0], e22 + s_ref[1]
        e_ref[0, u] = e11
        e_ref[1, u] = p[2] + p[4]
        e_ref[2, u] = p[1] + p[3]
        e_ref[3, u] = e22
        release(p[1])

    def add_67(u):
        p7, p6 = prod(6, u), prod(5, u)
        e_ref[0, u] = p7 + e_ref[0, u]
        e_ref[3, u] = p6 + e_ref[3, u]
        return p7

    def hold_67(u):
        p7, p6 = prod(6, u), prod(5, u)
        s_ref[0] = p7
        s_ref[1] = p6
        return p7

    def three_rounds(u):
        round_2345(u, False)
        p7 = add_67(u)
        hold_67(u + 1)
        release(p7)
        round_2345(u + 1, True)

    if first:
        for u in (0, 2, 4):
            three_rounds(u)
        round_2345(6, False)
        add_67(6)
    else:
        release(hold_67(0))
        round_2345(0, True)
        for u in (1, 3, 5):
            three_rounds(u)

    bt = jnp.concatenate(
        [jnp.concatenate([tile((0, h, p)) for p in range(2)], axis=1)
         for h in range(2)], axis=0)
    m1 = jnp.dot(_unpack(a1_ref[...]), bt, preferred_element_type=F32)
    t_ref[...] = m1
    release(m1)
    rem = jnp.dot(_unpack(ar_ref[...])[:, :KX], zr[...], preferred_element_type=F32)
    release(rem)

    def quadrant(f, q, p, base):
        if (q, p) == (0, 0):
            return base + e_ref[f, 0] + e_ref[f, 3] - e_ref[f, 4] + e_ref[f, 6]
        if (q, p) == (0, 1):
            return base + e_ref[f, 2] + e_ref[f, 4]
        if (q, p) == (1, 0):
            return base + e_ref[f, 1] + e_ref[f, 3]
        return base + e_ref[f, 0] - e_ref[f, 1] + e_ref[f, 2] + e_ref[f, 5]

    for half in range(2):
        for q in range(2):
            r0 = half * H + q * Q
            for p in range(2):
                left = rem[r0:r0 + Q, 256 * p:256 * p + 128]
                right = rem[r0:r0 + Q, 256 * p + 128:256 * p + 256]
                m1_part = t_ref[pl.ds(q * Q, Q), pl.ds(128 * p, 128)]
                if half == 0:
                    left = quadrant(0, q, p, left + m1_part)
                    right = quadrant(1, q, p, right)
                else:
                    left = quadrant(2, q, p, left)
                    right = quadrant(3, q, p, right + m1_part)
                o_ref[pl.ds(r0, Q), pl.ds(col0 + 256 * p, 256)] = jnp.concatenate(
                    [left, right], axis=1).astype(BF16)
            if after_rows is not None:
                after_rows(r0)


def _kernel(x_hbm, g_hbm, b_hbm, w_hbm, o_hbm,
            xbuf, obuf, gbuf, bbuf, wbuf, a1_ref, a2_ref, ar_ref, e_ref, s_ref, t_ref,
            zb0, zr0, zb1, zr1, c_ref, sem_x0, sem_w, sem_x, sem_o):
    S = xbuf.shape[0]
    n_ramp = sum(RAMP)
    n_body = (S - 1 - n_ramp) // SPB

    def x0_copy(h):
        cols = pl.ds(GW * h, GW)
        return pltpu.make_async_copy(x_hbm.at[0, :, cols], xbuf.at[0, :, cols],
                                     sem_x0.at[h])

    def x_copy(s):
        return pltpu.make_async_copy(x_hbm.at[s], xbuf.at[s], sem_x.at[s])

    def o_part_start(s, h, r0, rows):
        sl = (s, pl.ds(r0, rows), pl.ds(GW * h, GW))
        pltpu.make_async_copy(obuf.at[sl], o_hbm.at[sl], sem_o).start()

    def o_start(s0, n):
        for c in range(2 * GW // 128):
            sl = (pl.ds(s0, n), slice(None), pl.ds(c * 128, 128))
            pltpu.make_async_copy(obuf.at[sl], o_hbm.at[sl], sem_o).start(priority=c % 2)

    w_copies = [pltpu.make_async_copy(g_hbm, gbuf, sem_w.at[0]),
                pltpu.make_async_copy(b_hbm, bbuf, sem_w.at[1]),
                pltpu.make_async_copy(w_hbm, wbuf, sem_w.at[2])]

    head = [x0_copy(0)] + w_copies + [x0_copy(1)]

    def issue_head(k, carry):
        for kk, cp in enumerate(head):
            pl.when(k == kk)(cp.start)
        return carry

    jax.lax.fori_loop(0, len(head), issue_head, 0)

    def issue_x(s, carry):
        x_copy(s).start()
        return carry

    jax.lax.fori_loop(1, S, issue_x, 0)

    row = jax.lax.broadcasted_iota(jnp.int32, (16, GW), 0)
    ones = jnp.where(row < 3, 1.0, 0.0).astype(BF16)
    zr0[KR:, :] = ones
    zr1[KR:, :] = ones

    x0_copy(0).wait()
    for item, _ in _norm_items(xbuf.at[0], 0, zb0, zr0):
        item(lambda v: v)
    for c in w_copies:
        c.wait()
    _prep_weights(gbuf, bbuf, wbuf, a1_ref, a2_ref, ar_ref)
    x0_copy(1).wait()
    gv = jnp.broadcast_to(gbuf[...].astype(F32).reshape(1, D)[:, :128], (8, 128))
    never = gv != gv
    mm_a = functools.partial(_mm_group, a1_ref, a2_ref, ar_ref, e_ref.at[0],
                             s_ref.at[0], t_ref.at[0], True)
    mm_b = functools.partial(_mm_group, a1_ref, a2_ref, ar_ref, e_ref.at[1],
                             s_ref.at[1], t_ref.at[1], False)

    def ahead(i, h):
        return _Stats(xbuf.at[i], GW * h, save=c_ref.at[h]).items

    def block(i0, n, write):
        for u in range(n):
            i = i0 + u
            nxt = jnp.minimum(i + 1, S - 1)
            mm_a(zb0, zr0, obuf.at[i], 0,
                 _norm_items(xbuf.at[i], GW, zb1, zr1, c_ref.at[1]), ahead(nxt, 0), never)
            after_rows = None
            if write and u == n - 1:
                pl.when(i == S - 1)(functools.partial(o_part_start, i, 0, 0, D))

                def after_rows(r0, i=i):
                    pl.when(i == S - 1)(functools.partial(o_part_start, i, 1, r0, Q))
            mm_b(zb1, zr1, obuf.at[i], GW,
                 _norm_items(xbuf.at[nxt], 0, zb0, zr0, c_ref.at[0]), ahead(nxt, 1),
                 never, after_rows)
            if write:
                if (W_START - 2 - n_ramp) % SPB == u:
                    pl.when(i == W_START - 1)(functools.partial(o_start, 0, W_START))
                pl.when(jnp.logical_and(i >= W_START, i < S - 1))(
                    functools.partial(o_start, i, 1))

    mm_a(zb0, zr0, obuf.at[0], 0, _norm_items(xbuf.at[0], GW, zb1, zr1), [], never)
    x_copy(1).wait()
    mm_a(zb1, zr1, obuf.at[0], GW, _norm_items(xbuf.at[1], 0, zb0, zr0), ahead(1, 1),
         never)
    i = 1
    for n in RAMP:
        for u in range(n):
            x_copy(i + u + 1).wait()
        block(i, n, False)
        i += n

    def body(j, carry):
        i0 = 1 + n_ramp + j * SPB
        for u in range(SPB - 1):
            x_copy(i0 + u + 1).wait()
        pl.when(j < n_body - 1)(x_copy(jnp.minimum(i0 + SPB, S - 1)).wait)
        block(i0, SPB, True)
        return carry

    jax.lax.fori_loop(0, n_body, body, 0)
    pltpu.make_async_copy(obuf, o_hbm, sem_o).wait()


@jax.jit
def pallas_standalone__layernorm_linear__sampling_kernel(
    x: jax.Array,
    g: jax.Array,
    b: jax.Array,
    w: jax.Array,
):
    B, S, d = x.shape
    assert d == D and B == 2 * GW and (S - 1 - sum(RAMP)) % SPB == 0
    assert 1 + sum(RAMP) < W_START < S
    xt = jnp.transpose(x, (1, 2, 0))
    out = pl.pallas_call(
        _kernel,
        in_specs=[pl.BlockSpec(memory_space=pl.ANY)] * 4,
        out_specs=pl.BlockSpec(memory_space=pl.ANY),
        out_shape=jax.ShapeDtypeStruct((S, D, B), x.dtype),
        scratch_shapes=[
            pltpu.VMEM((S, D, B), BF16),
            pltpu.VMEM((S, D, B), BF16),
            pltpu.VMEM((D,), BF16),
            pltpu.VMEM((D,), BF16),
            pltpu.VMEM((D, D), BF16),
            pltpu.VMEM((H // 2, KH), U32),
            pltpu.VMEM((21, Q // 2, 256), U32),
            pltpu.VMEM((D // 2, 128), U32),
            pltpu.VMEM((2, 4, 7, Q, 128), F32),
            pltpu.VMEM((2, 2, Q, 128), F32),
            pltpu.VMEM((2, H, 256), F32),
            pltpu.VMEM((N_TILES // 2, 128, 256), BF16),
            pltpu.VMEM((KX, GW), BF16),
            pltpu.VMEM((N_TILES // 2, 128, 256), BF16),
            pltpu.VMEM((KX, GW), BF16),
            pltpu.VMEM((2, 2, 8, 256), F32),
            pltpu.SemaphoreType.DMA((2,)),
            pltpu.SemaphoreType.DMA((3,)),
            pltpu.SemaphoreType.DMA((S,)),
            pltpu.SemaphoreType.DMA(()),
        ],
        compiler_params=pltpu.CompilerParams(
            vmem_limit_bytes=110 * 1024 * 1024,
            disable_bounds_checks=True,
            disable_semaphore_checks=True,
        ),
    )(xt, g, b, w)
    return jnp.transpose(out, (2, 0, 1))
```

```python
import functools

import jax
import jax.numpy as jnp
import jax.experimental.pallas as pl
import jax.experimental.pallas.tpu as pltpu

F32 = jnp.float32
BF16 = jnp.bfloat16
U32 = jnp.uint32

EPS = 1e-5
D = 576
H = D // 2
Q = H // 2
KH = 256
KR = D - 2 * KH
KX = KR + 16
GW = 512
RAMP = (1, 2)
SPB = 4
W_START = 14

DEEP = (1, 2, 3, 4, 5, 6)
A_IDX = {(t, u): 7 * i + u for i, t in enumerate(DEEP) for u in range(7)}
TILE = {}
for _t in (1, 4, 2, 5, 3, 6):
    for _u in range(7):
        TILE[(_t, _u)] = len(TILE)
for _h in range(2):
    for _p in range(2):
        TILE[(0, _h, _p)] = len(TILE)
N_TILES = len(TILE)
HP = ((0, 0), (0, 1), (1, 0), (1, 1))
ROUNDS = {True: "qsq" * 3 + "q", False: "sq" + "qsq" * 3}
TAIL = {True: (1750, 2290), False: (1890, 2430)}


def _pack(v):
    return pltpu.bitcast(v, U32)


def _unpack(v):
    return pltpu.bitcast(v, BF16)


def _a_ops(a11, a12, a21, a22):
    return [a11 + a22, a21 + a22, a11, a22, a11 + a12, a21 - a11, a12 - a22]


def _b_ops(b11, b12, b21, b22):
    return [b11 + b22, b11, b12 - b22, b21 - b11, b22, b11 + b12, b21 + b22]


def _prep_weights(g_ref, b_ref, w_ref, a1_ref, a2_ref, ar_ref):
    g = g_ref[...].astype(F32).reshape(1, D)
    b16 = jnp.broadcast_to(b_ref[...].reshape(1, D), (16, D))
    c = jnp.dot(b16, w_ref[...], preferred_element_type=F32)
    c_hi = c.astype(BF16).astype(F32)
    rest = c - c_hi
    c_mid = rest.astype(BF16).astype(F32)
    c_lo = rest - c_mid
    row = jax.lax.broadcasted_iota(jnp.int32, (16, D), 0)
    ext = jnp.where(row == 0, c_hi,
                    jnp.where(row == 1, c_mid,
                              jnp.where(row == 2, c_lo, 0.0))).astype(BF16)
    wr = jnp.concatenate(
        [w_ref[2 * KH:, :], ext, jnp.zeros((128 - KX, D), BF16)], axis=0)
    gr = jnp.concatenate([g[:, 2 * KH:], jnp.ones((1, 128 - KR), F32)], axis=1)
    ar_ref[...] = _pack((wr.astype(F32).T * gr).astype(BF16))
    w1 = w_ref[:KH, :].astype(F32).T * g[:, :KH]
    w2 = w_ref[KH:2 * KH, :].astype(F32).T * g[:, KH:2 * KH]
    ops = _a_ops(w1[:H], w2[:H], w1[H:], w2[H:])
    a1_ref[...] = _pack(ops[0].astype(BF16))
    subs = []
    for t in DEEP:
        a = ops[t]
        subs += _a_ops(a[:Q, :128], a[:Q, 128:], a[Q:, :128], a[Q:, 128:])
    for e in range(0, len(subs), 2):
        a2_ref[e // 2] = _pack(
            jnp.concatenate([subs[e], subs[e + 1]], axis=1).astype(BF16))


class _Stats:
    def __init__(self, x_ref, col0, save=None, load=None):
        self.x, self.cs, self.save = x_ref, pl.ds(col0, 256), save
        self.s1 = self.s2 = self.p = self.m = self.r = None
        self.items = []
        if load is not None:
            self.m, self.r = load[0], load[1]
        else:
            self.items = [(functools.partial(self.stat, r0, 32), 40)
                          for r0 in range(0, D, 32)]

    def stat(self, r0, rows, tie):
        if self.p is None:
            first = self.x[0:16, self.cs].astype(F32)[0:1, :]
            self.p = jnp.broadcast_to(first, (8, 256))
        p = tie(self.p)
        s1 = s2 = None
        for r in range(r0, r0 + rows, 8):
            d = self.x[r:r + 8, self.cs].astype(F32) - p
            s1 = d if s1 is None else s1 + d
            s2 = d * d if s2 is None else s2 + d * d
        self.s1 = s1 if self.s1 is None else self.s1 + s1
        self.s2 = s2 if self.s2 is None else self.s2 + s2
        if r0 + rows == D:
            e1 = jnp.sum(self.s1, axis=0, keepdims=True) * (1.0 / D)
            e2 = jnp.sum(self.s2, axis=0, keepdims=True) * (1.0 / D)
            var = jnp.maximum(e2 - e1 * e1, 0.0)
            self.m = self.p + e1
            self.r = jnp.broadcast_to(jax.lax.rsqrt(var + EPS), (8, 256))
            if self.save is not None:
                self.save[0] = self.m
                self.save[1] = self.r


def _tie(never, src, v):
    if v.shape[1] == 256:
        src = jnp.concatenate([src, src], axis=1)
    return jax.lax.select(never[:, :v.shape[1]], src, v)


def _norm_items(x_ref, col0, zb, zr, stats0=None):
    st = [_Stats(x_ref, col0, load=stats0), _Stats(x_ref, col0 + 256)]
    held, pending = {}, {}

    def put(keys, j, vals):
        for key, v in zip(keys, vals):
            e = TILE[key]
            other = pending.pop((e ^ 1, j), None)
            if other is None:
                pending[(e, j)] = v
                continue
            pair = [v, other] if e % 2 == 0 else [other, v]
            zb[e // 2, j:j + 8, :] = jnp.concatenate(pair, axis=1).astype(BF16)

    def deep(t, j, bt):
        put([(t, u) for u in range(7)], j, _b_ops(*[bt[k] for k in HP]))

    def zblock(j, kq, side, tie):
        out = {}
        for p in range(2):
            ls = slice(128 * side, 128 * side + 128)
            m, r = tie(st[p].m[:, ls]), st[p].r[:, ls]
            for h in range(2):
                r0 = 128 * (kq + h) + j
                out[(h, p)] = (x_ref[r0:r0 + 8, st[p].cs].astype(F32)[:, ls] - m) * r
        return out

    def step1(j, tie):
        b11 = held[(j, 11)] = zblock(j, 0, 0, tie)
        deep(1, j, b11)

    def step2(j, tie):
        b11, b22 = held[(j, 11)], zblock(j, 2, 1, tie)
        held[(j, 22)] = b22
        deep(4, j, b22)
        put([(0,) + k for k in HP], j, [b11[k] + b22[k] for k in HP])

    def step3(j, tie):
        b11, b22, b12 = held[(j, 11)], held[(j, 22)], zblock(j, 0, 1, tie)
        deep(2, j, {k: b12[k] - b22[k] for k in HP})
        deep(5, j, {k: b11[k] + b12[k] for k in HP})

    def step4(j, tie):
        b11, b22, b21 = held[(j, 11)], held[(j, 22)], zblock(j, 2, 0, tie)
        deep(3, j, {k: b21[k] - b11[k] for k in HP})
        deep(6, j, {k: b21[k] + b22[k] for k in HP})

    def zrem(p, r0, tie):
        m = tie(st[p].m)
        xf = x_ref[2 * KH + r0:2 * KH + r0 + 32, st[p].cs].astype(F32)
        z = (xf.reshape(4, 8, 256) - m[None]) * st[p].r[None]
        zr[r0:r0 + 32, pl.ds(256 * p, 256)] = z.reshape(32, 256).astype(BF16)

    items = st[0].items + st[1].items
    items += [(functools.partial(zrem, 0, r0), 28) for r0 in range(0, KR, 32)]
    for j in range(0, 128, 8):
        items += [(functools.partial(step1, j), 20.5), (functools.partial(step2, j), 26.5),
                  (functools.partial(step3, j), 37), (functools.partial(step4, j), 37)]
    items += [(functools.partial(zrem, 1, r0), 28) for r0 in range(0, KR, 32)]
    return items


def _time_slots(items, first):
    room = []
    for kind in ROUNDS[first]:
        for _ in range(Q // 8):
            t = 8 * len(room)
            r = 2.1 if t < (400 if first else 472) else 1.6
            room.append(0.0 if t < 32 else r * (1.2 if kind == "s" else 1.0))
    room += [2.6] * (H // 8)
    scale = sum(room) / sum(cost for _, cost in items)
    pos, cum, acc, k = [], 0, 0.0, 0
    for _, cost in items:
        while acc + room[k] <= scale * cum + 1e-9:
            acc += room[k]
            k += 1
        pos.append(8 * k)
        cum += cost
    return pos


def _mm_group(a1_ref, a2_ref, ar_ref, e_ref, s_ref, t_ref, first, zb, zr, o_ref,
              col0, items, tail, never, after_rows=None):
    t0, t1 = TAIL[first]
    pos = _time_slots(items, first)
    pos += [t0 + (t1 - t0) * k / len(tail) for k in range(len(tail))]
    items = items + tail
    state = [0, 0]

    def release(mt):
        lo, span = state[1], mt.shape[0]
        while state[0] < len(items) and pos[state[0]] < lo + span:
            rr = min(span - 8, int(pos[state[0]] - lo) // 8 * 8)
            src = mt[rr:rr + 8, :128]
            items[state[0]][0](functools.partial(_tie, never, src))
            state[0] += 1
        state[1] += span

    def tile(key):
        e = TILE[key]
        return zb[e // 2, :, pl.ds(128 * (e % 2), 128)]

    def prod(t, u):
        e = A_IDX[(t, u)]
        a = _unpack(a2_ref[e // 2, :, pl.ds(128 * (e % 2), 128)])
        return jnp.dot(a, tile((t, u)), preferred_element_type=F32)

    def round_2345(u, with_67):
        p = {t: prod(t, u) for t in (1, 2, 3, 4)}
        e11, e22 = p[3] - p[4], p[2] - p[1]
        if with_67:
            e11, e22 = e11 + s_ref[0], e22 + s_ref[1]
        e_ref[0, u] = e11
        e_ref[1, u] = p[2] + p[4]
        e_ref[2, u] = p[1] + p[3]
        e_ref[3, u] = e22
        release(p[1])

    def add_67(u):
        p7, p6 = prod(6, u), prod(5, u)
        e_ref[0, u] = p7 + e_ref[0, u]
        e_ref[3, u] = p6 + e_ref[3, u]
        return p7

    def hold_67(u):
        p7, p6 = prod(6, u), prod(5, u)
        s_ref[0] = p7
        s_ref[1] = p6
        return p7

    def three_rounds(u):
        round_2345(u, False)
        p7 = add_67(u)
        hold_67(u + 1)
        release(p7)
        round_2345(u + 1, True)

    if first:
        for u in (0, 2, 4):
            three_rounds(u)
        round_2345(6, False)
        add_67(6)
    else:
        release(hold_67(0))
        round_2345(0, True)
        for u in (1, 3, 5):
            three_rounds(u)

    bt = jnp.concatenate(
        [jnp.concatenate([tile((0, h, p)) for p in range(2)], axis=1)
         for h in range(2)], axis=0)
    m1 = jnp.dot(_unpack(a1_ref[...]), bt, preferred_element_type=F32)
    t_ref[...] = m1
    release(m1)
    rem = jnp.dot(_unpack(ar_ref[...])[:, :KX], zr[...], preferred_element_type=F32)
    release(rem)

    def quadrant(f, q, p, base):
        if (q, p) == (0, 0):
            return base + e_ref[f, 0] + e_ref[f, 3] - e_ref[f, 4] + e_ref[f, 6]
        if (q, p) == (0, 1):
            return base + e_ref[f, 2] + e_ref[f, 4]
        if (q, p) == (1, 0):
            return base + e_ref[f, 1] + e_ref[f, 3]
        return base + e_ref[f, 0] - e_ref[f, 1] + e_ref[f, 2] + e_ref[f, 5]

    for half in range(2):
        for q in range(2):
            r0 = half * H + q * Q
            for p in range(2):
                left = rem[r0:r0 + Q, 256 * p:256 * p + 128]
                right = rem[r0:r0 + Q, 256 * p + 128:256 * p + 256]
                m1_part = t_ref[pl.ds(q * Q, Q), pl.ds(128 * p, 128)]
                if half == 0:
                    left = quadrant(0, q, p, left + m1_part)
                    right = quadrant(1, q, p, right)
                else:
                    left = quadrant(2, q, p, left)
                    right = quadrant(3, q, p, right + m1_part)
                o_ref[pl.ds(r0, Q), pl.ds(col0 + 256 * p, 256)] = jnp.concatenate(
                    [left, right], axis=1).astype(BF16)
            if after_rows is not None:
                after_rows(r0)


def _kernel(x_hbm, g_hbm, b_hbm, w_hbm, o_hbm,
            xbuf, obuf, gbuf, bbuf, wbuf, a1_ref, a2_ref, ar_ref, e_ref, s_ref, t_ref,
            zb0, zr0, zb1, zr1, c_ref, sem_x0, sem_w, sem_x, sem_o):
    S = xbuf.shape[0]
    n_ramp = sum(RAMP)
    n_body = (S - 1 - n_ramp) // SPB

    def x0_copy(h):
        cols = pl.ds(GW * h, GW)
        return pltpu.make_async_copy(x_hbm.at[0, :, cols], xbuf.at[0, :, cols],
                                     sem_x0.at[h])

    def x_copy(s):
        return pltpu.make_async_copy(x_hbm.at[s], xbuf.at[s], sem_x.at[s])

    def o_part_start(s, h, r0, rows):
        sl = (s, pl.ds(r0, rows), pl.ds(GW * h, GW))
        pltpu.make_async_copy(obuf.at[sl], o_hbm.at[sl], sem_o).start()

    def o_start(s0, n):
        for c in range(2 * GW // 128):
            sl = (pl.ds(s0, n), slice(None), pl.ds(c * 128, 128))
            pltpu.make_async_copy(obuf.at[sl], o_hbm.at[sl], sem_o).start(priority=c % 2)

    w_copies = [pltpu.make_async_copy(g_hbm, gbuf, sem_w.at[0]),
                pltpu.make_async_copy(b_hbm, bbuf, sem_w.at[1]),
                pltpu.make_async_copy(w_hbm, wbuf, sem_w.at[2])]

    head = [x0_copy(0)] + w_copies + [x0_copy(1)]

    def issue_head(k, carry):
        for kk, cp in enumerate(head):
            pl.when(k == kk)(cp.start)
        return carry

    jax.lax.fori_loop(0, len(head), issue_head, 0)

    def issue_x(s, carry):
        x_copy(s).start()
        return carry

    jax.lax.fori_loop(1, S, issue_x, 0)

    row = jax.lax.broadcasted_iota(jnp.int32, (16, GW), 0)
    ones = jnp.where(row < 3, 1.0, 0.0).astype(BF16)
    zr0[KR:, :] = ones
    zr1[KR:, :] = ones

    x0_copy(0).wait()
    for item, _ in _norm_items(xbuf.at[0], 0, zb0, zr0):
        item(lambda v: v)
    for c in w_copies:
        c.wait()
    _prep_weights(gbuf, bbuf, wbuf, a1_ref, a2_ref, ar_ref)
    x0_copy(1).wait()
    gv = jnp.broadcast_to(gbuf[...].astype(F32).reshape(1, D)[:, :256], (8, 256))
    never = gv != gv
    mm_a = functools.partial(_mm_group, a1_ref, a2_ref, ar_ref, e_ref.at[0],
                             s_ref.at[0], t_ref.at[0], True)
    mm_b = functools.partial(_mm_group, a1_ref, a2_ref, ar_ref, e_ref.at[1],
                             s_ref.at[1], t_ref.at[1], False)

    def ahead(i, h):
        return _Stats(xbuf.at[i], GW * h, save=c_ref.at[h]).items

    def block(i0, n, write):
        for u in range(n):
            i = i0 + u
            nxt = jnp.minimum(i + 1, S - 1)
            mm_a(zb0, zr0, obuf.at[i], 0,
                 _norm_items(xbuf.at[i], GW, zb1, zr1, c_ref.at[1]), ahead(nxt, 0), never)
            after_rows = None
            if write and u == n - 1:
                pl.when(i == S - 1)(functools.partial(o_part_start, i, 0, 0, D))

                def after_rows(r0, i=i):
                    pl.when(i == S - 1)(functools.partial(o_part_start, i, 1, r0, Q))
            mm_b(zb1, zr1, obuf.at[i], GW,
                 _norm_items(xbuf.at[nxt], 0, zb0, zr0, c_ref.at[0]), ahead(nxt, 1),
                 never, after_rows)
            if write:
                if (W_START - 2 - n_ramp) % SPB == u:
                    pl.when(i == W_START - 1)(functools.partial(o_start, 0, W_START))
                pl.when(jnp.logical_and(i >= W_START, i < S - 1))(
                    functools.partial(o_start, i, 1))

    mm_a(zb0, zr0, obuf.at[0], 0, _norm_items(xbuf.at[0], GW, zb1, zr1), [], never)
    x_copy(1).wait()
    mm_a(zb1, zr1, obuf.at[0], GW, _norm_items(xbuf.at[1], 0, zb0, zr0), ahead(1, 1),
         never)
    i = 1
    for n in RAMP:
        for u in range(n):
            x_copy(i + u + 1).wait()
        block(i, n, False)
        i += n

    def body(j, carry):
        i0 = 1 + n_ramp + j * SPB
        for u in range(SPB - 1):
            x_copy(i0 + u + 1).wait()
        pl.when(j < n_body - 1)(x_copy(jnp.minimum(i0 + SPB, S - 1)).wait)
        block(i0, SPB, True)
        return carry

    jax.lax.fori_loop(0, n_body, body, 0)
    pltpu.make_async_copy(obuf, o_hbm, sem_o).wait()


@jax.jit
def pallas_standalone__layernorm_linear__sampling_kernel(
    x: jax.Array,
    g: jax.Array,
    b: jax.Array,
    w: jax.Array,
):
    B, S, d = x.shape
    assert d == D and B == 2 * GW and (S - 1 - sum(RAMP)) % SPB == 0
    assert 1 + sum(RAMP) < W_START < S
    xt = jnp.transpose(x, (1, 2, 0))
    out = pl.pallas_call(
        _kernel,
        in_specs=[pl.BlockSpec(memory_space=pl.ANY)] * 4,
        out_specs=pl.BlockSpec(memory_space=pl.ANY),
        out_shape=jax.ShapeDtypeStruct((S, D, B), x.dtype),
        scratch_shapes=[
            pltpu.VMEM((S, D, B), BF16),
            pltpu.VMEM((S, D, B), BF16),
            pltpu.VMEM((D,), BF16),
            pltpu.VMEM((D,), BF16),
            pltpu.VMEM((D, D), BF16),
            pltpu.VMEM((H // 2, KH), U32),
            pltpu.VMEM((21, Q // 2, 256), U32),
            pltpu.VMEM((D // 2, 128), U32),
            pltpu.VMEM((2, 4, 7, Q, 128), F32),
            pltpu.VMEM((2, 2, Q, 128), F32),
            pltpu.VMEM((2, H, 256), F32),
            pltpu.VMEM((N_TILES // 2, 128, 256), BF16),
            pltpu.VMEM((KX, GW), BF16),
            pltpu.VMEM((N_TILES // 2, 128, 256), BF16),
            pltpu.VMEM((KX, GW), BF16),
            pltpu.VMEM((2, 2, 8, 256), F32),
            pltpu.SemaphoreType.DMA((2,)),
            pltpu.SemaphoreType.DMA((3,)),
            pltpu.SemaphoreType.DMA((S,)),
            pltpu.SemaphoreType.DMA(()),
        ],
        compiler_params=pltpu.CompilerParams(
            vmem_limit_bytes=110 * 1024 * 1024,
            disable_bounds_checks=True,
            disable_semaphore_checks=True,
        ),
    )(xt, g, b, w)
    return jnp.transpose(out, (2, 0, 1))
```

```python
import functools

import jax
import jax.numpy as jnp
import jax.experimental.pallas as pl
import jax.experimental.pallas.tpu as pltpu

F32 = jnp.float32
BF16 = jnp.bfloat16
U32 = jnp.uint32

EPS = 1e-5
D = 576
H = D // 2
Q = H // 2
KH = 256
KR = D - 2 * KH
KX = KR + 16
GW = 512
RAMP = (1, 2)
SPB = 4
W_START = 14

DEEP = (1, 2, 3, 4, 5, 6)
A_IDX = {(t, u): 7 * i + u for i, t in enumerate(DEEP) for u in range(7)}
TILE = {}
for _t in (1, 4, 2, 5, 3, 6):
    for _u in range(7):
        TILE[(_t, _u)] = len(TILE)
for _h in range(2):
    for _p in range(2):
        TILE[(0, _h, _p)] = len(TILE)
N_TILES = len(TILE)
HP = ((0, 0), (0, 1), (1, 0), (1, 1))
ROUNDS = {True: "qsq" * 3 + "q", False: "sq" + "qsq" * 3}
TAIL = {True: (1750, 2290), False: (1890, 2430)}


def _pack(v):
    return pltpu.bitcast(v, U32)


def _unpack(v):
    return pltpu.bitcast(v, BF16)


def _a_ops(a11, a12, a21, a22):
    return [a11 + a22, a21 + a22, a11, a22, a11 + a12, a21 - a11, a12 - a22]


def _b_ops(b11, b12, b21, b22):
    return [b11 + b22, b11, b12 - b22, b21 - b11, b22, b11 + b12, b21 + b22]


def _prep_weights(g_ref, b_ref, w_ref, a1_ref, a2_ref, ar_ref):
    g = g_ref[...].astype(F32).reshape(1, D)
    b16 = jnp.broadcast_to(b_ref[...].reshape(1, D), (16, D))
    c = jnp.dot(b16, w_ref[...], preferred_element_type=F32)
    c_hi = c.astype(BF16).astype(F32)
    rest = c - c_hi
    c_mid = rest.astype(BF16).astype(F32)
    c_lo = rest - c_mid
    row = jax.lax.broadcasted_iota(jnp.int32, (16, D), 0)
    ext = jnp.where(row == 0, c_hi,
                    jnp.where(row == 1, c_mid,
                              jnp.where(row == 2, c_lo, 0.0))).astype(BF16)
    wr = jnp.concatenate(
        [w_ref[2 * KH:, :], ext, jnp.zeros((128 - KX, D), BF16)], axis=0)
    gr = jnp.concatenate([g[:, 2 * KH:], jnp.ones((1, 128 - KR), F32)], axis=1)
    ar_ref[...] = _pack((wr.astype(F32).T * gr).astype(BF16))
    w1 = w_ref[:KH, :].astype(F32).T * g[:, :KH]
    w2 = w_ref[KH:2 * KH, :].astype(F32).T * g[:, KH:2 * KH]
    ops = _a_ops(w1[:H], w2[:H], w1[H:], w2[H:])
    a1_ref[...] = _pack(ops[0].astype(BF16))
    subs = []
    for t in DEEP:
        a = ops[t]
        subs += _a_ops(a[:Q, :128], a[:Q, 128:], a[Q:, :128], a[Q:, 128:])
    for e in range(0, len(subs), 2):
        a2_ref[e // 2] = _pack(
            jnp.concatenate([subs[e], subs[e + 1]], axis=1).astype(BF16))


class _Stats:
    def __init__(self, x_ref, col0, save=None, load=None):
        self.x, self.cs, self.save = x_ref, pl.ds(col0, 256), save
        self.s1 = self.s2 = self.p = self.m = self.r = None
        self.items = []
        if load is not None:
            self.m, self.r = load[0], load[1]
        else:
            self.items = [(functools.partial(self.stat, r0, 32), 40)
                          for r0 in range(0, D, 32)]

    def stat(self, r0, rows, tie):
        if self.p is None:
            first = self.x[0:16, self.cs].astype(F32)[0:1, :]
            self.p = jnp.broadcast_to(first, (8, 256))
        p = tie(self.p)
        s1 = s2 = None
        for r in range(r0, r0 + rows, 8):
            d = self.x[r:r + 8, self.cs].astype(F32) - p
            s1 = d if s1 is None else s1 + d
            s2 = d * d if s2 is None else s2 + d * d
        self.s1 = s1 if self.s1 is None else self.s1 + s1
        self.s2 = s2 if self.s2 is None else self.s2 + s2
        if r0 + rows == D:
            e1 = jnp.sum(self.s1, axis=0, keepdims=True) * (1.0 / D)
            e2 = jnp.sum(self.s2, axis=0, keepdims=True) * (1.0 / D)
            var = jnp.maximum(e2 - e1 * e1, 0.0)
            self.m = self.p + e1
            self.r = jnp.broadcast_to(jax.lax.rsqrt(var + EPS), (8, 256))
            if self.save is not None:
                self.save[0] = self.m
                self.save[1] = self.r


def _tie(never, src, v):
    if v.shape[1] == 256:
        src = jnp.concatenate([src, src], axis=1)
    return jax.lax.select(never[v.shape[1]], src, v)


def _norm_items(x_ref, col0, zb, zr, stats0=None):
    st = [_Stats(x_ref, col0, load=stats0), _Stats(x_ref, col0 + 256)]
    held, pending = {}, {}

    def put(keys, j, vals):
        for key, v in zip(keys, vals):
            e = TILE[key]
            other = pending.pop((e ^ 1, j), None)
            if other is None:
                pending[(e, j)] = v
                continue
            pair = [v, other] if e % 2 == 0 else [other, v]
            zb[e // 2, j:j + 8, :] = jnp.concatenate(pair, axis=1).astype(BF16)

    def deep(t, j, bt):
        put([(t, u) for u in range(7)], j, _b_ops(*[bt[k] for k in HP]))

    def zblock(j, kq, side, tie):
        out = {}
        for p in range(2):
            ls = slice(128 * side, 128 * side + 128)
            m, r = tie(st[p].m[:, ls]), st[p].r[:, ls]
            for h in range(2):
                r0 = 128 * (kq + h) + j
                out[(h, p)] = (x_ref[r0:r0 + 8, st[p].cs].astype(F32)[:, ls] - m) * r
        return out

    def step1(j, tie):
        b11 = held[(j, 11)] = zblock(j, 0, 0, tie)
        deep(1, j, b11)

    def step2(j, tie):
        b11, b22 = held[(j, 11)], zblock(j, 2, 1, tie)
        held[(j, 22)] = b22
        deep(4, j, b22)
        put([(0,) + k for k in HP], j, [b11[k] + b22[k] for k in HP])

    def step3(j, tie):
        b11, b22, b12 = held[(j, 11)], held[(j, 22)], zblock(j, 0, 1, tie)
        deep(2, j, {k: b12[k] - b22[k] for k in HP})
        deep(5, j, {k: b11[k] + b12[k] for k in HP})

    def step4(j, tie):
        b11, b22, b21 = held[(j, 11)], held[(j, 22)], zblock(j, 2, 0, tie)
        deep(3, j, {k: b21[k] - b11[k] for k in HP})
        deep(6, j, {k: b21[k] + b22[k] for k in HP})

    def zrem(p, r0, tie):
        m = tie(st[p].m)
        xf = x_ref[2 * KH + r0:2 * KH + r0 + 32, st[p].cs].astype(F32)
        z = (xf.reshape(4, 8, 256) - m[None]) * st[p].r[None]
        zr[r0:r0 + 32, pl.ds(256 * p, 256)] = z.reshape(32, 256).astype(BF16)

    items = st[0].items + st[1].items
    items += [(functools.partial(zrem, 0, r0), 28) for r0 in range(0, KR, 32)]
    for j in range(0, 128, 8):
        items += [(functools.partial(step1, j), 20.5), (functools.partial(step2, j), 26.5),
                  (functools.partial(step3, j), 37), (functools.partial(step4, j), 37)]
    items += [(functools.partial(zrem, 1, r0), 28) for r0 in range(0, KR, 32)]
    return items


def _time_slots(items, first):
    room = []
    for kind in ROUNDS[first]:
        for _ in range(Q // 8):
            t = 8 * len(room)
            r = 2.1 if t < (400 if first else 472) else 1.6
            room.append(0.0 if t < 32 else r * (1.2 if kind == "s" else 1.0))
    room += [2.6] * (H // 8)
    scale = sum(room) / sum(cost for _, cost in items)
    pos, cum, acc, k = [], 0, 0.0, 0
    for _, cost in items:
        while acc + room[k] <= scale * cum + 1e-9:
            acc += room[k]
            k += 1
        pos.append(8 * k)
        cum += cost
    return pos


def _mm_group(a1_ref, a2_ref, ar_ref, e_ref, s_ref, t_ref, first, zb, zr, o_ref,
              col0, items, tail, never, after_rows=None):
    t0, t1 = TAIL[first]
    pos = _time_slots(items, first)
    pos += [t0 + (t1 - t0) * k / len(tail) for k in range(len(tail))]
    items = items + tail
    state = [0, 0]

    def release(mt):
        lo, span = state[1], mt.shape[0]
        while state[0] < len(items) and pos[state[0]] < lo + span:
            rr = min(span - 8, int(pos[state[0]] - lo) // 8 * 8)
            src = mt[rr:rr + 8, :128]
            items[state[0]][0](functools.partial(_tie, never, src))
            state[0] += 1
        state[1] += span

    def tile(key):
        e = TILE[key]
        return zb[e // 2, :, pl.ds(128 * (e % 2), 128)]

    def prod(t, u):
        e = A_IDX[(t, u)]
        a = _unpack(a2_ref[e // 2, :, pl.ds(128 * (e % 2), 128)])
        return jnp.dot(a, tile((t, u)), preferred_element_type=F32)

    def round_2345(u, with_67):
        p = {t: prod(t, u) for t in (1, 2, 3, 4)}
        e11, e22 = p[3] - p[4], p[2] - p[1]
        if with_67:
            e11, e22 = e11 + s_ref[0], e22 + s_ref[1]
        e_ref[0, u] = e11
        e_ref[1, u] = p[2] + p[4]
        e_ref[2, u] = p[1] + p[3]
        e_ref[3, u] = e22
        release(p[1])

    def add_67(u):
        p7, p6 = prod(6, u), prod(5, u)
        e_ref[0, u] = p7 + e_ref[0, u]
        e_ref[3, u] = p6 + e_ref[3, u]
        return p7

    def hold_67(u):
        p7, p6 = prod(6, u), prod(5, u)
        s_ref[0] = p7
        s_ref[1] = p6
        return p7

    def three_rounds(u):
        round_2345(u, False)
        p7 = add_67(u)
        hold_67(u + 1)
        release(p7)
        round_2345(u + 1, True)

    if first:
        for u in (0, 2, 4):
            three_rounds(u)
        round_2345(6, False)
        add_67(6)
    else:
        release(hold_67(0))
        round_2345(0, True)
        for u in (1, 3, 5):
            three_rounds(u)

    bt = jnp.concatenate(
        [jnp.concatenate([tile((0, h, p)) for p in range(2)], axis=1)
         for h in range(2)], axis=0)
    m1 = jnp.dot(_unpack(a1_ref[...]), bt, preferred_element_type=F32)
    t_ref[...] = m1
    release(m1)
    rem = jnp.dot(_unpack(ar_ref[...])[:, :KX], zr[...], preferred_element_type=F32)
    release(rem)

    def quadrant(f, q, p, base):
        if (q, p) == (0, 0):
            return base + e_ref[f, 0] + e_ref[f, 3] - e_ref[f, 4] + e_ref[f, 6]
        if (q, p) == (0, 1):
            return base + e_ref[f, 2] + e_ref[f, 4]
        if (q, p) == (1, 0):
            return base + e_ref[f, 1] + e_ref[f, 3]
        return base + e_ref[f, 0] - e_ref[f, 1] + e_ref[f, 2] + e_ref[f, 5]

    for half in range(2):
        for q in range(2):
            r0 = half * H + q * Q
            for p in range(2):
                left = rem[r0:r0 + Q, 256 * p:256 * p + 128]
                right = rem[r0:r0 + Q, 256 * p + 128:256 * p + 256]
                m1_part = t_ref[pl.ds(q * Q, Q), pl.ds(128 * p, 128)]
                if half == 0:
                    left = quadrant(0, q, p, left + m1_part)
                    right = quadrant(1, q, p, right)
                else:
                    left = quadrant(2, q, p, left)
                    right = quadrant(3, q, p, right + m1_part)
                o_ref[pl.ds(r0, Q), pl.ds(col0 + 256 * p, 256)] = jnp.concatenate(
                    [left, right], axis=1).astype(BF16)
            if after_rows is not None:
                after_rows(r0)


def _kernel(x_hbm, g_hbm, b_hbm, w_hbm, o_hbm,
            xbuf, obuf, gbuf, bbuf, wbuf, a1_ref, a2_ref, ar_ref, e_ref, s_ref, t_ref,
            zb0, zr0, zb1, zr1, c_ref, sem_x0, sem_w, sem_x, sem_o):
    S = xbuf.shape[0]
    n_ramp = sum(RAMP)
    n_body = (S - 1 - n_ramp) // SPB

    def x0_copy(h):
        cols = pl.ds(GW * h, GW)
        return pltpu.make_async_copy(x_hbm.at[0, :, cols], xbuf.at[0, :, cols],
                                     sem_x0.at[h])

    def x_copy(s):
        return pltpu.make_async_copy(x_hbm.at[s], xbuf.at[s], sem_x.at[s])

    def o_part_start(s, h, r0, rows):
        sl = (s, pl.ds(r0, rows), pl.ds(GW * h, GW))
        pltpu.make_async_copy(obuf.at[sl], o_hbm.at[sl], sem_o).start()

    def o_start(s0, n):
        for c in range(2 * GW // 128):
            sl = (pl.ds(s0, n), slice(None), pl.ds(c * 128, 128))
            pltpu.make_async_copy(obuf.at[sl], o_hbm.at[sl], sem_o).start(priority=c % 2)

    w_copies = [pltpu.make_async_copy(g_hbm, gbuf, sem_w.at[0]),
                pltpu.make_async_copy(b_hbm, bbuf, sem_w.at[1]),
                pltpu.make_async_copy(w_hbm, wbuf, sem_w.at[2])]

    head = [x0_copy(0)] + w_copies + [x0_copy(1)]

    def issue_head(k, carry):
        for kk, cp in enumerate(head):
            pl.when(k == kk)(cp.start)
        return carry

    jax.lax.fori_loop(0, len(head), issue_head, 0)

    def issue_x(s, carry):
        x_copy(s).start()
        return carry

    jax.lax.fori_loop(1, S, issue_x, 0)

    row = jax.lax.broadcasted_iota(jnp.int32, (16, GW), 0)
    ones = jnp.where(row < 3, 1.0, 0.0).astype(BF16)
    zr0[KR:, :] = ones
    zr1[KR:, :] = ones

    x0_copy(0).wait()
    for item, _ in _norm_items(xbuf.at[0], 0, zb0, zr0):
        item(lambda v: v)
    for c in w_copies:
        c.wait()
    _prep_weights(gbuf, bbuf, wbuf, a1_ref, a2_ref, ar_ref)
    x0_copy(1).wait()
    gv = jnp.broadcast_to(gbuf[...].astype(F32).reshape(1, D)[:, :128], (8, 128))
    gv2 = jnp.concatenate([gv, gv], axis=1)
    never = {128: gv != gv, 256: gv2 != gv2}
    mm_a = functools.partial(_mm_group, a1_ref, a2_ref, ar_ref, e_ref.at[0],
                             s_ref.at[0], t_ref.at[0], True)
    mm_b = functools.partial(_mm_group, a1_ref, a2_ref, ar_ref, e_ref.at[1],
                             s_ref.at[1], t_ref.at[1], False)

    def ahead(i, h):
        return _Stats(xbuf.at[i], GW * h, save=c_ref.at[h]).items

    def block(i0, n, write):
        for u in range(n):
            i = i0 + u
            nxt = jnp.minimum(i + 1, S - 1)
            mm_a(zb0, zr0, obuf.at[i], 0,
                 _norm_items(xbuf.at[i], GW, zb1, zr1, c_ref.at[1]), ahead(nxt, 0), never)
            after_rows = None
            if write and u == n - 1:
                pl.when(i == S - 1)(functools.partial(o_part_start, i, 0, 0, D))

                def after_rows(r0, i=i):
                    pl.when(i == S - 1)(functools.partial(o_part_start, i, 1, r0, Q))
            mm_b(zb1, zr1, obuf.at[i], GW,
                 _norm_items(xbuf.at[nxt], 0, zb0, zr0, c_ref.at[0]), ahead(nxt, 1),
                 never, after_rows)
            if write:
                if (W_START - 2 - n_ramp) % SPB == u:
                    pl.when(i == W_START - 1)(functools.partial(o_start, 0, W_START))
                pl.when(jnp.logical_and(i >= W_START, i < S - 1))(
                    functools.partial(o_start, i, 1))

    mm_a(zb0, zr0, obuf.at[0], 0, _norm_items(xbuf.at[0], GW, zb1, zr1), [], never)
    x_copy(1).wait()
    mm_a(zb1, zr1, obuf.at[0], GW, _norm_items(xbuf.at[1], 0, zb0, zr0), ahead(1, 1),
         never)
    i = 1
    for n in RAMP:
        for u in range(n):
            x_copy(i + u + 1).wait()
        block(i, n, False)
        i += n

    def body(j, carry):
        i0 = 1 + n_ramp + j * SPB
        for u in range(SPB - 1):
            x_copy(i0 + u + 1).wait()
        pl.when(j < n_body - 1)(x_copy(jnp.minimum(i0 + SPB, S - 1)).wait)
        block(i0, SPB, True)
        return carry

    jax.lax.fori_loop(0, n_body, body, 0)
    pltpu.make_async_copy(obuf, o_hbm, sem_o).wait()


@jax.jit
def pallas_standalone__layernorm_linear__sampling_kernel(
    x: jax.Array,
    g: jax.Array,
    b: jax.Array,
    w: jax.Array,
):
    B, S, d = x.shape
    assert d == D and B == 2 * GW and (S - 1 - sum(RAMP)) % SPB == 0
    assert 1 + sum(RAMP) < W_START < S
    xt = jnp.transpose(x, (1, 2, 0))
    out = pl.pallas_call(
        _kernel,
        in_specs=[pl.BlockSpec(memory_space=pl.ANY)] * 4,
        out_specs=pl.BlockSpec(memory_space=pl.ANY),
        out_shape=jax.ShapeDtypeStruct((S, D, B), x.dtype),
        scratch_shapes=[
            pltpu.VMEM((S, D, B), BF16),
            pltpu.VMEM((S, D, B), BF16),
            pltpu.VMEM((D,), BF16),
            pltpu.VMEM((D,), BF16),
            pltpu.VMEM((D, D), BF16),
            pltpu.VMEM((H // 2, KH), U32),
            pltpu.VMEM((21, Q // 2, 256), U32),
            pltpu.VMEM((D // 2, 128), U32),
            pltpu.VMEM((2, 4, 7, Q, 128), F32),
            pltpu.VMEM((2, 2, Q, 128), F32),
            pltpu.VMEM((2, H, 256), F32),
            pltpu.VMEM((N_TILES // 2, 128, 256), BF16),
            pltpu.VMEM((KX, GW), BF16),
            pltpu.VMEM((N_TILES // 2, 128, 256), BF16),
            pltpu.VMEM((KX, GW), BF16),
            pltpu.VMEM((2, 2, 8, 256), F32),
            pltpu.SemaphoreType.DMA((2,)),
            pltpu.SemaphoreType.DMA((3,)),
            pltpu.SemaphoreType.DMA((S,)),
            pltpu.SemaphoreType.DMA(()),
        ],
        compiler_params=pltpu.CompilerParams(
            vmem_limit_bytes=110 * 1024 * 1024,
            disable_bounds_checks=True,
            disable_semaphore_checks=True,
        ),
    )(xt, g, b, w)
    return jnp.transpose(out, (2, 0, 1))
```

```python
import functools

import jax
import jax.numpy as jnp
import jax.experimental.pallas as pl
import jax.experimental.pallas.tpu as pltpu

F32 = jnp.float32
BF16 = jnp.bfloat16
U32 = jnp.uint32

EPS = 1e-5
D = 576
H = D // 2
Q = H // 2
KH = 256
KR = D - 2 * KH
KX = KR + 16
GW = 512
RAMP = (1, 2)
SPB = 4
W_START = 14

TILE = {(t, u): 7 * i + u for i, t in enumerate((1, 4, 2, 5, 3, 6, 0))
        for u in range(7)}
HP = ((0, 0), (0, 1), (1, 0), (1, 1))
COEF = (((0, 1), (3, 1)), ((2, 1), (3, -1)), ((1, 1), (3, 1)), ((0, 1), (2, 1)),
        ((0, -1), (1, 1)), ((3, 1),), ((0, 1),))
PACE = dict(lag=48, split=400, stats=2.1, ops=1.6, extra=150, extra_room=0.7,
            tail=(170, 560))


def _pack(v):
    return pltpu.bitcast(v, U32)


def _unpack(v):
    return pltpu.bitcast(v, BF16)


def _a_ops(a11, a12, a21, a22):
    return [a11 + a22, a21 + a22, a11, a22, a11 + a12, a21 - a11, a12 - a22]


def _b_ops(b11, b12, b21, b22):
    return [b11 + b22, b11, b12 - b22, b21 - b11, b22, b11 + b12, b21 + b22]


def _rounds(early):
    rest = [(t, u) for u in range(7) for t in (6, 0, 5)]
    out = [rest[:early]] if early else []
    rest = [rest[i:i + 4] for i in range(early, len(rest), 4)]
    for u in range(7):
        out.append([(t, u) for t in (1, 2, 3, 4)])
        if rest and (len(rest[0]) == 4 or u == 6):
            out.append(rest.pop(0))
    return out


def _prep_weights(g_ref, b_ref, w_ref, a_ref, ar_ref):
    g = g_ref[...].astype(F32).reshape(1, D)
    b16 = jnp.broadcast_to(b_ref[...].reshape(1, D), (16, D))
    c = jnp.dot(b16, w_ref[...], preferred_element_type=F32)
    c_hi = c.astype(BF16).astype(F32)
    rest = c - c_hi
    c_mid = rest.astype(BF16).astype(F32)
    c_lo = rest - c_mid
    row = jax.lax.broadcasted_iota(jnp.int32, (16, D), 0)
    ext = jnp.where(row == 0, c_hi,
                    jnp.where(row == 1, c_mid,
                              jnp.where(row == 2, c_lo, 0.0))).astype(BF16)
    wr = jnp.concatenate(
        [w_ref[2 * KH:, :], ext, jnp.zeros((128 - KX, D), BF16)], axis=0)
    gr = jnp.concatenate([g[:, 2 * KH:], jnp.ones((1, 128 - KR), F32)], axis=1)
    ar_ref[...] = _pack((wr.astype(F32).T * gr).astype(BF16))
    w1 = w_ref[:KH, :].astype(F32).T * g[:, :KH]
    w2 = w_ref[KH:2 * KH, :].astype(F32).T * g[:, KH:2 * KH]
    subs = []
    for a in _a_ops(w1[:H], w2[:H], w1[H:], w2[H:]):
        subs += _a_ops(a[:Q, :128], a[:Q, 128:], a[Q:, :128], a[Q:, 128:])
    for e in range(0, 48, 2):
        a_ref[e // 2] = _pack(
            jnp.concatenate([subs[e], subs[e + 1]], axis=1).astype(BF16))
    a_ref[24, :, :128] = _pack(subs[48].astype(BF16))


class _Stats:
    def __init__(self, x_ref, col0, save=None, load=None):
        self.x, self.cs, self.save = x_ref, pl.ds(col0, 256), save
        self.s1 = self.s2 = self.p = self.m = self.r = None
        self.items = []
        if load is not None:
            self.m, self.r = load[0], load[1]
        else:
            self.items = [(functools.partial(self.stat, r0, 32), 40)
                          for r0 in range(0, D, 32)]

    def stat(self, r0, rows, tie):
        if self.p is None:
            first = self.x[0:16, self.cs].astype(F32)[0:1, :]
            self.p = jnp.broadcast_to(first, (8, 256))
        p = tie(self.p)
        s1 = s2 = None
        for r in range(r0, r0 + rows, 8):
            d = self.x[r:r + 8, self.cs].astype(F32) - p
            s1 = d if s1 is None else s1 + d
            s2 = d * d if s2 is None else s2 + d * d
        self.s1 = s1 if self.s1 is None else self.s1 + s1
        self.s2 = s2 if self.s2 is None else self.s2 + s2
        if r0 + rows == D:
            e1 = jnp.sum(self.s1, axis=0, keepdims=True) * (1.0 / D)
            e2 = jnp.sum(self.s2, axis=0, keepdims=True) * (1.0 / D)
            var = jnp.maximum(e2 - e1 * e1, 0.0)
            self.m = self.p + e1
            self.r = jnp.broadcast_to(jax.lax.rsqrt(var + EPS), (8, 256))
            if self.save is not None:
                self.save[0] = self.m
                self.save[1] = self.r


def _tie(never, src, v):
    if v.shape[1] == 256:
        src = jnp.concatenate([src, src], axis=1)
    return jax.lax.select(never[v.shape[1]], src, v)


def _norm_items(x_ref, col0, zb, zr, stats0=None):
    st = [_Stats(x_ref, col0, load=stats0), _Stats(x_ref, col0 + 256)]
    held, pending = {}, {}

    def put(t, j, bt):
        for u, v in enumerate(_b_ops(*[bt[k] for k in HP])):
            e = TILE[(t, u)]
            if e == 48:
                zb[24, j:j + 8, :128] = v.astype(BF16)
            elif (e ^ 1, j) not in pending:
                pending[(e, j)] = v
            else:
                other = pending.pop((e ^ 1, j))
                pair = [v, other] if e % 2 == 0 else [other, v]
                zb[e // 2, j:j + 8, :] = jnp.concatenate(pair, axis=1).astype(BF16)

    def zblock(j, kq, side, tie):
        out = {}
        for p in range(2):
            ls = slice(128 * side, 128 * side + 128)
            m, r = tie(st[p].m[:, ls]), st[p].r[:, ls]
            for h in range(2):
                r0 = 128 * (kq + h) + j
                out[(h, p)] = (x_ref[r0:r0 + 8, st[p].cs].astype(F32)[:, ls] - m) * r
        return out

    def step1(j, tie):
        b11 = held[(j, 11)] = zblock(j, 0, 0, tie)
        put(1, j, b11)

    def step2(j, tie):
        b11, b22 = held[(j, 11)], zblock(j, 2, 1, tie)
        held[(j, 22)] = b22
        put(4, j, b22)
        put(0, j, {k: b11[k] + b22[k] for k in HP})

    def step3(j, tie):
        b11, b22, b12 = held[(j, 11)], held[(j, 22)], zblock(j, 0, 1, tie)
        put(2, j, {k: b12[k] - b22[k] for k in HP})
        put(5, j, {k: b11[k] + b12[k] for k in HP})

    def step4(j, tie):
        b11, b22, b21 = held[(j, 11)], held[(j, 22)], zblock(j, 2, 0, tie)
        put(3, j, {k: b21[k] - b11[k] for k in HP})
        put(6, j, {k: b21[k] + b22[k] for k in HP})

    def zrem(p, r0, tie):
        m = tie(st[p].m)
        xf = x_ref[2 * KH + r0:2 * KH + r0 + 32, st[p].cs].astype(F32)
        z = (xf.reshape(4, 8, 256) - m[None]) * st[p].r[None]
        zr[r0:r0 + 32, pl.ds(256 * p, 256)] = z.reshape(32, 256).astype(BF16)

    items = st[0].items + st[1].items
    items += [(functools.partial(zrem, 0, r0), 28) for r0 in range(0, KR, 32)]
    for j in range(0, 128, 8):
        items += [(functools.partial(step1, j), 20.5), (functools.partial(step2, j), 33),
                  (functools.partial(step3, j), 37), (functools.partial(step4, j), 37)]
    items += [(functools.partial(zrem, 1, r0), 28) for r0 in range(0, KR, 32)]
    return items


def _time_slots(items, tail, end):
    room = [0.0 if t < PACE["lag"] else
            PACE["stats"] if t < PACE["split"] else PACE["ops"]
            for t in range(0, end, 8)]
    room += [PACE["extra_room"]] * (PACE["extra"] // 8)
    scale = sum(room) / sum(cost for _, cost in items)
    pos, cum, acc, k = [], 0, 0.0, 0
    for _, cost in items:
        while acc + room[k] <= scale * cum + 1e-9:
            acc += room[k]
            k += 1
        pos.append(8 * k)
        cum += cost
    t0, t1 = PACE["tail"]
    return pos + [end + t0 + (t1 - t0) * k / len(tail) for k in range(len(tail))]


def _mm_group(a_ref, ar_ref, e_ref, early, zb, zr, o_ref, col0, items, tail, never,
              after_rows=None):
    rounds = _rounds(early)
    timed = [i == 0 or len(r) == 4 for i, r in enumerate(rounds)]
    pos = _time_slots(items, tail, Q * sum(timed))
    items = items + tail
    state = [0, 0]

    def release(mt):
        lo, span = state[1], mt.shape[0]
        while state[0] < len(items) and pos[state[0]] < lo + span:
            rr = min(span - 8, int(pos[state[0]] - lo) // 8 * 8)
            items[state[0]][0](functools.partial(_tie, never, mt[rr:rr + 8, :128]))
            state[0] += 1
        state[1] += span

    def prod(t, u):
        ea, eb = 7 * t + u, TILE[(t, u)]
        a = _unpack(a_ref[ea // 2, :, pl.ds(128 * (ea % 2), 128)])
        return jnp.dot(a, zb[eb // 2, :, pl.ds(128 * (eb % 2), 128)],
                       preferred_element_type=F32)

    started = set()
    for rnd, is_timed in zip(rounds, timed):
        ps = [prod(t, u) for t, u in rnd]
        terms = {}
        for (t, u), p in zip(rnd, ps):
            for f, sign in COEF[t]:
                terms.setdefault((f, u), []).append((sign, p))
        for (f, u), tm in terms.items():
            plus = [p for sign, p in tm if sign > 0]
            minus = [p for sign, p in tm if sign < 0]
            val = plus[0]
            for p in plus[1:]:
                val = val + p
            if (f, u) in started:
                val = val + e_ref[f, u]
            for p in minus:
                val = val - p
            e_ref[f, u] = val
            started.add((f, u))
        if is_timed:
            release(ps[0])
    rem = jnp.dot(_unpack(ar_ref[...])[:, :KX], zr[...], preferred_element_type=F32)
    release(rem)

    def quadrant(f, q, p, base):
        if (q, p) == (0, 0):
            return base + e_ref[f, 0] + e_ref[f, 3] - e_ref[f, 4] + e_ref[f, 6]
        if (q, p) == (0, 1):
            return base + e_ref[f, 2] + e_ref[f, 4]
        if (q, p) == (1, 0):
            return base + e_ref[f, 1] + e_ref[f, 3]
        return base + e_ref[f, 0] - e_ref[f, 1] + e_ref[f, 2] + e_ref[f, 5]

    for half in range(2):
        for q in range(2):
            r0 = half * H + q * Q
            for p in range(2):
                c0 = 256 * p
                left = quadrant(2 * half, q, p, rem[r0:r0 + Q, c0:c0 + 128])
                right = quadrant(2 * half + 1, q, p, rem[r0:r0 + Q, c0 + 128:c0 + 256])
                o_ref[pl.ds(r0, Q), pl.ds(col0 + c0, 256)] = jnp.concatenate(
                    [left, right], axis=1).astype(BF16)
            if after_rows is not None:
                after_rows(r0)


def _kernel(x_hbm, g_hbm, b_hbm, w_hbm, o_hbm,
            xbuf, obuf, gbuf, bbuf, wbuf, a_ref, ar_ref, e_ref,
            zb0, zr0, zb1, zr1, c_ref, sem_x0, sem_w, sem_x, sem_o):
    S = xbuf.shape[0]
    n_ramp = sum(RAMP)
    n_body = (S - 1 - n_ramp) // SPB

    def x0_copy(h):
        cols = pl.ds(GW * h, GW)
        return pltpu.make_async_copy(x_hbm.at[0, :, cols], xbuf.at[0, :, cols],
                                     sem_x0.at[h])

    def x_copy(s):
        return pltpu.make_async_copy(x_hbm.at[s], xbuf.at[s], sem_x.at[s])

    def o_part_start(s, h, r0, rows):
        sl = (s, pl.ds(r0, rows), pl.ds(GW * h, GW))
        pltpu.make_async_copy(obuf.at[sl], o_hbm.at[sl], sem_o).start()

    def o_start(s0, n):
        for c in range(2 * GW // 128):
            sl = (pl.ds(s0, n), slice(None), pl.ds(c * 128, 128))
            pltpu.make_async_copy(obuf.at[sl], o_hbm.at[sl], sem_o).start(priority=c % 2)

    w_copies = [pltpu.make_async_copy(g_hbm, gbuf, sem_w.at[0]),
                pltpu.make_async_copy(b_hbm, bbuf, sem_w.at[1]),
                pltpu.make_async_copy(w_hbm, wbuf, sem_w.at[2])]

    head = [x0_copy(0)] + w_copies + [x0_copy(1)]

    def issue_head(k, carry):
        for kk, cp in enumerate(head):
            pl.when(k == kk)(cp.start)
        return carry

    jax.lax.fori_loop(0, len(head), issue_head, 0)

    def issue_x(s, carry):
        x_copy(s).start()
        return carry

    jax.lax.fori_loop(1, S, issue_x, 0)

    row = jax.lax.broadcasted_iota(jnp.int32, (16, GW), 0)
    ones = jnp.where(row < 3, 1.0, 0.0).astype(BF16)
    zr0[KR:, :] = ones
    zr1[KR:, :] = ones

    x0_copy(0).wait()
    for item, _ in _norm_items(xbuf.at[0], 0, zb0, zr0):
        item(lambda v: v)
    for c in w_copies:
        c.wait()
    _prep_weights(gbuf, bbuf, wbuf, a_ref, ar_ref)
    x0_copy(1).wait()
    gv = jnp.broadcast_to(gbuf[...].astype(F32).reshape(1, D)[:, :128], (8, 128))
    gv2 = jnp.concatenate([gv, gv], axis=1)
    never = {128: gv != gv, 256: gv2 != gv2}

    def mm(k, *args):
        _mm_group(a_ref, ar_ref, e_ref.at[k % 2], -k % 4, *args)

    def ahead(i, h):
        return _Stats(xbuf.at[i], GW * h, save=c_ref.at[h]).items

    def block(i0, n, write):
        for u in range(n):
            i = i0 + u
            nxt = jnp.minimum(i + 1, S - 1)
            mm(2 * u, zb0, zr0, obuf.at[i], 0,
               _norm_items(xbuf.at[i], GW, zb1, zr1, c_ref.at[1]), ahead(nxt, 0), never)
            after_rows = None
            if write and u == n - 1:
                pl.when(i == S - 1)(functools.partial(o_part_start, i, 0, 0, D))

                def after_rows(r0, i=i):
                    pl.when(i == S - 1)(functools.partial(o_part_start, i, 1, r0, Q))
            mm(2 * u + 1, zb1, zr1, obuf.at[i], GW,
               _norm_items(xbuf.at[nxt], 0, zb0, zr0, c_ref.at[0]), ahead(nxt, 1),
               never, after_rows)
            if write:
                if (W_START - 2 - n_ramp) % SPB == u:
                    pl.when(i == W_START - 1)(functools.partial(o_start, 0, W_START))
                pl.when(jnp.logical_and(i >= W_START, i < S - 1))(
                    functools.partial(o_start, i, 1))

    mm(0, zb0, zr0, obuf.at[0], 0, _norm_items(xbuf.at[0], GW, zb1, zr1), [], never)
    x_copy(1).wait()
    mm(0, zb1, zr1, obuf.at[0], GW, _norm_items(xbuf.at[1], 0, zb0, zr0), ahead(1, 1),
       never)
    i = 1
    for n in RAMP:
        for u in range(n):
            x_copy(i + u + 1).wait()
        block(i, n, False)
        i += n

    def body(j, carry):
        i0 = 1 + n_ramp + j * SPB
        for u in range(SPB - 1):
            x_copy(i0 + u + 1).wait()
        pl.when(j < n_body - 1)(x_copy(jnp.minimum(i0 + SPB, S - 1)).wait)
        block(i0, SPB, True)
        return carry

    jax.lax.fori_loop(0, n_body, body, 0)
    pltpu.make_async_copy(obuf, o_hbm, sem_o).wait()


@jax.jit
def pallas_standalone__layernorm_linear__sampling_kernel(
    x: jax.Array,
    g: jax.Array,
    b: jax.Array,
    w: jax.Array,
):
    B, S, d = x.shape
    assert d == D and B == 2 * GW and (S - 1 - sum(RAMP)) % SPB == 0
    assert 1 + sum(RAMP) < W_START < S
    xt = jnp.transpose(x, (1, 2, 0))
    out = pl.pallas_call(
        _kernel,
        in_specs=[pl.BlockSpec(memory_space=pl.ANY)] * 4,
        out_specs=pl.BlockSpec(memory_space=pl.ANY),
        out_shape=jax.ShapeDtypeStruct((S, D, B), x.dtype),
        scratch_shapes=[
            pltpu.VMEM((S, D, B), BF16),
            pltpu.VMEM((S, D, B), BF16),
            pltpu.VMEM((D,), BF16),
            pltpu.VMEM((D,), BF16),
            pltpu.VMEM((D, D), BF16),
            pltpu.VMEM((25, Q // 2, 256), U32),
            pltpu.VMEM((D // 2, 128), U32),
            pltpu.VMEM((2, 4, 7, Q, 128), F32),
            pltpu.VMEM((25, 128, 256), BF16),
            pltpu.VMEM((KX, GW), BF16),
            pltpu.VMEM((25, 128, 256), BF16),
            pltpu.VMEM((KX, GW), BF16),
            pltpu.VMEM((2, 2, 8, 256), F32),
            pltpu.SemaphoreType.DMA((2,)),
            pltpu.SemaphoreType.DMA((3,)),
            pltpu.SemaphoreType.DMA((S,)),
            pltpu.SemaphoreType.DMA(()),
        ],
        compiler_params=pltpu.CompilerParams(
            vmem_limit_bytes=110 * 1024 * 1024,
            disable_bounds_checks=True,
            disable_semaphore_checks=True,
        ),
    )(xt, g, b, w)
    return jnp.transpose(out, (2, 0, 1))
```

```python
import functools

import jax
import jax.numpy as jnp
import jax.experimental.pallas as pl
import jax.experimental.pallas.tpu as pltpu

F32 = jnp.float32
BF16 = jnp.bfloat16
U32 = jnp.uint32

EPS = 1e-5
D = 576
H = D // 2
Q = H // 2
KH = 256
KR = D - 2 * KH
KX = KR + 16
GW = 512
RAMP = (1, 2)
SPB = 4
W_START = 14

TILE = {(t, u): 7 * i + u for i, t in enumerate((1, 4, 2, 5, 3, 6, 0))
        for u in range(7)}
HP = ((0, 0), (0, 1), (1, 0), (1, 1))
COEF = (((0, 1), (3, 1)), ((2, 1), (3, -1)), ((1, 1), (3, 1)), ((0, 1), (2, 1)),
        ((0, -1), (1, 1)), ((3, 1),), ((0, 1),))
PACE = dict(lag=48, split=400, stats=2.1, ops=1.6, extra=150, extra_room=0.7,
            tail=(170, 560))


def _pack(v):
    return pltpu.bitcast(v, U32)


def _unpack(v):
    return pltpu.bitcast(v, BF16)


def _a_ops(a11, a12, a21, a22):
    return [a11 + a22, a21 + a22, a11, a22, a11 + a12, a21 - a11, a12 - a22]


def _b_ops(b11, b12, b21, b22):
    return [b11 + b22, b11, b12 - b22, b21 - b11, b22, b11 + b12, b21 + b22]


def _rounds(early):
    rest = [(t, u) for u in range(7) for t in (6, 0, 5)]
    out = [rest[:early]] if early else []
    rest = [rest[i:i + 4] for i in range(early, len(rest), 4)]
    for u in range(7):
        out.append([(t, u) for t in (1, 2, 3, 4)])
        if rest and (len(rest[0]) == 4 or u == 6):
            out.append(rest.pop(0))
    return out


def _prep_weights(g_ref, b_ref, w_ref, a_ref, ar_ref):
    g = g_ref[...].astype(F32).reshape(1, D)
    row = jax.lax.broadcasted_iota(jnp.int32, (16, D), 0)
    bg = jnp.where(row < 8, b_ref[...].astype(F32).reshape(1, D), g).astype(BF16)
    cm = jnp.dot(bg, w_ref[...], preferred_element_type=F32)
    c = cm[0:1]
    c_hi = c.astype(BF16).astype(F32)
    rest = c - c_hi
    c_mid = rest.astype(BF16).astype(F32)
    c_lo = rest - c_mid
    mu = (cm[8:9] * (1.0 / D)).astype(BF16).astype(F32)
    ext = jnp.where(row == 0, c_hi,
                    jnp.where(row == 1, c_mid,
                              jnp.where(row == 2, c_lo,
                                        jnp.where(row == 15, mu, 0.0)))).astype(BF16)
    wr = jnp.concatenate(
        [w_ref[2 * KH:, :], ext, jnp.zeros((128 - KX, D), BF16)], axis=0).astype(F32).T
    mu = jnp.broadcast_to(wr[:, KX - 1:KX], (D, 128))
    lane = jax.lax.broadcasted_iota(jnp.int32, (1, 128), 1)
    gr = jnp.concatenate([g[:, 2 * KH:], jnp.ones((1, 128 - KR), F32)], axis=1)
    ar_ref[...] = _pack((wr * gr - jnp.where(lane < KR, mu, 0.0)).astype(BF16))
    mu = jnp.concatenate([mu, mu], axis=1)
    w1 = w_ref[:KH, :].astype(F32).T * g[:, :KH] - mu
    w2 = w_ref[KH:2 * KH, :].astype(F32).T * g[:, KH:2 * KH] - mu
    subs = []
    for a in _a_ops(w1[:H], w2[:H], w1[H:], w2[H:]):
        subs += _a_ops(a[:Q, :128], a[:Q, 128:], a[Q:, :128], a[Q:, 128:])
    for e in range(0, 48, 2):
        a_ref[e // 2] = _pack(
            jnp.concatenate([subs[e], subs[e + 1]], axis=1).astype(BF16))
    a_ref[24, :, :128] = _pack(subs[48].astype(BF16))


class _Stats:
    def __init__(self, x_ref, col0, save=None, load=None):
        self.x, self.cs, self.save = x_ref, pl.ds(col0, 256), save
        self.s1 = self.s2 = self.p = self.m = self.r = None
        self.items = []
        if load is not None:
            self.m, self.r = load[0], load[1]
        else:
            self.items = [(functools.partial(self.stat, r0, 32), 40)
                          for r0 in range(0, D, 32)]

    def stat(self, r0, rows, tie):
        if self.p is None:
            first = self.x[0:16, self.cs].astype(F32)[0:1, :]
            self.p = jnp.broadcast_to(first, (8, 256))
        p = tie(self.p)
        s1 = s2 = None
        for r in range(r0, r0 + rows, 8):
            d = self.x[r:r + 8, self.cs].astype(F32) - p
            s1 = d if s1 is None else s1 + d
            s2 = d * d if s2 is None else s2 + d * d
        self.s1 = s1 if self.s1 is None else self.s1 + s1
        self.s2 = s2 if self.s2 is None else self.s2 + s2
        if r0 + rows == D:
            e1 = jnp.sum(self.s1, axis=0, keepdims=True) * (1.0 / D)
            e2 = jnp.sum(self.s2, axis=0, keepdims=True) * (1.0 / D)
            var = jnp.maximum(e2 - e1 * e1, 0.0)
            self.m = self.p + e1
            self.r = jnp.broadcast_to(jax.lax.rsqrt(var + EPS), (8, 256))
            if self.save is not None:
                self.save[0] = self.m
                self.save[1] = self.r


def _tie(never, src, v):
    if v.shape[1] == 256:
        src = jnp.concatenate([src, src], axis=1)
    return jax.lax.select(never[v.shape[1]], src, v)


def _norm_items(x_ref, col0, zb, zr, stats0=None):
    st = [_Stats(x_ref, col0, load=stats0), _Stats(x_ref, col0 + 256)]
    held, pending = {}, {}

    def put(t, j, bt):
        for u, v in enumerate(_b_ops(*[bt[k] for k in HP])):
            e = TILE[(t, u)]
            if e == 48:
                zb[24, j:j + 8, :128] = v.astype(BF16)
            elif (e ^ 1, j) not in pending:
                pending[(e, j)] = v
            else:
                other = pending.pop((e ^ 1, j))
                pair = [v, other] if e % 2 == 0 else [other, v]
                zb[e // 2, j:j + 8, :] = jnp.concatenate(pair, axis=1).astype(BF16)

    def zblock(j, kq, side, tie):
        out = {}
        for p in range(2):
            ls = slice(128 * side, 128 * side + 128)
            m, r = tie(st[p].m[:, ls]), st[p].r[:, ls]
            for h in range(2):
                r0 = 128 * (kq + h) + j
                out[(h, p)] = (x_ref[r0:r0 + 8, st[p].cs].astype(F32)[:, ls] - m) * r
        return out

    def step1(j, tie):
        b11 = held[(j, 11)] = zblock(j, 0, 0, tie)
        put(1, j, b11)

    def step2(j, tie):
        b11, b22 = held[(j, 11)], zblock(j, 2, 1, tie)
        held[(j, 22)] = b22
        put(4, j, b22)
        put(0, j, {k: b11[k] + b22[k] for k in HP})

    def step3(j, tie):
        b11, b22, b12 = held[(j, 11)], held[(j, 22)], zblock(j, 0, 1, tie)
        put(2, j, {k: b12[k] - b22[k] for k in HP})
        put(5, j, {k: b11[k] + b12[k] for k in HP})

    def step4(j, tie):
        b11, b22, b21 = held[(j, 11)], held[(j, 22)], zblock(j, 2, 0, tie)
        put(3, j, {k: b21[k] - b11[k] for k in HP})
        put(6, j, {k: b21[k] + b22[k] for k in HP})

    def zrem(p, r0, tie):
        m = tie(st[p].m)
        xf = x_ref[2 * KH + r0:2 * KH + r0 + 32, st[p].cs].astype(F32)
        z = (xf.reshape(4, 8, 256) - m[None]) * st[p].r[None]
        zr[r0:r0 + 32, pl.ds(256 * p, 256)] = z.reshape(32, 256).astype(BF16)

    items = st[0].items + st[1].items
    items += [(functools.partial(zrem, 0, r0), 28) for r0 in range(0, KR, 32)]
    for j in range(0, 128, 8):
        items += [(functools.partial(step1, j), 20.5), (functools.partial(step2, j), 33),
                  (functools.partial(step3, j), 37), (functools.partial(step4, j), 37)]
    items += [(functools.partial(zrem, 1, r0), 28) for r0 in range(0, KR, 32)]
    return items


def _time_slots(items, tail, end):
    room = [0.0 if t < PACE["lag"] else
            PACE["stats"] if t < PACE["split"] else PACE["ops"]
            for t in range(0, end, 8)]
    room += [PACE["extra_room"]] * (PACE["extra"] // 8)
    scale = sum(room) / sum(cost for _, cost in items)
    pos, cum, acc, k = [], 0, 0.0, 0
    for _, cost in items:
        while acc + room[k] <= scale * cum + 1e-9:
            acc += room[k]
            k += 1
        pos.append(8 * k)
        cum += cost
    t0, t1 = PACE["tail"]
    return pos + [end + t0 + (t1 - t0) * k / len(tail) for k in range(len(tail))]


def _mm_group(a_ref, ar_ref, e_ref, early, zb, zr, o_ref, col0, items, tail, never,
              after_rows=None):
    rounds = _rounds(early)
    timed = [i == 0 or len(r) == 4 for i, r in enumerate(rounds)]
    pos = _time_slots(items, tail, Q * sum(timed))
    items = items + tail
    state = [0, 0]

    def release(mt):
        lo, span = state[1], mt.shape[0]
        while state[0] < len(items) and pos[state[0]] < lo + span:
            rr = min(span - 8, int(pos[state[0]] - lo) // 8 * 8)
            items[state[0]][0](functools.partial(_tie, never, mt[rr:rr + 8, :128]))
            state[0] += 1
        state[1] += span

    def prod(t, u):
        ea, eb = 7 * t + u, TILE[(t, u)]
        a = _unpack(a_ref[ea // 2, :, pl.ds(128 * (ea % 2), 128)])
        return jnp.dot(a, zb[eb // 2, :, pl.ds(128 * (eb % 2), 128)],
                       preferred_element_type=F32)

    started = set()
    for rnd, is_timed in zip(rounds, timed):
        ps = [prod(t, u) for t, u in rnd]
        terms = {}
        for (t, u), p in zip(rnd, ps):
            for f, sign in COEF[t]:
                terms.setdefault((f, u), []).append((sign, p))
        for (f, u), tm in terms.items():
            plus = [p for sign, p in tm if sign > 0]
            minus = [p for sign, p in tm if sign < 0]
            val = plus[0]
            for p in plus[1:]:
                val = val + p
            if (f, u) in started:
                val = val + e_ref[f, u]
            for p in minus:
                val = val - p
            e_ref[f, u] = val
            started.add((f, u))
        if is_timed:
            release(ps[0])
    rem = jnp.dot(_unpack(ar_ref[...])[:, :KX], zr[...], preferred_element_type=F32)
    release(rem)

    def quadrant(f, q, p, base):
        if (q, p) == (0, 0):
            return base + e_ref[f, 0] + e_ref[f, 3] - e_ref[f, 4] + e_ref[f, 6]
        if (q, p) == (0, 1):
            return base + e_ref[f, 2] + e_ref[f, 4]
        if (q, p) == (1, 0):
            return base + e_ref[f, 1] + e_ref[f, 3]
        return base + e_ref[f, 0] - e_ref[f, 1] + e_ref[f, 2] + e_ref[f, 5]

    for half in range(2):
        for q in range(2):
            r0 = half * H + q * Q
            for p in range(2):
                c0 = 256 * p
                left = quadrant(2 * half, q, p, rem[r0:r0 + Q, c0:c0 + 128])
                right = quadrant(2 * half + 1, q, p, rem[r0:r0 + Q, c0 + 128:c0 + 256])
                o_ref[pl.ds(r0, Q), pl.ds(col0 + c0, 256)] = jnp.concatenate(
                    [left, right], axis=1).astype(BF16)
            if after_rows is not None:
                after_rows(r0)


def _kernel(x_hbm, g_hbm, b_hbm, w_hbm, o_hbm,
            xbuf, obuf, gbuf, bbuf, wbuf, a_ref, ar_ref, e_ref,
            zb0, zr0, zb1, zr1, c_ref, sem_x0, sem_w, sem_x, sem_o):
    S = xbuf.shape[0]
    n_ramp = sum(RAMP)
    n_body = (S - 1 - n_ramp) // SPB

    def x0_copy(h):
        cols = pl.ds(GW * h, GW)
        return pltpu.make_async_copy(x_hbm.at[0, :, cols], xbuf.at[0, :, cols],
                                     sem_x0.at[h])

    def x_copy(s):
        return pltpu.make_async_copy(x_hbm.at[s], xbuf.at[s], sem_x.at[s])

    def o_part_start(s, h, r0, rows):
        sl = (s, pl.ds(r0, rows), pl.ds(GW * h, GW))
        pltpu.make_async_copy(obuf.at[sl], o_hbm.at[sl], sem_o).start()

    def o_start(s0, n):
        for c in range(2 * GW // 128):
            sl = (pl.ds(s0, n), slice(None), pl.ds(c * 128, 128))
            pltpu.make_async_copy(obuf.at[sl], o_hbm.at[sl], sem_o).start(priority=c % 2)

    w_copies = [pltpu.make_async_copy(g_hbm, gbuf, sem_w.at[0]),
                pltpu.make_async_copy(b_hbm, bbuf, sem_w.at[1]),
                pltpu.make_async_copy(w_hbm, wbuf, sem_w.at[2])]

    head = [x0_copy(0)] + w_copies + [x0_copy(1)]

    def issue_head(k, carry):
        for kk, cp in enumerate(head):
            pl.when(k == kk)(cp.start)
        return carry

    jax.lax.fori_loop(0, len(head), issue_head, 0)

    def issue_x(s, carry):
        x_copy(s).start()
        return carry

    jax.lax.fori_loop(1, S, issue_x, 0)

    row = jax.lax.broadcasted_iota(jnp.int32, (16, GW), 0)
    ones = jnp.where(row < 3, 1.0, 0.0).astype(BF16)
    zr0[KR:, :] = ones
    zr1[KR:, :] = ones

    x0_copy(0).wait()
    for item, _ in _norm_items(xbuf.at[0], 0, zb0, zr0):
        item(lambda v: v)
    for c in w_copies:
        c.wait()
    _prep_weights(gbuf, bbuf, wbuf, a_ref, ar_ref)
    x0_copy(1).wait()
    gv = jnp.broadcast_to(gbuf[...].astype(F32).reshape(1, D)[:, :128], (8, 128))
    gv2 = jnp.concatenate([gv, gv], axis=1)
    never = {128: gv != gv, 256: gv2 != gv2}

    def mm(k, *args):
        _mm_group(a_ref, ar_ref, e_ref.at[k % 2], -k % 4, *args)

    def ahead(i, h):
        return _Stats(xbuf.at[i], GW * h, save=c_ref.at[h]).items

    def block(i0, n, write):
        for u in range(n):
            i = i0 + u
            nxt = jnp.minimum(i + 1, S - 1)
            mm(2 * u, zb0, zr0, obuf.at[i], 0,
               _norm_items(xbuf.at[i], GW, zb1, zr1, c_ref.at[1]), ahead(nxt, 0), never)
            after_rows = None
            if write and u == n - 1:
                pl.when(i == S - 1)(functools.partial(o_part_start, i, 0, 0, D))

                def after_rows(r0, i=i):
                    pl.when(i == S - 1)(functools.partial(o_part_start, i, 1, r0, Q))
            mm(2 * u + 1, zb1, zr1, obuf.at[i], GW,
               _norm_items(xbuf.at[nxt], 0, zb0, zr0, c_ref.at[0]), ahead(nxt, 1),
               never, after_rows)
            if write:
                if (W_START - 2 - n_ramp) % SPB == u:
                    pl.when(i == W_START - 1)(functools.partial(o_start, 0, W_START))
                pl.when(jnp.logical_and(i >= W_START, i < S - 1))(
                    functools.partial(o_start, i, 1))

    mm(0, zb0, zr0, obuf.at[0], 0, _norm_items(xbuf.at[0], GW, zb1, zr1), [], never)
    x_copy(1).wait()
    mm(0, zb1, zr1, obuf.at[0], GW, _norm_items(xbuf.at[1], 0, zb0, zr0), ahead(1, 1),
       never)
    i = 1
    for n in RAMP:
        for u in range(n):
            x_copy(i + u + 1).wait()
        block(i, n, False)
        i += n

    def body(j, carry):
        i0 = 1 + n_ramp + j * SPB
        for u in range(SPB - 1):
            x_copy(i0 + u + 1).wait()
        pl.when(j < n_body - 1)(x_copy(jnp.minimum(i0 + SPB, S - 1)).wait)
        block(i0, SPB, True)
        return carry

    jax.lax.fori_loop(0, n_body, body, 0)
    pltpu.make_async_copy(obuf, o_hbm, sem_o).wait()


@jax.jit
def pallas_standalone__layernorm_linear__sampling_kernel(
    x: jax.Array,
    g: jax.Array,
    b: jax.Array,
    w: jax.Array,
):
    B, S, d = x.shape
    assert d == D and B == 2 * GW and (S - 1 - sum(RAMP)) % SPB == 0
    assert 1 + sum(RAMP) < W_START < S
    xt = jnp.transpose(x, (1, 2, 0))
    out = pl.pallas_call(
        _kernel,
        in_specs=[pl.BlockSpec(memory_space=pl.ANY)] * 4,
        out_specs=pl.BlockSpec(memory_space=pl.ANY),
        out_shape=jax.ShapeDtypeStruct((S, D, B), x.dtype),
        scratch_shapes=[
            pltpu.VMEM((S, D, B), BF16),
            pltpu.VMEM((S, D, B), BF16),
            pltpu.VMEM((D,), BF16),
            pltpu.VMEM((D,), BF16),
            pltpu.VMEM((D, D), BF16),
            pltpu.VMEM((25, Q // 2, 256), U32),
            pltpu.VMEM((D // 2, 128), U32),
            pltpu.VMEM((2, 4, 7, Q, 128), F32),
            pltpu.VMEM((25, 128, 256), BF16),
            pltpu.VMEM((KX, GW), BF16),
            pltpu.VMEM((25, 128, 256), BF16),
            pltpu.VMEM((KX, GW), BF16),
            pltpu.VMEM((2, 2, 8, 256), F32),
            pltpu.SemaphoreType.DMA((2,)),
            pltpu.SemaphoreType.DMA((3,)),
            pltpu.SemaphoreType.DMA((S,)),
            pltpu.SemaphoreType.DMA(()),
        ],
        compiler_params=pltpu.CompilerParams(
            vmem_limit_bytes=110 * 1024 * 1024,
            disable_bounds_checks=True,
            disable_semaphore_checks=True,
        ),
    )(xt, g, b, w)
    return jnp.transpose(out, (2, 0, 1))
```

```python
import functools

import jax
import jax.numpy as jnp
import jax.experimental.pallas as pl
import jax.experimental.pallas.tpu as pltpu

F32 = jnp.float32
BF16 = jnp.bfloat16
U32 = jnp.uint32

EPS = 1e-5
D = 576
H = D // 2
Q = H // 2
KH = 256
KR = D - 2 * KH
KX = KR + 16
GW = 512
RAMP = (1, 2)
SPB = 4
W_START = 14

TILE = {(t, u): 7 * i + u for i, t in enumerate((1, 4, 2, 5, 3, 6, 0))
        for u in range(7)}
HP = ((0, 0), (0, 1), (1, 0), (1, 1))
COEF = (((0, 1), (3, 1)), ((2, 1), (3, -1)), ((1, 1), (3, 1)), ((0, 1), (2, 1)),
        ((0, -1), (1, 1)), ((3, 1),), ((0, 1),))
PACE = dict(lag=48, split=400, stats=2.1, ops=1.6, extra=150, extra_room=0.7,
            tail=(170, 560))


def _pack(v):
    return pltpu.bitcast(v, U32)


def _unpack(v):
    return pltpu.bitcast(v, BF16)


def _a_ops(a11, a12, a21, a22):
    return [a11 + a22, a21 + a22, a11, a22, a11 + a12, a21 - a11, a12 - a22]


def _b_ops(b11, b12, b21, b22):
    return [b11 + b22, b11, b12 - b22, b21 - b11, b22, b11 + b12, b21 + b22]


def _rounds(early):
    rest = [(t, u) for u in range(7) for t in (6, 0, 5)]
    out = [rest[:early]] if early else []
    rest = [rest[i:i + 4] for i in range(early, len(rest), 4)]
    for u in range(7):
        out.append([(t, u) for t in (1, 2, 3, 4)])
        if rest and (len(rest[0]) == 4 or u == 6):
            out.append(rest.pop(0))
    return out


def _transpose(w):
    out = []
    for c0 in range(0, D, 128):
        n = min(128, D - c0)
        eye = (jax.lax.broadcasted_iota(jnp.int32, (n, n), 0)
               == jax.lax.broadcasted_iota(jnp.int32, (n, n), 1))
        eye = jnp.where(eye, 1.0, 0.0).astype(BF16)
        out.append(jax.lax.dot_general(eye, w[:, c0:c0 + n], (((1,), (1,)), ((), ())),
                                       preferred_element_type=F32))
    return jnp.concatenate(out, axis=0)


def _prep_weights(g_ref, b_ref, w_ref, a_ref, ar_ref):
    g = g_ref[...].astype(F32).reshape(1, D)
    row = jax.lax.broadcasted_iota(jnp.int32, (16, D), 0)
    bg = jnp.where(row < 8, b_ref[...].astype(F32).reshape(1, D), g).astype(BF16)
    cm = jnp.dot(bg, w_ref[...], preferred_element_type=F32)
    c = cm[0:1]
    c_hi = c.astype(BF16).astype(F32)
    rest = c - c_hi
    c_mid = rest.astype(BF16).astype(F32)
    c_lo = rest - c_mid
    mu = (cm[8:9] * (1.0 / D)).astype(BF16).astype(F32)
    ext = jnp.where(row == 0, c_hi,
                    jnp.where(row == 1, c_mid,
                              jnp.where(row == 2, c_lo,
                                        jnp.where(row == 15, mu, 0.0)))).astype(BF16)
    wr = _transpose(jnp.concatenate(
        [w_ref[2 * KH:, :], ext, jnp.zeros((128 - KX, D), BF16)], axis=0))
    mu = jnp.broadcast_to(wr[:, KX - 1:KX], (D, 128))
    lane = jax.lax.broadcasted_iota(jnp.int32, (1, 128), 1)
    gr = jnp.concatenate([g[:, 2 * KH:], jnp.ones((1, 128 - KR), F32)], axis=1)
    ar_ref[...] = _pack((wr * gr - jnp.where(lane < KR, mu, 0.0)).astype(BF16))
    mu = jnp.concatenate([mu, mu], axis=1)
    w1 = _transpose(w_ref[:KH, :]) * g[:, :KH] - mu
    w2 = _transpose(w_ref[KH:2 * KH, :]) * g[:, KH:2 * KH] - mu
    subs = []
    for a in _a_ops(w1[:H], w2[:H], w1[H:], w2[H:]):
        subs += _a_ops(a[:Q, :128], a[:Q, 128:], a[Q:, :128], a[Q:, 128:])
    for e in range(0, 48, 2):
        a_ref[e // 2] = _pack(
            jnp.concatenate([subs[e], subs[e + 1]], axis=1).astype(BF16))
    a_ref[24, :, :128] = _pack(subs[48].astype(BF16))


class _Stats:
    def __init__(self, x_ref, col0, save=None, load=None):
        self.x, self.cs, self.save = x_ref, pl.ds(col0, 256), save
        self.s1 = self.s2 = self.p = self.m = self.r = None
        self.items = []
        if load is not None:
            self.m, self.r = load[0], load[1]
        else:
            self.items = [(functools.partial(self.stat, r0, 32), 40)
                          for r0 in range(0, D, 32)]

    def stat(self, r0, rows, tie):
        if self.p is None:
            first = self.x[0:16, self.cs].astype(F32)[0:1, :]
            self.p = jnp.broadcast_to(first, (8, 256))
        p = tie(self.p)
        s1 = s2 = None
        for r in range(r0, r0 + rows, 8):
            d = self.x[r:r + 8, self.cs].astype(F32) - p
            s1 = d if s1 is None else s1 + d
            s2 = d * d if s2 is None else s2 + d * d
        self.s1 = s1 if self.s1 is None else self.s1 + s1
        self.s2 = s2 if self.s2 is None else self.s2 + s2
        if r0 + rows == D:
            e1 = jnp.sum(self.s1, axis=0, keepdims=True) * (1.0 / D)
            e2 = jnp.sum(self.s2, axis=0, keepdims=True) * (1.0 / D)
            var = jnp.maximum(e2 - e1 * e1, 0.0)
            self.m = self.p + e1
            self.r = jnp.broadcast_to(jax.lax.rsqrt(var + EPS), (8, 256))
            if self.save is not None:
                self.save[0] = self.m
                self.save[1] = self.r


def _tie(never, src, v):
    if v.shape[1] == 256:
        src = jnp.concatenate([src, src], axis=1)
    return jax.lax.select(never[v.shape[1]], src, v)


def _norm_items(x_ref, col0, zb, zr, stats0=None):
    st = [_Stats(x_ref, col0, load=stats0), _Stats(x_ref, col0 + 256)]
    held, pending = {}, {}

    def put(t, j, bt):
        for u, v in enumerate(_b_ops(*[bt[k] for k in HP])):
            e = TILE[(t, u)]
            if e == 48:
                zb[24, j:j + 8, :128] = v.astype(BF16)
            elif (e ^ 1, j) not in pending:
                pending[(e, j)] = v
            else:
                other = pending.pop((e ^ 1, j))
                pair = [v, other] if e % 2 == 0 else [other, v]
                zb[e // 2, j:j + 8, :] = jnp.concatenate(pair, axis=1).astype(BF16)

    def zblock(j, kq, side, tie):
        out = {}
        for p in range(2):
            ls = slice(128 * side, 128 * side + 128)
            m, r = tie(st[p].m[:, ls]), st[p].r[:, ls]
            for h in range(2):
                r0 = 128 * (kq + h) + j
                out[(h, p)] = (x_ref[r0:r0 + 8, st[p].cs].astype(F32)[:, ls] - m) * r
        return out

    def step1(j, tie):
        b11 = held[(j, 11)] = zblock(j, 0, 0, tie)
        put(1, j, b11)

    def step2(j, tie):
        b11, b22 = held[(j, 11)], zblock(j, 2, 1, tie)
        held[(j, 22)] = b22
        put(4, j, b22)
        put(0, j, {k: b11[k] + b22[k] for k in HP})

    def step3(j, tie):
        b11, b22, b12 = held[(j, 11)], held[(j, 22)], zblock(j, 0, 1, tie)
        put(2, j, {k: b12[k] - b22[k] for k in HP})
        put(5, j, {k: b11[k] + b12[k] for k in HP})

    def step4(j, tie):
        b11, b22, b21 = held[(j, 11)], held[(j, 22)], zblock(j, 2, 0, tie)
        put(3, j, {k: b21[k] - b11[k] for k in HP})
        put(6, j, {k: b21[k] + b22[k] for k in HP})

    def zrem(p, r0, tie):
        m = tie(st[p].m)
        xf = x_ref[2 * KH + r0:2 * KH + r0 + 32, st[p].cs].astype(F32)
        z = (xf.reshape(4, 8, 256) - m[None]) * st[p].r[None]
        zr[r0:r0 + 32, pl.ds(256 * p, 256)] = z.reshape(32, 256).astype(BF16)

    items = st[0].items + st[1].items
    items += [(functools.partial(zrem, 0, r0), 28) for r0 in range(0, KR, 32)]
    for j in range(0, 128, 8):
        items += [(functools.partial(step1, j), 20.5), (functools.partial(step2, j), 33),
                  (functools.partial(step3, j), 37), (functools.partial(step4, j), 37)]
    items += [(functools.partial(zrem, 1, r0), 28) for r0 in range(0, KR, 32)]
    return items


def _time_slots(items, tail, end):
    room = [0.0 if t < PACE["lag"] else
            PACE["stats"] if t < PACE["split"] else PACE["ops"]
            for t in range(0, end, 8)]
    room += [PACE["extra_room"]] * (PACE["extra"] // 8)
    scale = sum(room) / sum(cost for _, cost in items)
    pos, cum, acc, k = [], 0, 0.0, 0
    for _, cost in items:
        while acc + room[k] <= scale * cum + 1e-9:
            acc += room[k]
            k += 1
        pos.append(8 * k)
        cum += cost
    t0, t1 = PACE["tail"]
    return pos + [end + t0 + (t1 - t0) * k / len(tail) for k in range(len(tail))]


def _mm_group(a_ref, ar_ref, e_ref, early, zb, zr, o_ref, col0, items, tail, never,
              after_rows=None):
    rounds = _rounds(early)
    timed = [i == 0 or len(r) == 4 for i, r in enumerate(rounds)]
    pos = _time_slots(items, tail, Q * sum(timed))
    items = items + tail
    state = [0, 0]

    def release(mt):
        lo, span = state[1], mt.shape[0]
        while state[0] < len(items) and pos[state[0]] < lo + span:
            rr = min(span - 8, int(pos[state[0]] - lo) // 8 * 8)
            items[state[0]][0](functools.partial(_tie, never, mt[rr:rr + 8, :128]))
            state[0] += 1
        state[1] += span

    def prod(t, u):
        ea, eb = 7 * t + u, TILE[(t, u)]
        a = _unpack(a_ref[ea // 2, :, pl.ds(128 * (ea % 2), 128)])
        return jnp.dot(a, zb[eb // 2, :, pl.ds(128 * (eb % 2), 128)],
                       preferred_element_type=F32)

    started = set()
    for rnd, is_timed in zip(rounds, timed):
        ps = [prod(t, u) for t, u in rnd]
        terms = {}
        for (t, u), p in zip(rnd, ps):
            for f, sign in COEF[t]:
                terms.setdefault((f, u), []).append((sign, p))
        for (f, u), tm in terms.items():
            plus = [p for sign, p in tm if sign > 0]
            minus = [p for sign, p in tm if sign < 0]
            val = plus[0]
            for p in plus[1:]:
                val = val + p
            if (f, u) in started:
                val = val + e_ref[f, u]
            for p in minus:
                val = val - p
            e_ref[f, u] = val
            started.add((f, u))
        if is_timed:
            release(ps[0])
    rem = jnp.dot(_unpack(ar_ref[...])[:, :KX], zr[...], preferred_element_type=F32)
    release(rem)

    def quadrant(f, q, p, base):
        if (q, p) == (0, 0):
            return base + e_ref[f, 0] + e_ref[f, 3] - e_ref[f, 4] + e_ref[f, 6]
        if (q, p) == (0, 1):
            return base + e_ref[f, 2] + e_ref[f, 4]
        if (q, p) == (1, 0):
            return base + e_ref[f, 1] + e_ref[f, 3]
        return base + e_ref[f, 0] - e_ref[f, 1] + e_ref[f, 2] + e_ref[f, 5]

    for half in range(2):
        for q in range(2):
            r0 = half * H + q * Q
            for p in range(2):
                c0 = 256 * p
                left = quadrant(2 * half, q, p, rem[r0:r0 + Q, c0:c0 + 128])
                right = quadrant(2 * half + 1, q, p, rem[r0:r0 + Q, c0 + 128:c0 + 256])
                o_ref[pl.ds(r0, Q), pl.ds(col0 + c0, 256)] = jnp.concatenate(
                    [left, right], axis=1).astype(BF16)
            if after_rows is not None:
                after_rows(r0)


def _kernel(x_hbm, g_hbm, b_hbm, w_hbm, o_hbm,
            xbuf, obuf, gbuf, bbuf, wbuf, a_ref, ar_ref, e_ref,
            zb0, zr0, zb1, zr1, c_ref, sem_x0, sem_w, sem_x, sem_o):
    S = xbuf.shape[0]
    n_ramp = sum(RAMP)
    n_body = (S - 1 - n_ramp) // SPB

    def x0_copy(h):
        cols = pl.ds(GW * h, GW)
        return pltpu.make_async_copy(x_hbm.at[0, :, cols], xbuf.at[0, :, cols],
                                     sem_x0.at[h])

    def x_copy(s):
        return pltpu.make_async_copy(x_hbm.at[s], xbuf.at[s], sem_x.at[s])

    def o_part_start(s, h, r0, rows):
        sl = (s, pl.ds(r0, rows), pl.ds(GW * h, GW))
        pltpu.make_async_copy(obuf.at[sl], o_hbm.at[sl], sem_o).start()

    def o_start(s0, n):
        for c in range(2 * GW // 128):
            sl = (pl.ds(s0, n), slice(None), pl.ds(c * 128, 128))
            pltpu.make_async_copy(obuf.at[sl], o_hbm.at[sl], sem_o).start(priority=c % 2)

    w_copies = [pltpu.make_async_copy(g_hbm, gbuf, sem_w.at[0]),
                pltpu.make_async_copy(b_hbm, bbuf, sem_w.at[1]),
                pltpu.make_async_copy(w_hbm, wbuf, sem_w.at[2])]

    head = w_copies[::-1] + [x0_copy(0), x0_copy(1)]

    def issue_head(k, carry):
        for kk, cp in enumerate(head):
            pl.when(k == kk)(cp.start)
        return carry

    jax.lax.fori_loop(0, len(head), issue_head, 0)

    def issue_x(s, carry):
        x_copy(s).start()
        return carry

    jax.lax.fori_loop(1, S, issue_x, 0)

    row = jax.lax.broadcasted_iota(jnp.int32, (16, GW), 0)
    ones = jnp.where(row < 3, 1.0, 0.0).astype(BF16)
    zr0[KR:, :] = ones
    zr1[KR:, :] = ones

    for c in w_copies:
        c.wait()
    _prep_weights(gbuf, bbuf, wbuf, a_ref, ar_ref)
    x0_copy(0).wait()
    for item, _ in _norm_items(xbuf.at[0], 0, zb0, zr0):
        item(lambda v: v)
    x0_copy(1).wait()
    gv = jnp.broadcast_to(gbuf[...].astype(F32).reshape(1, D)[:, :128], (8, 128))
    gv2 = jnp.concatenate([gv, gv], axis=1)
    never = {128: gv != gv, 256: gv2 != gv2}

    def mm(k, *args):
        _mm_group(a_ref, ar_ref, e_ref.at[k % 2], -k % 4, *args)

    def ahead(i, h):
        return _Stats(xbuf.at[i], GW * h, save=c_ref.at[h]).items

    def block(i0, n, write):
        for u in range(n):
            i = i0 + u
            nxt = jnp.minimum(i + 1, S - 1)
            mm(2 * u, zb0, zr0, obuf.at[i], 0,
               _norm_items(xbuf.at[i], GW, zb1, zr1, c_ref.at[1]), ahead(nxt, 0), never)
            after_rows = None
            if write and u == n - 1:
                pl.when(i == S - 1)(functools.partial(o_part_start, i, 0, 0, D))

                def after_rows(r0, i=i):
                    pl.when(i == S - 1)(functools.partial(o_part_start, i, 1, r0, Q))
            mm(2 * u + 1, zb1, zr1, obuf.at[i], GW,
               _norm_items(xbuf.at[nxt], 0, zb0, zr0, c_ref.at[0]), ahead(nxt, 1),
               never, after_rows)
            if write:
                if (W_START - 2 - n_ramp) % SPB == u:
                    pl.when(i == W_START - 1)(functools.partial(o_start, 0, W_START))
                pl.when(jnp.logical_and(i >= W_START, i < S - 1))(
                    functools.partial(o_start, i, 1))

    mm(0, zb0, zr0, obuf.at[0], 0, _norm_items(xbuf.at[0], GW, zb1, zr1), [], never)
    x_copy(1).wait()
    mm(0, zb1, zr1, obuf.at[0], GW, _norm_items(xbuf.at[1], 0, zb0, zr0), ahead(1, 1),
       never)
    i = 1
    for n in RAMP:
        for u in range(n):
            x_copy(i + u + 1).wait()
        block(i, n, False)
        i += n

    def body(j, carry):
        i0 = 1 + n_ramp + j * SPB
        for u in range(SPB - 1):
            x_copy(i0 + u + 1).wait()
        pl.when(j < n_body - 1)(x_copy(jnp.minimum(i0 + SPB, S - 1)).wait)
        block(i0, SPB, True)
        return carry

    jax.lax.fori_loop(0, n_body, body, 0)
    pltpu.make_async_copy(obuf, o_hbm, sem_o).wait()


@jax.jit
def pallas_standalone__layernorm_linear__sampling_kernel(
    x: jax.Array,
    g: jax.Array,
    b: jax.Array,
    w: jax.Array,
):
    B, S, d = x.shape
    assert d == D and B == 2 * GW and (S - 1 - sum(RAMP)) % SPB == 0
    assert 1 + sum(RAMP) < W_START < S
    xt = jnp.transpose(x, (1, 2, 0))
    out = pl.pallas_call(
        _kernel,
        in_specs=[pl.BlockSpec(memory_space=pl.ANY)] * 4,
        out_specs=pl.BlockSpec(memory_space=pl.ANY),
        out_shape=jax.ShapeDtypeStruct((S, D, B), x.dtype),
        scratch_shapes=[
            pltpu.VMEM((S, D, B), BF16),
            pltpu.VMEM((S, D, B), BF16),
            pltpu.VMEM((D,), BF16),
            pltpu.VMEM((D,), BF16),
            pltpu.VMEM((D, D), BF16),
            pltpu.VMEM((25, Q // 2, 256), U32),
            pltpu.VMEM((D // 2, 128), U32),
            pltpu.VMEM((2, 4, 7, Q, 128), F32),
            pltpu.VMEM((25, 128, 256), BF16),
            pltpu.VMEM((KX, GW), BF16),
            pltpu.VMEM((25, 128, 256), BF16),
            pltpu.VMEM((KX, GW), BF16),
            pltpu.VMEM((2, 2, 8, 256), F32),
            pltpu.SemaphoreType.DMA((2,)),
            pltpu.SemaphoreType.DMA((3,)),
            pltpu.SemaphoreType.DMA((S,)),
            pltpu.SemaphoreType.DMA(()),
        ],
        compiler_params=pltpu.CompilerParams(
            vmem_limit_bytes=110 * 1024 * 1024,
            disable_bounds_checks=True,
            disable_semaphore_checks=True,
        ),
    )(xt, g, b, w)
    return jnp.transpose(out, (2, 0, 1))
```

```python
import functools

import jax
import jax.numpy as jnp
import jax.experimental.pallas as pl
import jax.experimental.pallas.tpu as pltpu

F32 = jnp.float32
BF16 = jnp.bfloat16
U32 = jnp.uint32

EPS = 1e-5
D = 576
H = D // 2
Q = H // 2
KH = 256
KR = D - 2 * KH
KX = KR + 16
GW = 512
RAMP = (1, 2)
SPB = 4
W_START = 14

TILE = {(t, u): 7 * i + u for i, t in enumerate((1, 4, 2, 5, 3, 6, 0))
        for u in range(7)}
HP = ((0, 0), (0, 1), (1, 0), (1, 1))
COEF = (((0, 1), (3, -1)), ((2, 1), (3, 1)), ((1, 1), (3, 1)), ((0, 1), (2, 1)),
        ((0, 1), (1, 1)), ((3, 1),), ((0, 1),))
PACE = dict(lag=48, split=400, stats=2.1, ops=1.7, extra=150, extra_room=0.7,
            tail=(170, 560))


def _pack(v):
    return pltpu.bitcast(v, U32)


def _unpack(v):
    return pltpu.bitcast(v, BF16)


def _a_ops(a11, a12, a21, a22):
    return [a11 + a22, a21 + a22, a11, a22, a11 + a12, a11 - a21, a12 - a22]


def _b_ops(b11, b12, b21, b22):
    return [b11 - b22, b11, b12 - b22, b21 - b11, b22, b11 - b12, b21 - b22]


def _rounds(early):
    rest = [(t, u) for u in range(7) for t in (6, 0, 5)]
    out = [rest[:early]] if early else []
    rest = [rest[i:i + 4] for i in range(early, len(rest), 4)]
    for u in range(7):
        out.append([(t, u) for t in (1, 2, 3, 4)])
        if rest and (len(rest[0]) == 4 or u == 6):
            out.append(rest.pop(0))
    return out


def _transpose(w):
    out = []
    for c0 in range(0, D, 128):
        n = min(128, D - c0)
        eye = (jax.lax.broadcasted_iota(jnp.int32, (n, n), 0)
               == jax.lax.broadcasted_iota(jnp.int32, (n, n), 1))
        eye = jnp.where(eye, 1.0, 0.0).astype(BF16)
        out.append(jax.lax.dot_general(eye, w[:, c0:c0 + n], (((1,), (1,)), ((), ())),
                                       preferred_element_type=F32))
    return jnp.concatenate(out, axis=0)


def _prep_weights(g_ref, b_ref, w_ref, a_ref, ar_ref):
    g = g_ref[...].astype(F32).reshape(1, D)
    row = jax.lax.broadcasted_iota(jnp.int32, (16, D), 0)
    bg = jnp.where(row < 8, b_ref[...].astype(F32).reshape(1, D), g).astype(BF16)
    cm = jnp.dot(bg, w_ref[...], preferred_element_type=F32)
    c = cm[0:1]
    c_hi = c.astype(BF16).astype(F32)
    rest = c - c_hi
    c_mid = rest.astype(BF16).astype(F32)
    c_lo = rest - c_mid
    mu = (cm[8:9] * (1.0 / D)).astype(BF16).astype(F32)
    ext = jnp.where(row == 0, c_hi,
                    jnp.where(row == 1, c_mid,
                              jnp.where(row == 2, c_lo,
                                        jnp.where(row == 15, mu, 0.0)))).astype(BF16)
    wr = _transpose(jnp.concatenate(
        [w_ref[2 * KH:, :], ext, jnp.zeros((128 - KX, D), BF16)], axis=0))
    mu = jnp.broadcast_to(wr[:, KX - 1:KX], (D, 128))
    lane = jax.lax.broadcasted_iota(jnp.int32, (1, 128), 1)
    gr = jnp.concatenate([g[:, 2 * KH:], jnp.ones((1, 128 - KR), F32)], axis=1)
    ar_ref[...] = _pack((wr * gr - jnp.where(lane < KR, mu, 0.0)).astype(BF16))
    mu = jnp.concatenate([mu, mu], axis=1)
    w1 = _transpose(w_ref[:KH, :]) * g[:, :KH] - mu
    w2 = _transpose(w_ref[KH:2 * KH, :]) * g[:, KH:2 * KH] - mu
    subs = []
    for a in _a_ops(w1[:H], w2[:H], w1[H:], w2[H:]):
        subs += _a_ops(a[:Q, :128], a[:Q, 128:], a[Q:, :128], a[Q:, 128:])
    for e in range(0, 48, 2):
        a_ref[e // 2] = _pack(
            jnp.concatenate([subs[e], subs[e + 1]], axis=1).astype(BF16))
    a_ref[24, :, :128] = _pack(subs[48].astype(BF16))


class _Stats:
    def __init__(self, x_ref, col0, save=None, load=None):
        self.x, self.cs, self.save = x_ref, pl.ds(col0, 256), save
        self.s1 = self.s2 = self.p = self.m = self.r = None
        self.items = []
        if load is not None:
            self.m, self.r = load[0], load[1]
        else:
            self.items = [(functools.partial(self.stat, r0, 32), 40)
                          for r0 in range(0, D, 32)]

    def stat(self, r0, rows, tie):
        if self.p is None:
            first = self.x[0:16, self.cs].astype(F32)[0:1, :]
            self.p = jnp.broadcast_to(first, (8, 256))
        p = tie(self.p)
        s1 = s2 = None
        for r in range(r0, r0 + rows, 8):
            d = self.x[r:r + 8, self.cs].astype(F32) - p
            s1 = d if s1 is None else s1 + d
            s2 = d * d if s2 is None else s2 + d * d
        self.s1 = s1 if self.s1 is None else self.s1 + s1
        self.s2 = s2 if self.s2 is None else self.s2 + s2
        if r0 + rows == D:
            e1 = jnp.sum(self.s1, axis=0, keepdims=True) * (1.0 / D)
            e2 = jnp.sum(self.s2, axis=0, keepdims=True) * (1.0 / D)
            var = jnp.maximum(e2 - e1 * e1, 0.0)
            self.m = self.p + e1
            self.r = jnp.broadcast_to(jax.lax.rsqrt(var + EPS), (8, 256))
            if self.save is not None:
                self.save[0] = self.m
                self.save[1] = self.r


def _tie(never, src, v):
    if v.shape[1] == 256:
        src = jnp.concatenate([src, src], axis=1)
    return jax.lax.select(never[v.shape[1]], src, v)


def _norm_items(x_ref, col0, zb, zr, stats0=None):
    st = [_Stats(x_ref, col0, load=stats0), _Stats(x_ref, col0 + 256)]
    held, pending = {}, {}

    def put(t, j, bt):
        for u, v in enumerate(_b_ops(*[bt[k] for k in HP])):
            e = TILE[(t, u)]
            if e == 48:
                zb[24, j:j + 8, :128] = v.astype(BF16)
            elif (e ^ 1, j) not in pending:
                pending[(e, j)] = v
            else:
                other = pending.pop((e ^ 1, j))
                pair = [v, other] if e % 2 == 0 else [other, v]
                zb[e // 2, j:j + 8, :] = jnp.concatenate(pair, axis=1).astype(BF16)

    def zblock(j, kq, side, tie):
        out = {}
        for p in range(2):
            ls = slice(128 * side, 128 * side + 128)
            m, r = tie(st[p].m[:, ls]), st[p].r[:, ls]
            for h in range(2):
                r0 = 128 * (kq + h) + j
                out[(h, p)] = (x_ref[r0:r0 + 8, st[p].cs].astype(F32)[:, ls] - m) * r
        return out

    def step1(j, tie):
        b11 = held[(j, 11)] = zblock(j, 0, 0, tie)
        put(1, j, b11)

    def step2(j, tie):
        b11, b22 = held[(j, 11)], zblock(j, 2, 1, tie)
        held[(j, 22)] = b22
        put(4, j, b22)
        put(0, j, {k: b11[k] - b22[k] for k in HP})

    def step3(j, tie):
        b11, b22, b12 = held[(j, 11)], held[(j, 22)], zblock(j, 0, 1, tie)
        put(2, j, {k: b12[k] - b22[k] for k in HP})
        put(5, j, {k: b11[k] - b12[k] for k in HP})

    def step4(j, tie):
        b11, b22, b21 = held[(j, 11)], held[(j, 22)], zblock(j, 2, 0, tie)
        put(3, j, {k: b21[k] - b11[k] for k in HP})
        put(6, j, {k: b21[k] - b22[k] for k in HP})

    def zrem(p, r0, tie):
        m = tie(st[p].m)
        xf = x_ref[2 * KH + r0:2 * KH + r0 + 32, st[p].cs].astype(F32)
        z = (xf.reshape(4, 8, 256) - m[None]) * st[p].r[None]
        zr[r0:r0 + 32, pl.ds(256 * p, 256)] = z.reshape(32, 256).astype(BF16)

    items = st[0].items + st[1].items
    items += [(functools.partial(zrem, 0, r0), 28) for r0 in range(0, KR, 32)]
    for j in range(0, 128, 8):
        items += [(functools.partial(step1, j), 20.5), (functools.partial(step2, j), 33),
                  (functools.partial(step3, j), 37), (functools.partial(step4, j), 37)]
    items += [(functools.partial(zrem, 1, r0), 28) for r0 in range(0, KR, 32)]
    return items


def _time_slots(items, tail, end):
    room = [0.0 if t < PACE["lag"] else
            PACE["stats"] if t < PACE["split"] else PACE["ops"]
            for t in range(0, end, 8)]
    room += [PACE["extra_room"]] * (PACE["extra"] // 8)
    scale = sum(room) / sum(cost for _, cost in items)
    pos, cum, acc, k = [], 0, 0.0, 0
    for _, cost in items:
        while acc + room[k] <= scale * cum + 1e-9:
            acc += room[k]
            k += 1
        pos.append(8 * k)
        cum += cost
    t0, t1 = PACE["tail"]
    return pos + [end + t0 + (t1 - t0) * k / len(tail) for k in range(len(tail))]


def _mm_group(a_ref, ar_ref, e_ref, early, zb, zr, o_ref, col0, items, tail, never,
              after_rows=None):
    rounds = _rounds(early)
    timed = [i == 0 or len(r) == 4 for i, r in enumerate(rounds)]
    pos = _time_slots(items, tail, Q * sum(timed))
    items = items + tail
    state = [0, 0]

    def release(mt):
        lo, span = state[1], mt.shape[0]
        while state[0] < len(items) and pos[state[0]] < lo + span:
            rr = min(span - 8, int(pos[state[0]] - lo) // 8 * 8)
            items[state[0]][0](functools.partial(_tie, never, mt[rr:rr + 8, :128]))
            state[0] += 1
        state[1] += span

    def prod(t, u):
        ea, eb = 7 * t + u, TILE[(t, u)]
        a = _unpack(a_ref[ea // 2, :, pl.ds(128 * (ea % 2), 128)])
        return jnp.dot(a, zb[eb // 2, :, pl.ds(128 * (eb % 2), 128)],
                       preferred_element_type=F32)

    stored = {}
    for rnd, is_timed in zip(rounds, timed):
        ps = [prod(t, u) for t, u in rnd]
        terms = {}
        for (t, u), p in zip(rnd, ps):
            for f, sign in COEF[t]:
                terms.setdefault((f, u), []).append((sign, p))
        for (f, u), tm in terms.items():
            if (f, u) in stored:
                tm.append((stored[(f, u)], e_ref[f, u]))
            plus = [p for sign, p in tm if sign > 0]
            minus = [p for sign, p in tm if sign < 0]
            stored[(f, u)] = 1 if plus else -1
            val = functools.reduce(jnp.add, plus or minus)
            e_ref[f, u] = functools.reduce(jnp.subtract, minus, val) if plus else val
        if is_timed:
            release(ps[0])
    assert min(stored.values()) > 0
    rem = jnp.dot(_unpack(ar_ref[...])[:, :KX], zr[...], preferred_element_type=F32)
    release(rem)
    assert state[0] == len(items)

    def quadrant(f, q, p, base):
        if (q, p) == (0, 0):
            return base + e_ref[f, 0] + e_ref[f, 3] + e_ref[f, 4] + e_ref[f, 6]
        if (q, p) == (0, 1):
            return base + e_ref[f, 2] + e_ref[f, 4]
        if (q, p) == (1, 0):
            return base + e_ref[f, 1] + e_ref[f, 3]
        return base - e_ref[f, 0] + e_ref[f, 1] + e_ref[f, 2] + e_ref[f, 5]

    for half in range(2):
        for q in range(2):
            r0 = half * H + q * Q
            for p in range(2):
                c0 = 256 * p
                left = quadrant(2 * half, q, p, rem[r0:r0 + Q, c0:c0 + 128])
                right = quadrant(2 * half + 1, q, p, rem[r0:r0 + Q, c0 + 128:c0 + 256])
                o_ref[pl.ds(r0, Q), pl.ds(col0 + c0, 256)] = jnp.concatenate(
                    [left, right], axis=1).astype(BF16)
            if after_rows is not None:
                after_rows(r0)


def _kernel(x_hbm, g_hbm, b_hbm, w_hbm, o_hbm,
            xbuf, obuf, gbuf, bbuf, wbuf, a_ref, ar_ref, e_ref,
            zb0, zr0, zb1, zr1, c_ref, sem_x0, sem_w, sem_x, sem_o):
    S = xbuf.shape[0]
    n_ramp = sum(RAMP)
    n_body = (S - 1 - n_ramp) // SPB

    def x0_copy(h):
        cols = pl.ds(GW * h, GW)
        return pltpu.make_async_copy(x_hbm.at[0, :, cols], xbuf.at[0, :, cols],
                                     sem_x0.at[h])

    def x_copy(s):
        return pltpu.make_async_copy(x_hbm.at[s], xbuf.at[s], sem_x.at[s])

    def o_part_start(s, h, r0, rows):
        sl = (s, pl.ds(r0, rows), pl.ds(GW * h, GW))
        pltpu.make_async_copy(obuf.at[sl], o_hbm.at[sl], sem_o).start()

    def o_start(s0, n):
        for c in range(2 * GW // 128):
            sl = (pl.ds(s0, n), slice(None), pl.ds(c * 128, 128))
            pltpu.make_async_copy(obuf.at[sl], o_hbm.at[sl], sem_o).start(priority=c % 2)

    w_copies = [pltpu.make_async_copy(g_hbm, gbuf, sem_w.at[0]),
                pltpu.make_async_copy(b_hbm, bbuf, sem_w.at[1]),
                pltpu.make_async_copy(w_hbm, wbuf, sem_w.at[2])]

    head = w_copies[::-1] + [x0_copy(0), x0_copy(1)]

    def issue_head(k, carry):
        for kk, cp in enumerate(head):
            pl.when(k == kk)(cp.start)
        return carry

    jax.lax.fori_loop(0, len(head), issue_head, 0)

    def issue_x(s, carry):
        x_copy(s).start()
        return carry

    jax.lax.fori_loop(1, S, issue_x, 0)

    row = jax.lax.broadcasted_iota(jnp.int32, (16, GW), 0)
    ones = jnp.where(row < 3, 1.0, 0.0).astype(BF16)
    zr0[KR:, :] = ones
    zr1[KR:, :] = ones

    for c in w_copies:
        c.wait()
    _prep_weights(gbuf, bbuf, wbuf, a_ref, ar_ref)
    x0_copy(0).wait()
    for item, _ in _norm_items(xbuf.at[0], 0, zb0, zr0):
        item(lambda v: v)
    x0_copy(1).wait()
    gv = jnp.broadcast_to(gbuf[...].astype(F32).reshape(1, D)[:, :128], (8, 128))
    gv2 = jnp.concatenate([gv, gv], axis=1)
    never = {128: gv != gv, 256: gv2 != gv2}

    def mm(k, *args):
        _mm_group(a_ref, ar_ref, e_ref.at[k % 2], -k % 4, *args)

    def ahead(i, h):
        return _Stats(xbuf.at[i], GW * h, save=c_ref.at[h]).items

    def block(i0, n, write):
        for u in range(n):
            i = i0 + u
            nxt = jnp.minimum(i + 1, S - 1)
            mm(2 * u, zb0, zr0, obuf.at[i], 0,
               _norm_items(xbuf.at[i], GW, zb1, zr1, c_ref.at[1]), ahead(nxt, 0), never)
            after_rows = None
            if write and u == n - 1:
                pl.when(i == S - 1)(functools.partial(o_part_start, i, 0, 0, D))

                def after_rows(r0, i=i):
                    pl.when(i == S - 1)(functools.partial(o_part_start, i, 1, r0, Q))
            mm(2 * u + 1, zb1, zr1, obuf.at[i], GW,
               _norm_items(xbuf.at[nxt], 0, zb0, zr0, c_ref.at[0]), ahead(nxt, 1),
               never, after_rows)
            if write:
                if (W_START - 2 - n_ramp) % SPB == u:
                    pl.when(i == W_START - 1)(functools.partial(o_start, 0, W_START))
                pl.when(jnp.logical_and(i >= W_START, i < S - 1))(
                    functools.partial(o_start, i, 1))

    mm(0, zb0, zr0, obuf.at[0], 0, _norm_items(xbuf.at[0], GW, zb1, zr1), [], never)
    x_copy(1).wait()
    mm(0, zb1, zr1, obuf.at[0], GW, _norm_items(xbuf.at[1], 0, zb0, zr0), ahead(1, 1),
       never)
    i = 1
    for n in RAMP:
        for u in range(n):
            x_copy(i + u + 1).wait()
        block(i, n, False)
        i += n

    def body(j, carry):
        i0 = 1 + n_ramp + j * SPB
        for u in range(SPB - 1):
            x_copy(i0 + u + 1).wait()
        pl.when(j < n_body - 1)(x_copy(jnp.minimum(i0 + SPB, S - 1)).wait)
        block(i0, SPB, True)
        return carry

    jax.lax.fori_loop(0, n_body, body, 0)
    pltpu.make_async_copy(obuf, o_hbm, sem_o).wait()


@jax.jit
def pallas_standalone__layernorm_linear__sampling_kernel(
    x: jax.Array,
    g: jax.Array,
    b: jax.Array,
    w: jax.Array,
):
    B, S, d = x.shape
    assert d == D and B == 2 * GW and (S - 1 - sum(RAMP)) % SPB == 0
    assert 1 + sum(RAMP) < W_START < S
    xt = jnp.transpose(x, (1, 2, 0))
    out = pl.pallas_call(
        _kernel,
        in_specs=[pl.BlockSpec(memory_space=pl.ANY)] * 4,
        out_specs=pl.BlockSpec(memory_space=pl.ANY),
        out_shape=jax.ShapeDtypeStruct((S, D, B), x.dtype),
        scratch_shapes=[
            pltpu.VMEM((S, D, B), BF16),
            pltpu.VMEM((S, D, B), BF16),
            pltpu.VMEM((D,), BF16),
            pltpu.VMEM((D,), BF16),
            pltpu.VMEM((D, D), BF16),
            pltpu.VMEM((25, Q // 2, 256), U32),
            pltpu.VMEM((D // 2, 128), U32),
            pltpu.VMEM((2, 4, 7, Q, 128), F32),
            pltpu.VMEM((25, 128, 256), BF16),
            pltpu.VMEM((KX, GW), BF16),
            pltpu.VMEM((25, 128, 256), BF16),
            pltpu.VMEM((KX, GW), BF16),
            pltpu.VMEM((2, 2, 8, 256), F32),
            pltpu.SemaphoreType.DMA((2,)),
            pltpu.SemaphoreType.DMA((3,)),
            pltpu.SemaphoreType.DMA((S,)),
            pltpu.SemaphoreType.DMA(()),
        ],
        compiler_params=pltpu.CompilerParams(
            vmem_limit_bytes=110 * 1024 * 1024,
            disable_bounds_checks=True,
            disable_semaphore_checks=True,
        ),
    )(xt, g, b, w)
    return jnp.transpose(out, (2, 0, 1))
```

```python
import functools

import jax
import jax.numpy as jnp
import jax.experimental.pallas as pl
import jax.experimental.pallas.tpu as pltpu

F32 = jnp.float32
BF16 = jnp.bfloat16
U32 = jnp.uint32

EPS = 1e-5
D = 576
H = D // 2
Q = H // 2
KH = 256
KR = D - 2 * KH
KX = KR + 16
GW = 512
RAMP = (1, 2)
SPB = 4
W_START = 14

TILE = {(t, u): 7 * i + u for i, t in enumerate((1, 4, 2, 5, 3, 6, 0))
        for u in range(7)}
HP = ((0, 0), (0, 1), (1, 0), (1, 1))
COEF = (((0, 1), (3, -1)), ((2, 1), (3, 1)), ((1, 1), (3, 1)), ((0, 1), (2, 1)),
        ((0, 1), (1, 1)), ((3, 1),), ((0, 1),))
PACE = dict(lag=48, split=400, stats=2.1, ops=1.6, extra=150, extra_room=0.7,
            tail=(170, 560))


def _pack(v):
    return pltpu.bitcast(v, U32)


def _unpack(v):
    return pltpu.bitcast(v, BF16)


def _a_ops(a11, a12, a21, a22):
    return [a11 + a22, a21 + a22, a11, a22, a11 + a12, a11 - a21, a12 - a22]


def _b_ops(b11, b12, b21, b22):
    return [b11 - b22, b11, b12 - b22, b21 - b11, b22, b11 - b12, b21 - b22]


def _rounds(early):
    rest = [(t, u) for u in range(7) for t in (6, 0, 5)]
    out = [rest[:early]] if early else []
    rest = [rest[i:i + 4] for i in range(early, len(rest), 4)]
    for u in range(7):
        out.append([(t, u) for t in (1, 2, 3, 4)])
        if rest and (len(rest[0]) == 4 or u == 6):
            out.append(rest.pop(0))
    return out


def _transpose(w):
    out = []
    for c0 in range(0, D, 128):
        n = min(128, D - c0)
        eye = (jax.lax.broadcasted_iota(jnp.int32, (n, n), 0)
               == jax.lax.broadcasted_iota(jnp.int32, (n, n), 1))
        eye = jnp.where(eye, 1.0, 0.0).astype(BF16)
        out.append(jax.lax.dot_general(eye, w[:, c0:c0 + n], (((1,), (1,)), ((), ())),
                                       preferred_element_type=F32))
    return jnp.concatenate(out, axis=0)


def _prep_weights(g_ref, b_ref, w_ref, a_ref, ar_ref):
    g = g_ref[...].astype(F32).reshape(1, D)
    row = jax.lax.broadcasted_iota(jnp.int32, (16, D), 0)
    bg = jnp.where(row < 8, b_ref[...].astype(F32).reshape(1, D), g).astype(BF16)
    cm = jnp.dot(bg, w_ref[...], preferred_element_type=F32)
    c = cm[0:1]
    c_hi = c.astype(BF16).astype(F32)
    rest = c - c_hi
    c_mid = rest.astype(BF16).astype(F32)
    c_lo = rest - c_mid
    mu = (cm[8:9] * (1.0 / D)).astype(BF16).astype(F32)
    ext = jnp.where(row == 0, c_hi,
                    jnp.where(row == 1, c_mid,
                              jnp.where(row == 2, c_lo,
                                        jnp.where(row == 15, mu, 0.0)))).astype(BF16)
    wr = _transpose(jnp.concatenate(
        [w_ref[2 * KH:, :], ext, jnp.zeros((128 - KX, D), BF16)], axis=0))
    mu = jnp.broadcast_to(wr[:, KX - 1:KX], (D, 128))
    lane = jax.lax.broadcasted_iota(jnp.int32, (1, 128), 1)
    gr = jnp.concatenate([g[:, 2 * KH:], jnp.ones((1, 128 - KR), F32)], axis=1)
    ar_ref[...] = _pack((wr * gr - jnp.where(lane < KR, mu, 0.0)).astype(BF16))
    mu = jnp.concatenate([mu, mu], axis=1)
    w1 = _transpose(w_ref[:KH, :]) * g[:, :KH] - mu
    w2 = _transpose(w_ref[KH:2 * KH, :]) * g[:, KH:2 * KH] - mu
    subs = []
    for a in _a_ops(w1[:H], w2[:H], w1[H:], w2[H:]):
        subs += _a_ops(a[:Q, :128], a[:Q, 128:], a[Q:, :128], a[Q:, 128:])
    for e in range(0, 48, 2):
        a_ref[e // 2] = _pack(
            jnp.concatenate([subs[e], subs[e + 1]], axis=1).astype(BF16))
    a_ref[24, :, :128] = _pack(subs[48].astype(BF16))


class _Stats:
    def __init__(self, x_ref, col0, save=None, load=None):
        self.x, self.cs, self.save = x_ref, pl.ds(col0, 256), save
        self.s1 = self.s2 = self.p = self.m = self.r = None
        self.items = []
        if load is not None:
            self.m, self.r = load[0], load[1]
        else:
            self.items = [(functools.partial(self.stat, r0, 32), 40)
                          for r0 in range(0, D, 32)]

    def stat(self, r0, rows, tie):
        if self.p is None:
            first = self.x[0:16, self.cs].astype(F32)[0:1, :]
            self.p = jnp.broadcast_to(first, (8, 256))
        p = tie(self.p)
        s1 = s2 = None
        for r in range(r0, r0 + rows, 8):
            d = self.x[r:r + 8, self.cs].astype(F32) - p
            s1 = d if s1 is None else s1 + d
            s2 = d * d if s2 is None else s2 + d * d
        self.s1 = s1 if self.s1 is None else self.s1 + s1
        self.s2 = s2 if self.s2 is None else self.s2 + s2
        if r0 + rows == D:
            e1 = jnp.sum(self.s1, axis=0, keepdims=True) * (1.0 / D)
            e2 = jnp.sum(self.s2, axis=0, keepdims=True) * (1.0 / D)
            var = jnp.maximum(e2 - e1 * e1, 0.0)
            self.m = self.p + e1
            self.r = jnp.broadcast_to(jax.lax.rsqrt(var + EPS), (8, 256))
            if self.save is not None:
                self.save[0] = self.m
                self.save[1] = self.r


def _tie(never, src, v):
    if v.shape[1] == 256:
        src = jnp.concatenate([src, src], axis=1)
    return jax.lax.select(never[v.shape[1]], src, v)


def _norm_items(x_ref, col0, zb, zr, stats0=None):
    st = [_Stats(x_ref, col0, load=stats0), _Stats(x_ref, col0 + 256)]
    held, pending = {}, {}

    def put(t, j, bt):
        for u, v in enumerate(_b_ops(*[bt[k] for k in HP])):
            e = TILE[(t, u)]
            if e == 48:
                zb[24, j:j + 8, :128] = v.astype(BF16)
            elif (e ^ 1, j) not in pending:
                pending[(e, j)] = v
            else:
                other = pending.pop((e ^ 1, j))
                pair = [v, other] if e % 2 == 0 else [other, v]
                zb[e // 2, j:j + 8, :] = jnp.concatenate(pair, axis=1).astype(BF16)

    def zblock(j, kq, side, tie):
        out = {}
        for p in range(2):
            ls = slice(128 * side, 128 * side + 128)
            m, r = st[p].m[:, ls], st[p].r[:, ls]
            if p == 0:
                m = tie(m)
            for h in range(2):
                r0 = 128 * (kq + h) + j
                out[(h, p)] = (x_ref[r0:r0 + 8, st[p].cs].astype(F32)[:, ls] - m) * r
        return out

    def step1(j, tie):
        b11 = held[(j, 11)] = zblock(j, 0, 0, tie)
        put(1, j, b11)

    def step2(j, tie):
        b11, b22 = held[(j, 11)], zblock(j, 2, 1, tie)
        held[(j, 22)] = b22
        put(4, j, b22)
        put(0, j, {k: b11[k] - b22[k] for k in HP})

    def step3(j, tie):
        b11, b22, b12 = held[(j, 11)], held[(j, 22)], zblock(j, 0, 1, tie)
        put(2, j, {k: b12[k] - b22[k] for k in HP})
        put(5, j, {k: b11[k] - b12[k] for k in HP})

    def step4(j, tie):
        b11, b22, b21 = held[(j, 11)], held[(j, 22)], zblock(j, 2, 0, tie)
        put(3, j, {k: b21[k] - b11[k] for k in HP})
        put(6, j, {k: b21[k] - b22[k] for k in HP})

    def zrem(p, r0, tie):
        m = tie(st[p].m)
        xf = x_ref[2 * KH + r0:2 * KH + r0 + 32, st[p].cs].astype(F32)
        z = (xf.reshape(4, 8, 256) - m[None]) * st[p].r[None]
        zr[r0:r0 + 32, pl.ds(256 * p, 256)] = z.reshape(32, 256).astype(BF16)

    items = st[0].items + st[1].items
    items += [(functools.partial(zrem, 0, r0), 28) for r0 in range(0, KR, 32)]
    for j in range(0, 128, 8):
        items += [(functools.partial(step1, j), 20.5), (functools.partial(step2, j), 33),
                  (functools.partial(step3, j), 37), (functools.partial(step4, j), 37)]
    items += [(functools.partial(zrem, 1, r0), 28) for r0 in range(0, KR, 32)]
    return items


def _time_slots(items, tail, end):
    room = [0.0 if t < PACE["lag"] else
            PACE["stats"] if t < PACE["split"] else PACE["ops"]
            for t in range(0, end, 8)]
    room += [PACE["extra_room"]] * (PACE["extra"] // 8)
    scale = sum(room) / sum(cost for _, cost in items)
    pos, cum, acc, k = [], 0, 0.0, 0
    for _, cost in items:
        while acc + room[k] <= scale * cum + 1e-9:
            acc += room[k]
            k += 1
        pos.append(8 * k)
        cum += cost
    t0, t1 = PACE["tail"]
    return pos + [end + t0 + (t1 - t0) * k / len(tail) for k in range(len(tail))]


def _mm_group(a_ref, ar_ref, e_ref, early, zb, zr, o_ref, col0, items, tail, never,
              after_rows=None):
    rounds = _rounds(early)
    timed = [i == 0 or len(r) == 4 for i, r in enumerate(rounds)]
    pos = _time_slots(items, tail, Q * sum(timed))
    items = items + tail
    state = [0, 0]

    def release(mt):
        lo, span = state[1], mt.shape[0]
        while state[0] < len(items) and pos[state[0]] < lo + span:
            rr = min(span - 8, int(pos[state[0]] - lo) // 8 * 8)
            items[state[0]][0](functools.partial(_tie, never, mt[rr:rr + 8, :128]))
            state[0] += 1
        state[1] += span

    def prod(t, u):
        ea, eb = 7 * t + u, TILE[(t, u)]
        a = _unpack(a_ref[ea // 2, :, pl.ds(128 * (ea % 2), 128)])
        return jnp.dot(a, zb[eb // 2, :, pl.ds(128 * (eb % 2), 128)],
                       preferred_element_type=F32)

    stored = {}
    for rnd, is_timed in zip(rounds, timed):
        ps = [prod(t, u) for t, u in rnd]
        terms = {}
        for (t, u), p in zip(rnd, ps):
            for f, sign in COEF[t]:
                terms.setdefault((f, u), []).append((sign, p))
        for (f, u), tm in terms.items():
            if (f, u) in stored:
                tm.append((stored[(f, u)], e_ref[f, u]))
            plus = [p for sign, p in tm if sign > 0]
            minus = [p for sign, p in tm if sign < 0]
            stored[(f, u)] = 1 if plus else -1
            val = functools.reduce(jnp.add, plus or minus)
            e_ref[f, u] = functools.reduce(jnp.subtract, minus, val) if plus else val
        if is_timed:
            release(ps[0])
    assert min(stored.values()) > 0
    rem = jnp.dot(_unpack(ar_ref[...])[:, :KX], zr[...], preferred_element_type=F32)
    release(rem)
    assert state[0] == len(items)

    def quadrant(f, q, p, base):
        if (q, p) == (0, 0):
            return base + e_ref[f, 0] + e_ref[f, 3] + e_ref[f, 4] + e_ref[f, 6]
        if (q, p) == (0, 1):
            return base + e_ref[f, 2] + e_ref[f, 4]
        if (q, p) == (1, 0):
            return base + e_ref[f, 1] + e_ref[f, 3]
        return base - e_ref[f, 0] + e_ref[f, 1] + e_ref[f, 2] + e_ref[f, 5]

    for half in range(2):
        for q in range(2):
            r0 = half * H + q * Q
            for p in range(2):
                c0 = 256 * p
                left = quadrant(2 * half, q, p, rem[r0:r0 + Q, c0:c0 + 128])
                right = quadrant(2 * half + 1, q, p, rem[r0:r0 + Q, c0 + 128:c0 + 256])
                o_ref[pl.ds(r0, Q), pl.ds(col0 + c0, 256)] = jnp.concatenate(
                    [left, right], axis=1).astype(BF16)
            if after_rows is not None:
                after_rows(r0)


def _kernel(x_hbm, g_hbm, b_hbm, w_hbm, o_hbm,
            xbuf, obuf, gbuf, bbuf, wbuf, a_ref, ar_ref, e_ref,
            zb0, zr0, zb1, zr1, c_ref, sem_x0, sem_w, sem_x, sem_o):
    S = xbuf.shape[0]
    n_ramp = sum(RAMP)
    n_body = (S - 1 - n_ramp) // SPB

    def x0_copy(h):
        cols = pl.ds(GW * h, GW)
        return pltpu.make_async_copy(x_hbm.at[0, :, cols], xbuf.at[0, :, cols],
                                     sem_x0.at[h])

    def x_copy(s):
        return pltpu.make_async_copy(x_hbm.at[s], xbuf.at[s], sem_x.at[s])

    def o_part_start(s, h, r0, rows):
        sl = (s, pl.ds(r0, rows), pl.ds(GW * h, GW))
        pltpu.make_async_copy(obuf.at[sl], o_hbm.at[sl], sem_o).start()

    def o_start(s0, n):
        for c in range(2 * GW // 128):
            sl = (pl.ds(s0, n), slice(None), pl.ds(c * 128, 128))
            pltpu.make_async_copy(obuf.at[sl], o_hbm.at[sl], sem_o).start(priority=c % 2)

    w_copies = [pltpu.make_async_copy(g_hbm, gbuf, sem_w.at[0]),
                pltpu.make_async_copy(b_hbm, bbuf, sem_w.at[1]),
                pltpu.make_async_copy(w_hbm, wbuf, sem_w.at[2])]

    head = w_copies[::-1] + [x0_copy(0), x0_copy(1)]

    def issue_head(k, carry):
        for kk, cp in enumerate(head):
            pl.when(k == kk)(cp.start)
        return carry

    jax.lax.fori_loop(0, len(head), issue_head, 0)

    def issue_x(s, carry):
        x_copy(s).start()
        return carry

    jax.lax.fori_loop(1, S, issue_x, 0)

    row = jax.lax.broadcasted_iota(jnp.int32, (16, GW), 0)
    ones = jnp.where(row < 3, 1.0, 0.0).astype(BF16)
    zr0[KR:, :] = ones
    zr1[KR:, :] = ones

    for c in w_copies:
        c.wait()
    _prep_weights(gbuf, bbuf, wbuf, a_ref, ar_ref)
    x0_copy(0).wait()
    for item, _ in _norm_items(xbuf.at[0], 0, zb0, zr0):
        item(lambda v: v)
    x0_copy(1).wait()
    gv = jnp.broadcast_to(gbuf[...].astype(F32).reshape(1, D)[:, :128], (8, 128))
    gv2 = jnp.concatenate([gv, gv], axis=1)
    never = {128: gv != gv, 256: gv2 != gv2}

    def mm(k, *args):
        _mm_group(a_ref, ar_ref, e_ref.at[k % 2], -k % 4, *args)

    def ahead(i, h):
        return _Stats(xbuf.at[i], GW * h, save=c_ref.at[h]).items

    def block(i0, n, write):
        for u in range(n):
            i = i0 + u
            nxt = jnp.minimum(i + 1, S - 1)
            mm(2 * u, zb0, zr0, obuf.at[i], 0,
               _norm_items(xbuf.at[i], GW, zb1, zr1, c_ref.at[1]), ahead(nxt, 0), never)
            after_rows = None
            if write and u == n - 1:
                pl.when(i == S - 1)(functools.partial(o_part_start, i, 0, 0, D))

                def after_rows(r0, i=i):
                    pl.when(i == S - 1)(functools.partial(o_part_start, i, 1, r0, Q))
            mm(2 * u + 1, zb1, zr1, obuf.at[i], GW,
               _norm_items(xbuf.at[nxt], 0, zb0, zr0, c_ref.at[0]), ahead(nxt, 1),
               never, after_rows)
            if write:
                if (W_START - 2 - n_ramp) % SPB == u:
                    pl.when(i == W_START - 1)(functools.partial(o_start, 0, W_START))
                pl.when(jnp.logical_and(i >= W_START, i < S - 1))(
                    functools.partial(o_start, i, 1))

    mm(0, zb0, zr0, obuf.at[0], 0, _norm_items(xbuf.at[0], GW, zb1, zr1), [], never)
    x_copy(1).wait()
    mm(0, zb1, zr1, obuf.at[0], GW, _norm_items(xbuf.at[1], 0, zb0, zr0), ahead(1, 1),
       never)
    i = 1
    for n in RAMP:
        for u in range(n):
            x_copy(i + u + 1).wait()
        block(i, n, False)
        i += n

    def body(j, carry):
        i0 = 1 + n_ramp + j * SPB
        for u in range(SPB - 1):
            x_copy(i0 + u + 1).wait()
        pl.when(j < n_body - 1)(x_copy(jnp.minimum(i0 + SPB, S - 1)).wait)
        block(i0, SPB, True)
        return carry

    jax.lax.fori_loop(0, n_body, body, 0)
    pltpu.make_async_copy(obuf, o_hbm, sem_o).wait()


@jax.jit
def pallas_standalone__layernorm_linear__sampling_kernel(
    x: jax.Array,
    g: jax.Array,
    b: jax.Array,
    w: jax.Array,
):
    B, S, d = x.shape
    assert d == D and B == 2 * GW and (S - 1 - sum(RAMP)) % SPB == 0
    assert 1 + sum(RAMP) < W_START < S
    xt = jnp.transpose(x, (1, 2, 0))
    out = pl.pallas_call(
        _kernel,
        in_specs=[pl.BlockSpec(memory_space=pl.ANY)] * 4,
        out_specs=pl.BlockSpec(memory_space=pl.ANY),
        out_shape=jax.ShapeDtypeStruct((S, D, B), x.dtype),
        scratch_shapes=[
            pltpu.VMEM((S, D, B), BF16),
            pltpu.VMEM((S, D, B), BF16),
            pltpu.VMEM((D,), BF16),
            pltpu.VMEM((D,), BF16),
            pltpu.VMEM((D, D), BF16),
            pltpu.VMEM((25, Q // 2, 256), U32),
            pltpu.VMEM((D // 2, 128), U32),
            pltpu.VMEM((2, 4, 7, Q, 128), F32),
            pltpu.VMEM((25, 128, 256), BF16),
            pltpu.VMEM((KX, GW), BF16),
            pltpu.VMEM((25, 128, 256), BF16),
            pltpu.VMEM((KX, GW), BF16),
            pltpu.VMEM((2, 2, 8, 256), F32),
            pltpu.SemaphoreType.DMA((2,)),
            pltpu.SemaphoreType.DMA((3,)),
            pltpu.SemaphoreType.DMA((S,)),
            pltpu.SemaphoreType.DMA(()),
        ],
        compiler_params=pltpu.CompilerParams(
            vmem_limit_bytes=110 * 1024 * 1024,
            disable_bounds_checks=True,
            disable_semaphore_checks=True,
        ),
    )(xt, g, b, w)
    return jnp.transpose(out, (2, 0, 1))
```

```python
import functools

import jax
import jax.numpy as jnp
import jax.experimental.pallas as pl
import jax.experimental.pallas.tpu as pltpu

F32 = jnp.float32
BF16 = jnp.bfloat16
U32 = jnp.uint32

EPS = 1e-5
D = 576
H = D // 2
Q = H // 2
KH = 256
KR = D - 2 * KH
KX = KR + 16
GW = 512
RAMP = (1, 2)
SPB = 4
W_START = 14

TILE = {(t, u): 7 * i + u for i, t in enumerate((1, 4, 2, 5, 3, 6, 0))
        for u in range(7)}
HP = ((0, 0), (0, 1), (1, 0), (1, 1))
COEF = (((0, 1), (3, -1)), ((2, 1), (3, 1)), ((1, 1), (3, 1)), ((0, 1), (2, 1)),
        ((0, 1), (1, 1)), ((3, 1),), ((0, 1),))
PACE = dict(lag=48, split=400, stats=2.1, ops=1.6, extra=150, extra_room=0.7,
            tail=(170, 560))


def _pack(v):
    return pltpu.bitcast(v, U32)


def _unpack(v):
    return pltpu.bitcast(v, BF16)


def _a_ops(a11, a12, a21, a22):
    return [a11 + a22, a21 + a22, a11, a22, a11 + a12, a11 - a21, a12 - a22]


def _b_ops(b11, b12, b21, b22):
    return [b11 - b22, b11, b12 - b22, b21 - b11, b22, b11 - b12, b21 - b22]


def _rounds(early):
    rest = [(t, u) for u in range(7) for t in (6, 0, 5)]
    out = [rest[:early]] if early else []
    rest = [rest[i:i + 4] for i in range(early, len(rest), 4)]
    for u in range(7):
        out.append([(t, u) for t in (1, 2, 3, 4)])
        if rest and (len(rest[0]) == 4 or u == 6):
            out.append(rest.pop(0))
    return out


def _transpose(w):
    out = []
    for c0 in range(0, D, 128):
        n = min(128, D - c0)
        eye = (jax.lax.broadcasted_iota(jnp.int32, (n, n), 0)
               == jax.lax.broadcasted_iota(jnp.int32, (n, n), 1))
        eye = jnp.where(eye, 1.0, 0.0).astype(BF16)
        out.append(jax.lax.dot_general(eye, w[:, c0:c0 + n], (((1,), (1,)), ((), ())),
                                       preferred_element_type=F32))
    return jnp.concatenate(out, axis=0)


def _prep_weights(g_ref, b_ref, w_ref, a_ref, ar_ref):
    g = g_ref[...].astype(F32).reshape(1, D)
    row = jax.lax.broadcasted_iota(jnp.int32, (16, D), 0)
    bg = jnp.where(row < 8, b_ref[...].astype(F32).reshape(1, D), g).astype(BF16)
    cm = jnp.dot(bg, w_ref[...], preferred_element_type=F32)
    c = cm[0:1]
    c_hi = c.astype(BF16).astype(F32)
    rest = c - c_hi
    c_mid = rest.astype(BF16).astype(F32)
    c_lo = rest - c_mid
    mu = (cm[8:9] * (1.0 / D)).astype(BF16).astype(F32)
    ext = jnp.where(row == 0, c_hi,
                    jnp.where(row == 1, c_mid,
                              jnp.where(row == 2, c_lo,
                                        jnp.where(row == 15, mu, 0.0)))).astype(BF16)
    wr = _transpose(jnp.concatenate(
        [w_ref[2 * KH:, :], ext, jnp.zeros((128 - KX, D), BF16)], axis=0))
    mu = jnp.broadcast_to(wr[:, KX - 1:KX], (D, 128))
    lane = jax.lax.broadcasted_iota(jnp.int32, (1, 128), 1)
    gr = jnp.concatenate([g[:, 2 * KH:], jnp.ones((1, 128 - KR), F32)], axis=1)
    ar_ref[...] = _pack((wr * gr - jnp.where(lane < KR, mu, 0.0)).astype(BF16))
    mu = jnp.concatenate([mu, mu], axis=1)
    w1 = _transpose(w_ref[:KH, :]) * g[:, :KH] - mu
    w2 = _transpose(w_ref[KH:2 * KH, :]) * g[:, KH:2 * KH] - mu
    subs = []
    for a in _a_ops(w1[:H], w2[:H], w1[H:], w2[H:]):
        subs += _a_ops(a[:Q, :128], a[:Q, 128:], a[Q:, :128], a[Q:, 128:])
    for e in range(0, 48, 2):
        a_ref[e // 2] = _pack(
            jnp.concatenate([subs[e], subs[e + 1]], axis=1).astype(BF16))
    a_ref[24, :, :128] = _pack(subs[48].astype(BF16))


class _Stats:
    def __init__(self, x_ref, col0, save=None, load=None):
        self.x, self.cs, self.save = x_ref, pl.ds(col0, 256), save
        self.s1 = self.s2 = self.p = self.m = self.r = None
        self.items = []
        if load is not None:
            self.m, self.r = load[0], load[1]
        else:
            self.items = [(functools.partial(self.stat, r0, 32), 40)
                          for r0 in range(0, D, 32)]

    def stat(self, r0, rows, tie):
        if self.p is None:
            first = self.x[0:16, self.cs].astype(F32)[0:1, :]
            self.p = jnp.broadcast_to(first, (8, 256))
        p = tie(self.p)
        s1 = s2 = None
        for r in range(r0, r0 + rows, 8):
            d = self.x[r:r + 8, self.cs].astype(F32) - p
            s1 = d if s1 is None else s1 + d
            s2 = d * d if s2 is None else s2 + d * d
        self.s1 = s1 if self.s1 is None else self.s1 + s1
        self.s2 = s2 if self.s2 is None else self.s2 + s2
        if r0 + rows == D:
            e1 = jnp.sum(self.s1, axis=0, keepdims=True) * (1.0 / D)
            e2 = jnp.sum(self.s2, axis=0, keepdims=True) * (1.0 / D)
            var = jnp.maximum(e2 - e1 * e1, 0.0)
            self.m = self.p + e1
            self.r = jnp.broadcast_to(jax.lax.rsqrt(var + EPS), (8, 256))
            if self.save is not None:
                self.save[0] = self.m
                self.save[1] = self.r


def _tie(never, src, v):
    if v.shape[1] == 256:
        src = jnp.concatenate([src, src], axis=1)
    return jax.lax.select(never[v.shape[1]], src, v)


def _norm_items(x_ref, col0, zb, zr, stats0=None):
    st = [_Stats(x_ref, col0, load=stats0), _Stats(x_ref, col0 + 256)]
    held, pending = {}, {}

    def put(t, j, bt):
        for u, v in enumerate(_b_ops(*[bt[k] for k in HP])):
            e = TILE[(t, u)]
            if e == 48:
                zb[24, j:j + 8, :128] = v.astype(BF16)
            elif (e ^ 1, j) not in pending:
                pending[(e, j)] = v
            else:
                other = pending.pop((e ^ 1, j))
                pair = [v, other] if e % 2 == 0 else [other, v]
                zb[e // 2, j:j + 8, :] = jnp.concatenate(pair, axis=1).astype(BF16)

    def zblock(j, kq, side, tie):
        out = {}
        for p in range(2):
            ls = slice(128 * side, 128 * side + 128)
            m, r = st[p].m[:, ls], st[p].r[:, ls]
            if p == 0:
                m = tie(m)
            for h in range(2):
                r0 = 128 * (kq + h) + j
                out[(h, p)] = (x_ref[r0:r0 + 8, st[p].cs].astype(F32)[:, ls] - m) * r
        return out

    def step1(j, tie):
        b11 = held[(j, 11)] = zblock(j, 0, 0, tie)
        put(1, j, b11)

    def step2(j, tie):
        b11, b22 = held[(j, 11)], zblock(j, 2, 1, tie)
        held[(j, 22)] = b22
        put(4, j, b22)
        put(0, j, {k: b11[k] - b22[k] for k in HP})

    def step3(j, tie):
        b11, b22, b12 = held[(j, 11)], held[(j, 22)], zblock(j, 0, 1, tie)
        put(2, j, {k: b12[k] - b22[k] for k in HP})
        put(5, j, {k: b11[k] - b12[k] for k in HP})

    def step4(j, tie):
        b11, b22, b21 = held[(j, 11)], held[(j, 22)], zblock(j, 2, 0, tie)
        put(3, j, {k: b21[k] - b11[k] for k in HP})
        put(6, j, {k: b21[k] - b22[k] for k in HP})

    def zrem(p, r0, tie):
        m = tie(st[p].m)
        xf = x_ref[2 * KH + r0:2 * KH + r0 + 32, st[p].cs].astype(F32)
        z = (xf.reshape(4, 8, 256) - m[None]) * st[p].r[None]
        zr[r0:r0 + 32, pl.ds(256 * p, 256)] = z.reshape(32, 256).astype(BF16)

    items = st[0].items + st[1].items
    items += [(functools.partial(zrem, 0, r0), 28) for r0 in range(0, KR, 32)]
    for j in range(0, 128, 8):
        items += [(functools.partial(step1, j), 20.5), (functools.partial(step2, j), 33),
                  (functools.partial(step3, j), 37), (functools.partial(step4, j), 37)]
    items += [(functools.partial(zrem, 1, r0), 28) for r0 in range(0, KR, 32)]
    return items


def _time_slots(items, tail, end):
    room = [0.0 if t < PACE["lag"] else
            PACE["stats"] if t < PACE["split"] else PACE["ops"]
            for t in range(0, end, 8)]
    room += [PACE["extra_room"]] * (PACE["extra"] // 8)
    scale = sum(room) / sum(cost for _, cost in items)
    pos, cum, acc, k = [], 0, 0.0, 0
    for _, cost in items:
        while acc + room[k] <= scale * cum + 1e-9:
            acc += room[k]
            k += 1
        pos.append(8 * k)
        cum += cost
    t0, t1 = PACE["tail"]
    return pos + [end + t0 + (t1 - t0) * k / len(tail) for k in range(len(tail))]


def _mm_group(a_ref, ar_ref, e_ref, early, closed, zb, zr, o_ref, col0, items, tail, never,
              after_rows=None):
    rounds = _rounds(early)
    timed = [i == 0 or len(r) == 4 for i, r in enumerate(rounds)]
    pos = _time_slots(items, tail, Q * sum(timed))
    items = items + tail
    state = [0, 0]

    def release(mt):
        lo, span = state[1], mt.shape[0]
        while state[0] < len(items) and pos[state[0]] < lo + span:
            rr = min(span - 8, int(pos[state[0]] - lo) // 8 * 8)
            items[state[0]][0](functools.partial(_tie, never, mt[rr:rr + 8, :128]))
            state[0] += 1
        state[1] += span

    def prod(t, u, cuts=(0, Q)):
        ea, eb = 7 * t + u, TILE[(t, u)]
        parts = [jnp.dot(_unpack(a_ref[ea // 2, pl.ds(lo // 2, (hi - lo) // 2),
                                       pl.ds(128 * (ea % 2), 128)]),
                         zb[eb // 2, :, pl.ds(128 * (eb % 2), 128)],
                         preferred_element_type=F32)
                 for lo, hi in zip(cuts[:-1], cuts[1:])]
        return parts[0] if len(parts) == 1 else jnp.concatenate(parts, axis=0)

    stored = {}
    for rnd, is_timed in zip(rounds, timed):
        if closed and not is_timed:
            cuts = {1: (0, 48, 80, 112, Q), 2: (0, 80, Q)}[len(rnd)]
            ps = [prod(t, u, cuts) for t, u in rnd]
        else:
            ps = [prod(t, u) for t, u in rnd]
        terms = {}
        for (t, u), p in zip(rnd, ps):
            for f, sign in COEF[t]:
                terms.setdefault((f, u), []).append((sign, p))
        for (f, u), tm in terms.items():
            if (f, u) in stored:
                tm.append((stored[(f, u)], e_ref[f, u]))
            plus = [p for sign, p in tm if sign > 0]
            minus = [p for sign, p in tm if sign < 0]
            stored[(f, u)] = 1 if plus else -1
            val = functools.reduce(jnp.add, plus or minus)
            e_ref[f, u] = functools.reduce(jnp.subtract, minus, val) if plus else val
        if is_timed:
            release(ps[0])
    assert min(stored.values()) > 0
    rem = jnp.dot(_unpack(ar_ref[...])[:, :KX], zr[...], preferred_element_type=F32)
    release(rem)
    assert state[0] == len(items)

    def quadrant(f, q, p, base):
        if (q, p) == (0, 0):
            return base + e_ref[f, 0] + e_ref[f, 3] + e_ref[f, 4] + e_ref[f, 6]
        if (q, p) == (0, 1):
            return base + e_ref[f, 2] + e_ref[f, 4]
        if (q, p) == (1, 0):
            return base + e_ref[f, 1] + e_ref[f, 3]
        return base - e_ref[f, 0] + e_ref[f, 1] + e_ref[f, 2] + e_ref[f, 5]

    for half in range(2):
        for q in range(2):
            r0 = half * H + q * Q
            for p in range(2):
                c0 = 256 * p
                left = quadrant(2 * half, q, p, rem[r0:r0 + Q, c0:c0 + 128])
                right = quadrant(2 * half + 1, q, p, rem[r0:r0 + Q, c0 + 128:c0 + 256])
                o_ref[pl.ds(r0, Q), pl.ds(col0 + c0, 256)] = jnp.concatenate(
                    [left, right], axis=1).astype(BF16)
            if after_rows is not None:
                after_rows(r0)


def _kernel(x_hbm, g_hbm, b_hbm, w_hbm, o_hbm,
            xbuf, obuf, gbuf, bbuf, wbuf, a_ref, ar_ref, e_ref,
            zb0, zr0, zb1, zr1, c_ref, sem_x0, sem_w, sem_x, sem_o):
    S = xbuf.shape[0]
    n_ramp = sum(RAMP)
    n_body = (S - 1 - n_ramp) // SPB

    def x0_copy(h):
        cols = pl.ds(GW * h, GW)
        return pltpu.make_async_copy(x_hbm.at[0, :, cols], xbuf.at[0, :, cols],
                                     sem_x0.at[h])

    def x_copy(s):
        return pltpu.make_async_copy(x_hbm.at[s], xbuf.at[s], sem_x.at[s])

    def o_part_start(s, h, r0, rows):
        sl = (s, pl.ds(r0, rows), pl.ds(GW * h, GW))
        pltpu.make_async_copy(obuf.at[sl], o_hbm.at[sl], sem_o).start()

    def o_start(s0, n):
        for c in range(2 * GW // 128):
            sl = (pl.ds(s0, n), slice(None), pl.ds(c * 128, 128))
            pltpu.make_async_copy(obuf.at[sl], o_hbm.at[sl], sem_o).start(priority=c % 2)

    w_copies = [pltpu.make_async_copy(g_hbm, gbuf, sem_w.at[0]),
                pltpu.make_async_copy(b_hbm, bbuf, sem_w.at[1]),
                pltpu.make_async_copy(w_hbm, wbuf, sem_w.at[2])]

    head = w_copies[::-1] + [x0_copy(0), x0_copy(1)]

    def issue_head(k, carry):
        for kk, cp in enumerate(head):
            pl.when(k == kk)(cp.start)
        return carry

    jax.lax.fori_loop(0, len(head), issue_head, 0)

    def issue_x(s, carry):
        x_copy(s).start()
        return carry

    jax.lax.fori_loop(1, S, issue_x, 0)

    row = jax.lax.broadcasted_iota(jnp.int32, (16, GW), 0)
    ones = jnp.where(row < 3, 1.0, 0.0).astype(BF16)
    zr0[KR:, :] = ones
    zr1[KR:, :] = ones

    for c in w_copies:
        c.wait()
    _prep_weights(gbuf, bbuf, wbuf, a_ref, ar_ref)
    x0_copy(0).wait()
    for item, _ in _norm_items(xbuf.at[0], 0, zb0, zr0):
        item(lambda v: v)
    x0_copy(1).wait()
    gv = jnp.broadcast_to(gbuf[...].astype(F32).reshape(1, D)[:, :128], (8, 128))
    gv2 = jnp.concatenate([gv, gv], axis=1)
    never = {128: gv != gv, 256: gv2 != gv2}

    def mm(k, n, *args):
        _mm_group(a_ref, ar_ref, e_ref.at[k % 2], -k % 4, k == n - 1, *args)

    def ahead(i, h):
        return _Stats(xbuf.at[i], GW * h, save=c_ref.at[h]).items

    def block(i0, n, write):
        for u in range(n):
            i = i0 + u
            nxt = jnp.minimum(i + 1, S - 1)
            mm(2 * u, 2 * n, zb0, zr0, obuf.at[i], 0,
               _norm_items(xbuf.at[i], GW, zb1, zr1, c_ref.at[1]), ahead(nxt, 0), never)
            after_rows = None
            if write and u == n - 1:
                pl.when(i == S - 1)(functools.partial(o_part_start, i, 0, 0, D))

                def after_rows(r0, i=i):
                    pl.when(i == S - 1)(functools.partial(o_part_start, i, 1, r0, Q))
            mm(2 * u + 1, 2 * n, zb1, zr1, obuf.at[i], GW,
               _norm_items(xbuf.at[nxt], 0, zb0, zr0, c_ref.at[0]), ahead(nxt, 1),
               never, after_rows)
            if write:
                if (W_START - 2 - n_ramp) % SPB == u:
                    pl.when(i == W_START - 1)(functools.partial(o_start, 0, W_START))
                pl.when(jnp.logical_and(i >= W_START, i < S - 1))(
                    functools.partial(o_start, i, 1))

    mm(0, 1, zb0, zr0, obuf.at[0], 0, _norm_items(xbuf.at[0], GW, zb1, zr1), [], never)
    x_copy(1).wait()
    mm(0, 1, zb1, zr1, obuf.at[0], GW, _norm_items(xbuf.at[1], 0, zb0, zr0), ahead(1, 1),
       never)
    i = 1
    for n in RAMP:
        for u in range(n):
            x_copy(i + u + 1).wait()
        block(i, n, False)
        i += n

    def body(j, carry):
        i0 = 1 + n_ramp + j * SPB
        for u in range(SPB - 1):
            x_copy(i0 + u + 1).wait()
        pl.when(j < n_body - 1)(x_copy(jnp.minimum(i0 + SPB, S - 1)).wait)
        block(i0, SPB, True)
        return carry

    jax.lax.fori_loop(0, n_body, body, 0)
    pltpu.make_async_copy(obuf, o_hbm, sem_o).wait()


@jax.jit
def pallas_standalone__layernorm_linear__sampling_kernel(
    x: jax.Array,
    g: jax.Array,
    b: jax.Array,
    w: jax.Array,
):
    B, S, d = x.shape
    assert d == D and B == 2 * GW and (S - 1 - sum(RAMP)) % SPB == 0
    assert 1 + sum(RAMP) < W_START < S
    xt = jnp.transpose(x, (1, 2, 0))
    out = pl.pallas_call(
        _kernel,
        in_specs=[pl.BlockSpec(memory_space=pl.ANY)] * 4,
        out_specs=pl.BlockSpec(memory_space=pl.ANY),
        out_shape=jax.ShapeDtypeStruct((S, D, B), x.dtype),
        scratch_shapes=[
            pltpu.VMEM((S, D, B), BF16),
            pltpu.VMEM((S, D, B), BF16),
            pltpu.VMEM((D,), BF16),
            pltpu.VMEM((D,), BF16),
            pltpu.VMEM((D, D), BF16),
            pltpu.VMEM((25, Q // 2, 256), U32),
            pltpu.VMEM((D // 2, 128), U32),
            pltpu.VMEM((2, 4, 7, Q, 128), F32),
            pltpu.VMEM((25, 128, 256), BF16),
            pltpu.VMEM((KX, GW), BF16),
            pltpu.VMEM((25, 128, 256), BF16),
            pltpu.VMEM((KX, GW), BF16),
            pltpu.VMEM((2, 2, 8, 256), F32),
            pltpu.SemaphoreType.DMA((2,)),
            pltpu.SemaphoreType.DMA((3,)),
            pltpu.SemaphoreType.DMA((S,)),
            pltpu.SemaphoreType.DMA(()),
        ],
        compiler_params=pltpu.CompilerParams(
            vmem_limit_bytes=110 * 1024 * 1024,
            disable_bounds_checks=True,
            disable_semaphore_checks=True,
        ),
    )(xt, g, b, w)
    return jnp.transpose(out, (2, 0, 1))
```
